```python
import jax
import jax.numpy as jnp

def _softmax(x, axis=-1):
    return jax.nn.softmax(x, axis=axis)
def _gelu(x):
    return jax.nn.gelu(x, approximate=True)
def _silu(x):
    return jax.nn.silu(x)
def _sigmoid(x):
    return jax.nn.sigmoid(x)
def _layernorm(x, axis=-1, eps=1e-5):
    m = jnp.mean(x, axis=axis, keepdims=True)
    v = jnp.var(x, axis=axis, keepdims=True)
    return (x - m) / jnp.sqrt(v + eps)
def _scatter_add(tgt, idx, src, axis=0):
    return tgt.at[idx].add(src)
def _segment_sum(src, seg, n):
    return jax.ops.segment_sum(src, seg, n)
class _Rng:
    def __init__(self, key):
        self._k = key
    def _next(self):
        self._k, sub = jax.random.split(self._k)
        return sub
    def normal(self, shape):
        return jax.random.normal(self._next(), shape, dtype=jnp.bfloat16)
    def randint(self, lo, hi, shape):
        return jax.random.randint(self._next(), shape, lo, hi, dtype=jnp.int32)
    def uniform(self, shape, lo=0.0, hi=1.0):
        return jax.random.uniform(self._next(), shape, jnp.bfloat16, lo, hi)
    def permutation(self, n):
        return jax.random.permutation(self._next(), n)


kernel_name = 'concat_heads__compressed_kv_cla__spectral_gfnet__prompt'

def setup_inputs():
    _rng = _Rng(jax.random.key(int.from_bytes(__import__("os").urandom(4), "little")))
    _w = (lambda a: (lambda t: t.astype(jnp.bfloat16) if jnp.issubdtype(t.dtype, jnp.floating) else t)(jnp.asarray(a)))
    def _A_setup():
        B, H, Sq, Sk, D, M = 1, 32, 2048, 2048, 128, 1024
        Dc = 4 * D
        return {
            "x": _w((lambda *s: _rng.normal(s) * 0.05)(B, Sq, M)),
            "c_kv": _w((lambda *s: _rng.normal(s) * 0.05)(B, Sk, Dc)),
            "w_q": _w((lambda *s: _rng.normal(s) * 0.05)(M, H, D) * (M ** -0.5)),
            "w_uk": _w((lambda *s: _rng.normal(s) * 0.05)(Dc, H, D) * (Dc ** -0.5)),
            "w_uv": _w((lambda *s: _rng.normal(s) * 0.05)(Dc, H, D) * (Dc ** -0.5)),
            "w_o": _w((lambda *s: _rng.normal(s) * 0.05)(H, D, M) * ((H * D) ** -0.5)),
        }
    _A_in = _A_setup()

    def _B_setup():
        B, S, D = 1, 2048, 1024
        Df = D // 2 + 1
        return {
            "x": _w((lambda *s: _rng.normal(s) * 0.05)(B, S, D)),
            "w_r": _w((lambda *s: _rng.normal(s) * 0.05)(S, Df) * 0.02),
            "w_i": _w((lambda *s: _rng.normal(s) * 0.05)(S, Df) * 0.02),
        }
    _B_in = _B_setup()

    return {
        "A_x": _A_in["x"],
        "A_c_kv": _A_in["c_kv"],
        "A_w_q": _A_in["w_q"],
        "A_w_uk": _A_in["w_uk"],
        "A_w_uv": _A_in["w_uv"],
        "A_w_o": _A_in["w_o"],
        "B_x": _B_in["x"],
        "B_w_r": _B_in["w_r"],
        "B_w_i": _B_in["w_i"],
    }

def reference(A_x, A_c_kv, A_w_q, A_w_uk, A_w_uv, A_w_o, B_x, B_w_r, B_w_i):
    def _A_ref(x, c_kv, w_q, w_uk, w_uv, w_o):
        B, Sq, M = x.shape[0], x.shape[1], x.shape[2]
        Sk = c_kv.shape[1]
        H, D = w_q.shape[1], w_q.shape[2]
        q = jnp.einsum("bqm,mhd->bhqd", x, w_q)
        k = jnp.einsum("bkc,chd->bhkd", c_kv, w_uk)
        v = jnp.einsum("bkc,chd->bhkd", c_kv, w_uv)
        scores = jnp.einsum("bhqd,bhkd->bhqk", q, k) * (D ** -0.5)
        off = Sk - Sq
        qi = jnp.arange(Sq)[:, None]
        kj = jnp.arange(Sk)[None, :]
        cmask = kj <= (qi + off)
        scores = jnp.where(cmask[None, None], scores, -1e9)
        p = _softmax(scores, axis=-1)
        ctx = jnp.einsum("bhqk,bhkd->bhqd", p, v)
        return jnp.einsum("bhqd,hdm->bqm", ctx, w_o)

    def _B_ref(x, w_r, w_i):
        B, S, D = x.shape
        X = (lambda x, axes=(-2,-1): jnp.fft.rfft2(x.astype(jnp.float32), axes=axes))(x, axes=(-2, -1))
        W = w_r + 1j * w_i
        X = X * W
        y = (lambda x, s, axes=(-2,-1): jnp.fft.irfft2(x, s=s, axes=axes).astype(jnp.bfloat16))(X, (S, D), axes=(-2, -1))
        return y

    a = _A_ref(A_x, A_c_kv, A_w_q, A_w_uk, A_w_uv, A_w_o)
    b = _B_ref(B_x, B_w_r, B_w_i)
    return jnp.concatenate([a, b], axis=-1)
```

```python
import functools
import numpy as np
import ml_dtypes
import jax
import jax.numpy as jnp
from jax.experimental import pallas as pl
from jax.experimental.pallas import tpu as pltpu

f32, bf16, u32 = jnp.float32, jnp.bfloat16, jnp.uint32
S, DM, H, D, DC = 2048, 1024, 32, 128, 512
NT = (((1,), (1,)), ((), ()))
QSCALE = float((D ** -0.5) * 1.4426950408889634)
R2 = float(np.sqrt(0.5))
NPAIR = H // 2


def _lane_freq():
    v = np.zeros((4, 128), np.int64)
    for p in range(4):
        ka, kb = (0, 4) if p == 0 else (p, 8 - p)
        v[p, :64] = ka + 8 * np.arange(64)
        v[p, 64:] = kb + 8 * np.arange(64)
    return v


def _fwd_butterfly8(x):
    a0, a1, a2, a3 = x[0] + x[4], x[1] + x[5], x[2] + x[6], x[3] + x[7]
    c0, c1, c2, c3 = x[0] - x[4], x[1] - x[5], x[2] - x[6], x[3] - x[7]
    s02, s13 = a0 + a2, a1 + a3
    d02, d13 = a0 - a2, a1 - a3
    t1, t2 = (c1 - c3) * R2, (c1 + c3) * R2
    return [(s02, s13), (c0 + t1, c2 + t2), (d02, d13), (c0 - t1, c2 - t2)]


def _inv_butterfly8(u):
    (s02, s13), (b1r, b1i), (d02, d13), (b3r, b3i) = u
    a0, a2 = s02 + d02, s02 - d02
    a1, a3 = s13 + d13, s13 - d13
    c0, t1 = b1r + b3r, b1r - b3r
    c2, t2 = b1i + b3i, b1i - b3i
    c1, c3 = (t1 + t2) * R2, (t2 - t1) * R2
    return [a0 + c0, a1 + c1, a2 + c2, a3 + c3, a0 - c0, a1 - c1, a2 - c2, a3 - c3]


def _d_axis_mats():
    v = _lane_freq()
    d = np.arange(DM)
    eye = np.eye(8)
    F = np.zeros((DM, 4, 2, 128))
    G = np.zeros((4, 2, 128, DM))
    for p in range(4):
        for l in range(128):
            th = 2 * np.pi * ((v[p, l] * d) % DM) / DM
            if v[p, l] == 0:
                ny = np.where(d % 2 == 0, 1.0, -1.0)
                F[:, p, 0, l], F[:, p, 1, l] = 1.0, ny
                G[p, 0, l], G[p, 1, l] = 1.0 / DM, ny / DM
            else:
                F[:, p, 0, l], F[:, p, 1, l] = np.cos(th), -np.sin(th)
                G[p, 0, l], G[p, 1, l] = 2 * np.cos(th) / DM, -2 * np.sin(th) / DM
    F = F.reshape(8, 128, 1024)
    L = np.array([[o for pr in _fwd_butterfly8([eye[i, j] for j in range(8)]) for o in pr] for i in range(8)])
    Mfull = np.einsum('ji,inc->jnc', np.linalg.inv(L), F)
    K = np.array([_inv_butterfly8([(eye[i, 2 * q], eye[i, 2 * q + 1]) for q in range(4)]) for i in range(8)])
    Ufull = np.einsum('sbn,bj->sjn', G.reshape(1024, 8, 128), np.linalg.inv(K))
    M = np.stack([Mfull[2 * p:2 * p + 2, :, 256 * p:256 * p + 256].reshape(256, 256) for p in range(4)])
    Mi = np.stack([Ufull[256 * p:256 * p + 256, 2 * p:2 * p + 2, :].reshape(256, 256) for p in range(4)])
    return M, Mi


def _s_axis_mats():
    A = np.zeros((16, 256, 256))
    Ai = np.zeros((16, 256, 256))
    m = np.arange(128)
    b = np.arange(128)
    for r in range(16):
        th = 2 * np.pi * (np.outer(b, 16 * m + r) % S) / S
        Mr, Mi = np.cos(th), -np.sin(th)
        A[r] = np.block([[Mr, -Mi], [Mi, Mr]])
        Nr, Ni = np.cos(th).T / S, np.sin(th).T / S
        Ai[r] = np.block([[Nr, -Ni], [Ni, Nr]])
    return A, Ai


def _np_consts():
    M, Mi = _d_axis_mats()
    A, Ai = _s_axis_mats()
    c = lambda a: np.asarray(a, np.float32).astype(ml_dtypes.bfloat16)
    return c(M), c(Mi), c(A), c(Ai)


def _dft16(zr, zi, sign):
    def bfly4(r, i):
        t0r, t0i = r[0] + r[2], i[0] + i[2]
        t1r, t1i = r[0] - r[2], i[0] - i[2]
        t2r, t2i = r[1] + r[3], i[1] + i[3]
        t3r, t3i = r[1] - r[3], i[1] - i[3]
        if sign < 0:
            o1r, o1i, o3r, o3i = t1r + t3i, t1i - t3r, t1r - t3i, t1i + t3r
        else:
            o1r, o1i, o3r, o3i = t1r - t3i, t1i + t3r, t1r + t3i, t1i - t3r
        return [t0r + t2r, o1r, t0r - t2r, o3r], [t0i + t2i, o1i, t0i - t2i, o3i]

    def twid(r, i, m):
        if m == 0:
            return r, i
        c = np.cos(2 * np.pi * m / 16)
        s = sign * np.sin(2 * np.pi * m / 16)
        if m == 4:
            return (-i, r) if s > 0 else (i, -r)
        if m in (2, 6):
            cs = 1 if c > 0 else -1
            ss = 1 if s > 0 else -1
            a = (r - i) if cs * ss > 0 else (r + i)
            b = (i + r) if cs * ss > 0 else (i - r)
            return a * (cs * R2), b * (cs * R2)
        c, s = float(c), float(s)
        return r * c - i * s, i * c + r * s

    yr = [[None] * 4 for _ in range(4)]
    yi = [[None] * 4 for _ in range(4)]
    for b in range(4):
        r, i = bfly4([zr[4 * a + b] for a in range(4)], [zi[4 * a + b] for a in range(4)])
        for c in range(4):
            yr[c][b], yi[c][b] = twid(r[c], i[c], b * c)
    outr, outi = [None] * 16, [None] * 16
    for c in range(4):
        r, i = bfly4(yr[c], yi[c])
        for d in range(4):
            outr[c + 4 * d], outi[c + 4 * d] = r[d], i[d]
    return outr, outi


def _lo(u):
    return pltpu.bitcast(u << 16, f32)


def _hi(u):
    return pltpu.bitcast(u & jnp.uint32(0xFFFF0000), f32)


def _pack2(lo, hi):
    lo_b = pltpu.bitcast(lo.astype(bf16).astype(f32), u32) >> 16
    hi_b = pltpu.bitcast(hi.astype(bf16).astype(f32), u32)
    return lo_b | hi_b


BQ = 256
NBLK = S // BQ


def _kernel(x_hbm, c_hbm, wq_hbm, wk_hbm, wv_hbm, wo_hbm, bx_hbm, wr_hbm, wi_hbm, m_hbm, mi_hbm, a_hbm, ai_hbm,
            out_hbm,
            x_v, c_v, wq_buf, wk_buf, wv_buf, wo_buf, wq_s, wkv_s, q_s, k_s, v_s, ctx_s, acc,
            xbuf, wraw, wny, wt, ubuf, m_v, mi_v, a_v, ai_v, ybuf,
            sem_x, sem_w, sem_c, sem_wt, sem_o):
    def bx_copy(a):
        return pltpu.make_async_copy(bx_hbm.bitcast(u32).at[:, a, :], xbuf.at[a], sem_x.at[a])

    def a_copy(hbm, dst, a, k):
        return pltpu.make_async_copy(hbm.at[pl.ds(2 * a, 2)], dst.at[pl.ds(2 * a, 2)], sem_c.at[k, a])

    m_copy = pltpu.make_async_copy(m_hbm, m_v, sem_c.at[2, 0])
    mi_copy = pltpu.make_async_copy(mi_hbm, mi_v, sem_c.at[2, 1])
    xa_copy = pltpu.make_async_copy(x_hbm, x_v, sem_c.at[2, 2])
    c_copy = pltpu.make_async_copy(c_hbm, c_v, sem_c.at[2, 3])

    def wraw_copies(ri):
        src = (wr_hbm, wi_hbm)[ri]
        cps = [pltpu.make_async_copy(src.at[0:512, pl.ds(128 * a, 128)], wraw.at[ri, a], sem_wt.at[ri, a]) for a in range(16)]
        cps.append(pltpu.make_async_copy(src.at[pl.ds(512, 1), :], wny.at[ri], sem_wt.at[ri, 16]))
        return cps

    def w_copies(j, slot):
        return (pltpu.make_async_copy(wq_hbm.bitcast(u32).at[:, j, :], wq_buf.at[slot], sem_w.at[0, slot]),
                pltpu.make_async_copy(wk_hbm.bitcast(u32).at[:, j, :], wk_buf.at[slot], sem_w.at[1, slot]),
                pltpu.make_async_copy(wv_hbm.bitcast(u32).at[:, j, :], wv_buf.at[slot], sem_w.at[2, slot]),
                pltpu.make_async_copy(wo_hbm.at[j], wo_buf.at[slot], sem_w.at[3, slot]))

    bx_copy(0).start(); m_copy.start(); a_copy(a_hbm, a_v, 0, 0).start()
    for a in range(1, 8):
        bx_copy(a).start(); a_copy(a_hbm, a_v, a, 0).start()
    for ri in range(2):
        for cp in wraw_copies(ri): cp.start()
    c_copy.start()
    for cp in w_copies(0, 0): cp.start()
    xa_copy.start()
    mi_copy.start()
    for a in range(8): a_copy(ai_hbm, ai_v, a, 1).start()

    lane = jax.lax.broadcasted_iota(jnp.int32, (128, 128), 1)

    m_copy.wait()

    def p1(a, carry):
        bx_copy(a).wait(); a_copy(a_hbm, a_v, a, 0).wait()
        xb = []
        for b in range(8):
            u = xbuf[a, :, 128 * b:128 * b + 128]
            xb.append(jnp.concatenate([_lo(u), _hi(u)], axis=0))
        Bp = _fwd_butterfly8(xb)
        T = [jnp.dot(jnp.concatenate([Bp[p][0].astype(bf16), Bp[p][1].astype(bf16)], axis=1), m_v[p],
                     preferred_element_type=f32) for p in range(4)]
        for h in range(2):
            r = 2 * a + h
            tr = [T[p][128 * h:128 * h + 128, 0:128] for p in range(4)]
            ti = [T[p][128 * h:128 * h + 128, 128:256] for p in range(4)]
            ny = jnp.where(lane == 0, ti[0], 0.0)
            ti[0] = jnp.where(lane == 0, 0.0, ti[0])
            rhs = jnp.concatenate([jnp.concatenate(tr, axis=1), jnp.concatenate(ti, axis=1)], axis=0).astype(bf16)
            U = jnp.dot(a_v[r], rhs, preferred_element_type=f32)
            ubuf[r, :, :, 0:512] = U.reshape(2, 128, 512)
            Un = jnp.dot(a_v[r, :, 0:128], ny.astype(bf16), preferred_element_type=f32)
            ubuf[r, :, :, 512:640] = Un.reshape(2, 128, 128)
        return carry
    jax.lax.fori_loop(0, 8, p1, 0)

    for ri in range(2):
        cps = wraw_copies(ri)
        for cp in cps: cp.wait()
    wu = wraw.bitcast(u32)

    def wpass(a, carry):
        a0 = pl.multiple_of(a * 128, 128)
        for ri in range(2):
            halves = {}
            for c in range(4):
                u = wu[ri, a, pl.ds(c, 64, stride=4), :]
                halves[2 * c], halves[2 * c + 1] = _lo(u), _hi(u)
            for p in range(4):
                ka, kb = (0, 4) if p == 0 else (p, 8 - p)
                t = jnp.concatenate([halves[ka], halves[kb]], axis=0)
                wt[ri, pl.ds(a0, 128), 128 * p:128 * p + 128] = t.T
            ny = wny[ri, :, pl.ds(a0, 128)].astype(f32)
            wt[ri, pl.ds(a0, 128), 512:640] = jnp.broadcast_to(ny, (128, 128)).T
        return carry
    jax.lax.fori_loop(0, 16, wpass, 0)

    acc[...] = jnp.zeros(acc.shape, f32)
    c_copy.wait(); xa_copy.wait()
    row_i = jax.lax.broadcasted_iota(jnp.int32, (128, 128), 0)
    tri = lane <= row_i

    def proj(r0, nr):
        kv = jnp.dot(c_v[r0:r0 + nr, :], wkv_s[...], preferred_element_type=f32)
        k_s[r0:r0 + nr, :] = kv[:, 0:256].astype(bf16)
        v_s[r0:r0 + nr, :] = kv[:, 256:512].astype(bf16)
        q = jnp.dot(x_v[r0:r0 + nr, :], wq_s[...], preferred_element_type=f32)
        q_s[r0:r0 + nr, :] = (q * QSCALE).astype(bf16)

    def qk(hh, i):
        c0 = hh * D
        r0 = i * BQ
        kmain = r0 + 128
        q = q_s[r0:r0 + BQ, c0:c0 + D]
        s = jax.lax.dot_general(q, k_s[0:kmain, c0:c0 + D], NT, preferred_element_type=f32)
        sb = jax.lax.dot_general(q[128:256], k_s[kmain:kmain + 128, c0:c0 + D], NT, preferred_element_type=f32)
        top = s[0:128]
        top_d = jnp.where(tri, top[:, r0:kmain], -1e30)
        top = jnp.concatenate([top[:, 0:r0], top_d], axis=1) if r0 else top_d
        bot = jnp.concatenate([s[128:256], jnp.where(tri, sb, -1e30)], axis=1)
        return top, bot

    def sm_pv(hh, i, tb):
        c0 = hh * D
        r0 = i * BQ
        kmain = r0 + 128
        ps, ls = [], []
        for s in tb:
            m = jnp.max(s, axis=1, keepdims=True)
            p = jnp.exp2(s - m)
            ls.append(jnp.sum(p, axis=1, keepdims=True))
            ps.append(p.astype(bf16))
        pmain = jnp.concatenate([ps[0], ps[1][:, 0:kmain]], axis=0)
        o = jnp.dot(pmain, v_s[0:kmain, c0:c0 + D], preferred_element_type=f32)
        ob = jnp.dot(ps[1][:, kmain:kmain + 128], v_s[kmain:kmain + 128, c0:c0 + D], preferred_element_type=f32)
        ctx_s[r0:r0 + 128, c0:c0 + D] = (o[0:128] / ls[0]).astype(bf16)
        ctx_s[r0 + 128:r0 + 256, c0:c0 + D] = ((o[128:256] + ob) / ls[1]).astype(bf16)

    def oproj(i, slot):
        r0 = i * BQ
        acc[r0:r0 + BQ, :] += jnp.dot(ctx_s[r0:r0 + BQ, :], wo_buf[slot], preferred_element_type=f32)

    def p2_unit(j, p):
        b0 = pl.multiple_of(j * 8, 8)
        ls = slice(128 * p, 128 * p + 128)
        ur = [ubuf[r, 0, pl.ds(b0, 8), ls] for r in range(16)]
        ui = [ubuf[r, 1, pl.ds(b0, 8), ls] for r in range(16)]
        xr, xi = _dft16(ur, ui, -1)
        yr, yi = [], []
        for a in range(16):
            wr = wt[0, pl.ds(128 * a + b0, 8), ls]
            wi = wt[1, pl.ds(128 * a + b0, 8), ls]
            yr.append(xr[a] * wr - xi[a] * wi)
            yi.append(xr[a] * wi + xi[a] * wr)
        vr, vi = _dft16(yr, yi, +1)
        for r in range(16):
            ubuf[r, 0, pl.ds(b0, 8), ls] = vr[r]
            ubuf[r, 1, pl.ds(b0, 8), ls] = vi[r]

    def a_iter(j, carry):
        slot = j % 2

        @pl.when(j + 1 < NPAIR)
        def _():
            for cp in w_copies(j + 1, 1 - slot): cp.start()
        for cp in w_copies(j, slot): cp.wait()
        u = wq_buf[slot]
        wq_s[:, 0:128] = _lo(u).astype(bf16); wq_s[:, 128:256] = _hi(u).astype(bf16)
        u = wk_buf[slot]
        wkv_s[:, 0:128] = _lo(u).astype(bf16); wkv_s[:, 128:256] = _hi(u).astype(bf16)
        u = wv_buf[slot]
        wkv_s[:, 256:384] = _lo(u).astype(bf16); wkv_s[:, 384:512] = _hi(u).astype(bf16)
        sc = {}
        def QK(i):
            for hh in range(2): sc[hh, i] = qk(hh, i)
        def PV(i):
            for hh in range(2): sm_pv(hh, i, sc.pop((hh, i)))
        proj(0, 512)
        QK(0)
        proj(512, 512)
        PV(0); QK(1)
        proj(1024, 512)
        PV(1); QK(2)
        proj(1536, 512)
        PV(2); QK(3); p2_unit(j, 0); oproj(0, slot)
        PV(3); QK(4); p2_unit(j, 1); oproj(1, slot)
        PV(4); QK(5); p2_unit(j, 2); oproj(2, slot); oproj(3, slot)
        PV(5); QK(6); p2_unit(j, 3); oproj(4, slot)
        PV(6); QK(7); p2_unit(j, 4); oproj(5, slot)
        PV(7); oproj(6, slot)
        oproj(7, slot)
        return carry
    jax.lax.fori_loop(0, NPAIR, a_iter, 0)

    mi_copy.wait()
    out_u = out_hbm.bitcast(u32)

    def y_copy(a):
        return pltpu.make_async_copy(ybuf.at[a], out_u.at[:, a, pl.ds(DM, DM)], sem_o.at[0, a])

    def o_copy(a):
        return pltpu.make_async_copy(x_v.at[pl.ds(a * 256, 256)].reshape(16, 16, DM),
                                     out_hbm.at[pl.ds(a * 16, 16), :, pl.ds(0, DM)], sem_o.at[1, a])

    def p3(a, carry):
        r0 = pl.multiple_of(a * 256, 256)
        x_v[pl.ds(r0, 256), :] = acc[pl.ds(r0, 256), :].astype(bf16)
        o_copy(a).start()
        a_copy(ai_hbm, ai_v, a, 1).wait()
        zs = []
        for h in range(2):
            r = 2 * a + h
            rhs = ubuf[r].reshape(256, 640).astype(bf16)
            Z = jnp.dot(ai_v[r], rhs[:, 0:512], preferred_element_type=f32)
            Zn = jnp.dot(ai_v[r, 0:128, :], rhs[:, 512:640], preferred_element_type=f32)
            zs.append((Z, Zn))
        U = []
        for p in range(4):
            rows = []
            for h in range(2):
                Z, Zn = zs[h]
                zr = Z[0:128, 128 * p:128 * p + 128]
                zi = Z[128:256, 128 * p:128 * p + 128]
                if p == 0:
                    zi = jnp.where(lane == 0, Zn, zi)
                rows.append(jnp.concatenate([zr, zi], axis=1))
            lhs = jnp.concatenate(rows, axis=0).astype(bf16)
            u = jnp.dot(lhs, mi_v[p], preferred_element_type=f32)
            U.append((u[:, 0:128], u[:, 128:256]))
        xs = _inv_butterfly8(U)
        for b in range(8):
            ybuf[a, :, 128 * b:128 * b + 128] = _pack2(xs[b][0:128], xs[b][128:256])
        y_copy(a).start()
        return carry
    jax.lax.fori_loop(0, 8, p3, 0)
    for a in range(8):
        y_copy(a).wait(); o_copy(a).wait()


_CONSTS = _np_consts()


@jax.jit
def pallas_concat_heads__compressed_kv_cla__spectral_gfnet__prompt_kernel(
        A_x, A_c_kv, A_w_q, A_w_uk, A_w_uv, A_w_o, B_x, B_w_r, B_w_i):
    vmem_mb = 110
    M, Mi, A, Ai = _CONSTS
    anyspec = pl.BlockSpec(memory_space=pl.ANY)
    V = pltpu.VMEM
    call = pl.pallas_call(
        _kernel,
        in_specs=[anyspec] * 13, out_specs=anyspec,
        out_shape=jax.ShapeDtypeStruct((128, 16, 2 * DM), bf16),
        scratch_shapes=[
            V((S, DM), bf16), V((S, DC), bf16),
            V((2, DM, D), u32), V((2, DC, D), u32), V((2, DC, D), u32), V((2, 256, DM), bf16),
            V((DM, 256), bf16), V((DC, 512), bf16),
            V((S, 256), bf16), V((S, 256), bf16), V((S, 256), bf16), V((S, 256), bf16), V((S, DM), f32),
            V((8, 128, DM), u32), V((2, 16, 512, 128), bf16), V((2, 1, S), bf16), V((2, S, 640), f32),
            V((16, 2, 128, 640), f32),
            V((4, 256, 256), bf16), V((4, 256, 256), bf16), V((16, 256, 256), bf16), V((16, 256, 256), bf16),
            V((8, 128, DM), u32),
            pltpu.SemaphoreType.DMA((8,)), pltpu.SemaphoreType.DMA((4, 2)), pltpu.SemaphoreType.DMA((3, 8)),
            pltpu.SemaphoreType.DMA((2, 17)), pltpu.SemaphoreType.DMA((2, 8)),
        ],
        compiler_params=pltpu.CompilerParams(vmem_limit_bytes=vmem_mb * 1024 * 1024),
    )
    o = call(A_x.reshape(S, DM), A_c_kv.reshape(S, DC), A_w_q, A_w_uk, A_w_uv, A_w_o.reshape(NPAIR, 256, DM),
             B_x.reshape(128, 16, DM), B_w_r.T, B_w_i.T, M, Mi, A, Ai)
    return o.reshape(1, S, 2 * DM)
```

```python
import functools
import numpy as np
import ml_dtypes
import jax
import jax.numpy as jnp
from jax.experimental import pallas as pl
from jax.experimental.pallas import tpu as pltpu

f32, bf16, u32 = jnp.float32, jnp.bfloat16, jnp.uint32
S, DM, H, D, DC = 2048, 1024, 32, 128, 512
NT = (((1,), (1,)), ((), ()))
QSCALE = float((D ** -0.5) * 1.4426950408889634)
R2 = float(np.sqrt(0.5))
NPAIR = H // 2


def _lane_freq():
    v = np.zeros((4, 128), np.int64)
    for p in range(4):
        ka, kb = (0, 4) if p == 0 else (p, 8 - p)
        v[p, :64] = ka + 8 * np.arange(64)
        v[p, 64:] = kb + 8 * np.arange(64)
    return v


def _fwd_butterfly8(x):
    a0, a1, a2, a3 = x[0] + x[4], x[1] + x[5], x[2] + x[6], x[3] + x[7]
    c0, c1, c2, c3 = x[0] - x[4], x[1] - x[5], x[2] - x[6], x[3] - x[7]
    s02, s13 = a0 + a2, a1 + a3
    d02, d13 = a0 - a2, a1 - a3
    t1, t2 = (c1 - c3) * R2, (c1 + c3) * R2
    return [(s02, s13), (c0 + t1, c2 + t2), (d02, d13), (c0 - t1, c2 - t2)]


def _inv_butterfly8(u):
    (s02, s13), (b1r, b1i), (d02, d13), (b3r, b3i) = u
    a0, a2 = s02 + d02, s02 - d02
    a1, a3 = s13 + d13, s13 - d13
    c0, t1 = b1r + b3r, b1r - b3r
    c2, t2 = b1i + b3i, b1i - b3i
    c1, c3 = (t1 + t2) * R2, (t2 - t1) * R2
    return [a0 + c0, a1 + c1, a2 + c2, a3 + c3, a0 - c0, a1 - c1, a2 - c2, a3 - c3]


def _d_axis_mats():
    v = _lane_freq()
    d = np.arange(DM)
    eye = np.eye(8)
    F = np.zeros((DM, 4, 2, 128))
    G = np.zeros((4, 2, 128, DM))
    for p in range(4):
        for l in range(128):
            th = 2 * np.pi * ((v[p, l] * d) % DM) / DM
            if v[p, l] == 0:
                ny = np.where(d % 2 == 0, 1.0, -1.0)
                F[:, p, 0, l], F[:, p, 1, l] = 1.0, ny
                G[p, 0, l], G[p, 1, l] = 1.0 / DM, ny / DM
            else:
                F[:, p, 0, l], F[:, p, 1, l] = np.cos(th), -np.sin(th)
                G[p, 0, l], G[p, 1, l] = 2 * np.cos(th) / DM, -2 * np.sin(th) / DM
    F = F.reshape(8, 128, 1024)
    L = np.array([[o for pr in _fwd_butterfly8([eye[i, j] for j in range(8)]) for o in pr] for i in range(8)])
    Mfull = np.einsum('ji,inc->jnc', np.linalg.inv(L), F)
    K = np.array([_inv_butterfly8([(eye[i, 2 * q], eye[i, 2 * q + 1]) for q in range(4)]) for i in range(8)])
    Ufull = np.einsum('sbn,bj->sjn', G.reshape(1024, 8, 128), np.linalg.inv(K))
    M = np.stack([Mfull[2 * p:2 * p + 2, :, 256 * p:256 * p + 256].reshape(256, 256) for p in range(4)])
    Mi = np.stack([Ufull[256 * p:256 * p + 256, 2 * p:2 * p + 2, :].reshape(256, 256) for p in range(4)])
    return M, Mi


def _s_axis_mats():
    A = np.zeros((16, 256, 256))
    Ai = np.zeros((16, 256, 256))
    m = np.arange(128)
    b = np.arange(128)
    for r in range(16):
        th = 2 * np.pi * (np.outer(b, 16 * m + r) % S) / S
        Mr, Mi = np.cos(th), -np.sin(th)
        A[r] = np.block([[Mr, -Mi], [Mi, Mr]])
        Nr, Ni = np.cos(th).T / S, np.sin(th).T / S
        Ai[r] = np.block([[Nr, -Ni], [Ni, Nr]])
    return A, Ai


def _np_consts():
    M, Mi = _d_axis_mats()
    A, Ai = _s_axis_mats()
    c = lambda a: np.asarray(a, np.float32).astype(ml_dtypes.bfloat16)
    return c(M), c(Mi), c(A), c(Ai)


def _bfly4(r, i, sign):
    t0r, t0i = r[0] + r[2], i[0] + i[2]
    t1r, t1i = r[0] - r[2], i[0] - i[2]
    t2r, t2i = r[1] + r[3], i[1] + i[3]
    t3r, t3i = r[1] - r[3], i[1] - i[3]
    if sign < 0:
        o1r, o1i, o3r, o3i = t1r + t3i, t1i - t3r, t1r - t3i, t1i + t3r
    else:
        o1r, o1i, o3r, o3i = t1r - t3i, t1i + t3r, t1r + t3i, t1i - t3r
    return [t0r + t2r, o1r, t0r - t2r, o3r], [t0i + t2i, o1i, t0i - t2i, o3i]


def _twid16(r, i, m, sign):
    if m == 0:
        return r, i
    c = np.cos(2 * np.pi * m / 16)
    s = sign * np.sin(2 * np.pi * m / 16)
    if m == 4:
        return (-i, r) if s > 0 else (i, -r)
    if m in (2, 6):
        cs = 1 if c > 0 else -1
        ss = 1 if s > 0 else -1
        a = (r - i) if cs * ss > 0 else (r + i)
        b = (i + r) if cs * ss > 0 else (i - r)
        return a * (cs * R2), b * (cs * R2)
    c, s = float(c), float(s)
    return r * c - i * s, i * c + r * s


def _dft16(zr, zi, sign):
    def bfly4(r, i):
        t0r, t0i = r[0] + r[2], i[0] + i[2]
        t1r, t1i = r[0] - r[2], i[0] - i[2]
        t2r, t2i = r[1] + r[3], i[1] + i[3]
        t3r, t3i = r[1] - r[3], i[1] - i[3]
        if sign < 0:
            o1r, o1i, o3r, o3i = t1r + t3i, t1i - t3r, t1r - t3i, t1i + t3r
        else:
            o1r, o1i, o3r, o3i = t1r - t3i, t1i + t3r, t1r + t3i, t1i - t3r
        return [t0r + t2r, o1r, t0r - t2r, o3r], [t0i + t2i, o1i, t0i - t2i, o3i]

    def twid(r, i, m):
        if m == 0:
            return r, i
        c = np.cos(2 * np.pi * m / 16)
        s = sign * np.sin(2 * np.pi * m / 16)
        if m == 4:
            return (-i, r) if s > 0 else (i, -r)
        if m in (2, 6):
            cs = 1 if c > 0 else -1
            ss = 1 if s > 0 else -1
            a = (r - i) if cs * ss > 0 else (r + i)
            b = (i + r) if cs * ss > 0 else (i - r)
            return a * (cs * R2), b * (cs * R2)
        c, s = float(c), float(s)
        return r * c - i * s, i * c + r * s

    yr = [[None] * 4 for _ in range(4)]
    yi = [[None] * 4 for _ in range(4)]
    for b in range(4):
        r, i = bfly4([zr[4 * a + b] for a in range(4)], [zi[4 * a + b] for a in range(4)])
        for c in range(4):
            yr[c][b], yi[c][b] = twid(r[c], i[c], b * c)
    outr, outi = [None] * 16, [None] * 16
    for c in range(4):
        r, i = bfly4(yr[c], yi[c])
        for d in range(4):
            outr[c + 4 * d], outi[c + 4 * d] = r[d], i[d]
    return outr, outi


def _lo(u):
    return pltpu.bitcast(u << 16, f32)


def _hi(u):
    return pltpu.bitcast(u & jnp.uint32(0xFFFF0000), f32)


def _recip(l):
    r = pl.reciprocal(l, approx=True)
    return r * (2.0 - l * r)


def _pack2(lo, hi):
    lo_b = pltpu.bitcast(lo.astype(bf16).astype(f32), u32) >> 16
    hi_b = pltpu.bitcast(hi.astype(bf16).astype(f32), u32)
    return lo_b | hi_b


BQ = 256
NBLK = S // BQ


def _strassen_lhs(a11, a12, a21, a22):
    return a11 + a22, a21 + a22, a11 + a12, a21 - a11, a12 - a22


def _strassen_rhs(b11, b12, b21, b22):
    return b11 + b22, b11, b12 - b22, b21 - b11, b22, b11 + b12, b21 + b22


def _strassen_mul(L, R):
    m = [jnp.dot(L[t](), R[t](), preferred_element_type=f32) for t in range(7)]
    return m[0] + m[3] - m[4] + m[6], m[2] + m[4], m[1] + m[3], m[0] - m[1] + m[2] + m[5]


def _ld(ref, r0, nr, c0, nc):
    return pltpu.bitcast(ref[r0 // 2:(r0 + nr) // 2, c0:c0 + nc], bf16)


def _st(ref, r0, c0, val):
    nr, nc = val.shape
    ref[r0 // 2:(r0 + nr) // 2, c0:c0 + nc] = pltpu.bitcast(val, u32)


def _kernel(x_hbm, c_hbm, wq_hbm, wk_hbm, wv_hbm, wo_hbm, bx_hbm, wr_hbm, wi_hbm, m_hbm, mi_hbm, a_hbm, ai_hbm,
            out_hbm,
            x_v, c_v, xs, cs, wq_buf, wk_buf, wv_buf, wo_buf, wq_s, wkv_s, wo_s, q_s, k_s, v_s, ctx_s, acc,
            xbuf, wraw, wny, wt, ubuf, m_v, mi_v, a_v, ai_v, ybuf, obuf, pb0, pb1, pb2, pb3,
            sem_x, sem_w, sem_c, sem_wt, sem_o, sem_xc):
    def bx_copy(a):
        return pltpu.make_async_copy(bx_hbm.bitcast(u32).at[:, a, :], xbuf.at[a], sem_x.at[a])

    def a_copy(hbm, dst, a, k):
        return pltpu.make_async_copy(hbm.at[pl.ds(2 * a, 2)], dst.at[pl.ds(2 * a, 2)], sem_c.at[k, a])

    m_copy = pltpu.make_async_copy(m_hbm, m_v, sem_c.at[2, 0])
    mi_copy = pltpu.make_async_copy(mi_hbm, mi_v, sem_c.at[2, 1])

    def xa_copy(a):
        return pltpu.make_async_copy(x_hbm.bitcast(u32).at[pl.ds(a * 128, 128)], x_v.at[pl.ds(a * 128, 128)], sem_xc.at[0, a])

    def c_copy(a):
        return pltpu.make_async_copy(c_hbm.bitcast(u32).at[pl.ds(a * 128, 128)], c_v.at[pl.ds(a * 128, 128)], sem_xc.at[1, a])

    def wraw_copies(ri):
        src = (wr_hbm, wi_hbm)[ri]
        cps = [pltpu.make_async_copy(src.at[0:512, pl.ds(128 * a, 128)], wraw.at[ri, a], sem_wt.at[ri, a]) for a in range(16)]
        cps.append(pltpu.make_async_copy(src.at[pl.ds(512, 1), :], wny.at[ri], sem_wt.at[ri, 16]))
        return cps

    def raw_copies(j, slot):
        return (pltpu.make_async_copy(wk_hbm.bitcast(u32).at[:, j, :], wk_buf.at[slot], sem_w.at[1, slot]),
                pltpu.make_async_copy(wv_hbm.bitcast(u32).at[:, j, :], wv_buf.at[slot], sem_w.at[2, slot]),
                pltpu.make_async_copy(wq_hbm.bitcast(u32).at[:, j, :], wq_buf.at[slot], sem_w.at[0, slot]))

    def wo_copy(j, slot):
        return pltpu.make_async_copy(wo_hbm.bitcast(u32).at[j], wo_buf.at[slot], sem_w.at[3, slot])

    bx_copy(0).start(); m_copy.start(); a_copy(a_hbm, a_v, 0, 0).start(); c_copy(0).start(); xa_copy(0).start()
    for a in range(1, 8):
        bx_copy(a).start(); a_copy(a_hbm, a_v, a, 0).start(); c_copy(a).start(); xa_copy(a).start()
    for cp in raw_copies(0, 0): cp.start()
    for ri in range(2):
        for cp in wraw_copies(ri): cp.start()
    for cp in raw_copies(1, 1): cp.start()
    wo_copy(0, 0).start()
    mi_copy.start()
    for a in range(8): a_copy(ai_hbm, ai_v, a, 1).start()

    lane = jax.lax.broadcasted_iota(jnp.int32, (128, 128), 1)

    m_copy.wait()

    def prepass(i):
        r = pl.multiple_of(i * 128, 128)
        h = pl.multiple_of(i * 64, 64)
        for src, dst, w in ((c_v, cs, 256), (x_v, xs, 512)):
            top = pltpu.bitcast(src[pl.ds(r, 64), :], bf16).astype(f32)
            bot = pltpu.bitcast(src[pl.ds(r + 64, 64), :], bf16).astype(f32)
            L = _strassen_lhs(top[:, 0:w], top[:, w:2 * w], bot[:, 0:w], bot[:, w:2 * w])
            for t in range(5): dst[t, pl.ds(h, 64), :] = pltpu.bitcast(L[t].astype(bf16), u32)

    def p1(a, carry):
        bx_copy(a).wait(); a_copy(a_hbm, a_v, a, 0).wait(); c_copy(a).wait(); xa_copy(a).wait()
        prepass(a)
        acc[pl.ds(pl.multiple_of(a * 256, 256), 256), :] = jnp.zeros((256, DM), f32)
        xb = []
        for b in range(8):
            u = xbuf[a, :, 128 * b:128 * b + 128]
            xb.append(jnp.concatenate([_lo(u), _hi(u)], axis=0))
        Bp = _fwd_butterfly8(xb)
        T = [jnp.dot(jnp.concatenate([Bp[p][0], Bp[p][1]], axis=1).astype(bf16), m_v[p],
                     preferred_element_type=f32) for p in range(4)]
        for h in range(2):
            r = 2 * a + h
            tr = [T[p][128 * h:128 * h + 128, 0:128] for p in range(4)]
            ti = [T[p][128 * h:128 * h + 128, 128:256] for p in range(4)]
            ny = jnp.where(lane == 0, ti[0], 0.0)
            ti[0] = jnp.where(lane == 0, 0.0, ti[0])
            rhs = jnp.concatenate([jnp.concatenate(tr, axis=1), jnp.concatenate(ti, axis=1)], axis=0).astype(bf16)
            U = jnp.dot(a_v[r], rhs, preferred_element_type=f32)
            ubuf[r, :, 0:128, 0:512] = U.reshape(2, 128, 512)
            Un = jnp.dot(a_v[r, :, 0:128], ny.astype(bf16), preferred_element_type=f32)
            ubuf[r, :, 0:128, 512:640] = Un.reshape(2, 128, 128)
        return carry
    jax.lax.fori_loop(0, 8, p1, 0)

    wu = wraw.bitcast(u32)

    def wpass(a, carry):
        a0 = pl.multiple_of(a * 128, 128)
        for ri in range(2):
            halves = {}
            for c in range(4):
                u = wu[ri, a, pl.ds(c, 64, stride=4), :]
                halves[2 * c], halves[2 * c + 1] = _lo(u), _hi(u)
            for p in range(4):
                ka, kb = (0, 4) if p == 0 else (p, 8 - p)
                t = jnp.concatenate([halves[ka], halves[kb]], axis=0)
                wt[ri, pl.ds(a0, 128), 128 * p:128 * p + 128] = t.T
            ny = wny[ri, :, pl.ds(a0, 128)].astype(f32)
            wt[ri, pl.ds(a0, 128), 512:640] = jnp.broadcast_to(ny, (128, 128)).T
        return carry

    def w_transpose():
        for ri in range(2):
            for cp in wraw_copies(ri): cp.wait()
        jax.lax.fori_loop(0, 16, wpass, 0, unroll=OPT["wunroll"])

    row_i = jax.lax.broadcasted_iota(jnp.int32, (128, 128), 0)
    tri = lane <= row_i

    def ldu(ref, *idx):
        return pltpu.bitcast(ref[idx], bf16)

    def kvproj(i):
        t0, b0 = 128 * i, 128 * i + 64
        h0 = 64 * i
        L = [lambda: ldu(cs, 0, slice(h0, h0 + 64), slice(None)), lambda: ldu(cs, 1, slice(h0, h0 + 64), slice(None)),
             lambda: ldu(c_v, slice(t0, t0 + 64), slice(0, 256)), lambda: ldu(c_v, slice(b0, b0 + 64), slice(256, 512)),
             lambda: ldu(cs, 2, slice(h0, h0 + 64), slice(None)), lambda: ldu(cs, 3, slice(h0, h0 + 64), slice(None)),
             lambda: ldu(cs, 4, slice(h0, h0 + 64), slice(None))]
        R = [(lambda t=t: ldu(wkv_s, t, slice(None), slice(None))) for t in range(7)]
        c11, c12, c21, c22 = _strassen_mul(L, R)
        r0 = 256 * i
        _st(k_s, r0, 0, c11.astype(bf16)); _st(v_s, r0, 0, c12.astype(bf16))
        _st(k_s, r0 + 128, 0, c21.astype(bf16)); _st(v_s, r0 + 128, 0, c22.astype(bf16))

    def qproj(i):
        t0, b0 = 128 * i, 128 * i + 64
        h0 = 64 * i
        L = [lambda: ldu(xs, 0, slice(h0, h0 + 64), slice(None)), lambda: ldu(xs, 1, slice(h0, h0 + 64), slice(None)),
             lambda: ldu(x_v, slice(t0, t0 + 64), slice(0, 512)), lambda: ldu(x_v, slice(b0, b0 + 64), slice(512, 1024)),
             lambda: ldu(xs, 2, slice(h0, h0 + 64), slice(None)), lambda: ldu(xs, 3, slice(h0, h0 + 64), slice(None)),
             lambda: ldu(xs, 4, slice(h0, h0 + 64), slice(None))]
        R = [(lambda t=t: ldu(wq_s, t, slice(None), slice(None))) for t in range(7)]
        c11, c12, c21, c22 = _strassen_mul(L, R)
        r0 = 256 * i
        _st(q_s, r0, 0, (jnp.concatenate([c11, c12], axis=1) * QSCALE).astype(bf16))
        _st(q_s, r0 + 128, 0, (jnp.concatenate([c21, c22], axis=1) * QSCALE).astype(bf16))

    def qk(hh, i):
        c0 = hh * D
        r0 = i * BQ
        kmain = r0 + 128
        q = _ld(q_s, r0, BQ, c0, D)
        s = jax.lax.dot_general(q, _ld(k_s, 0, kmain, c0, D), NT, preferred_element_type=f32)
        sb = jax.lax.dot_general(q[128:256], _ld(k_s, kmain, 128, c0, D), NT, preferred_element_type=f32)
        top = s[0:128]
        top_d = jnp.where(tri, top[:, r0:kmain], -1e30)
        top = jnp.concatenate([top[:, 0:r0], top_d], axis=1) if r0 else top_d
        bot = jnp.concatenate([s[128:256], jnp.where(tri, sb, -1e30)], axis=1)
        return top, bot

    Z = [0]
    pbufs = [pb0, pb1, pb2, pb3]

    def softmax(hh, i, tb):
        r0 = i * BQ
        kend = r0 + 256
        ls = []
        ps = []
        for half, s in enumerate(tb):
            kk = s.shape[1]
            if OPT["slab"]:
                sl = OPT["slab"]
                lparts, pparts = [], []
                for t in range(0, 128, sl):
                    ss = s[t:t + sl]
                    m = jnp.max(ss, axis=1, keepdims=True)
                    p = jnp.exp2(ss - m)
                    lparts.append(jnp.sum(p, axis=1, keepdims=True))
                    pb = p
                    if OPT["pbuf"]:
                        pb = p.astype(bf16)
                        pbufs[2 * hh + i % 2][(128 * half + t) // 2:(128 * half + t + sl) // 2, 0:kk] = pltpu.bitcast(pb, u32)
                    pparts.append(pb)
                ls.append(jnp.concatenate(lparts, axis=0))
                ps.append(jnp.concatenate(pparts, axis=0))
            else:
                m = jnp.max(s, axis=1, keepdims=True)
                p = jnp.exp2(s - m)
                ls.append(jnp.sum(p, axis=1, keepdims=True))
                pb = p
                if OPT["pbuf"]:
                    pb = p.astype(bf16)
                    pbufs[2 * hh + i % 2][64 * half:64 * half + 64, 0:kk] = pltpu.bitcast(pb, u32)
                ps.append(pb)
        return ps, ls

    def pv(hh, i, pl_):
        ps, ls = pl_
        c0 = hh * D
        r0 = i * BQ
        kmain = r0 + 128
        if OPT["pbuf"]:
            pmain = pltpu.bitcast(pbufs[2 * hh + i % 2][pl.ds(Z[0], 128), 0:kmain], bf16)
            pb = pltpu.bitcast(pbufs[2 * hh + i % 2][pl.ds(Z[0] + 64, 64), kmain:kmain + 128], bf16)
        else:
            pmain = jnp.concatenate([ps[0], ps[1][:, 0:kmain]], axis=0).astype(bf16)
            pb = ps[1][:, kmain:kmain + 128].astype(bf16)
        o = jnp.dot(pmain, _ld(v_s, 0, kmain, c0, D), preferred_element_type=f32)
        ob = jnp.dot(pb, _ld(v_s, kmain, 128, c0, D), preferred_element_type=f32)
        return o[0:128] * _recip(ls[0]), (o[128:256] + ob) * _recip(ls[1])

    def store_ctx(i, c0_, c1_):
        (a11, a21), (a12, a22) = c0_, c1_
        l1, l2, l5, l6, l7 = _strassen_lhs(a11, a12, a21, a22)
        for t, v in enumerate((l1, l2, a11, a22, l5, l6, l7)):
            ctx_s[64 * i:64 * i + 64, 128 * t:128 * t + 128] = pltpu.bitcast(v.astype(bf16), u32)

    def oproj(i, slot):
        r0 = i * BQ
        L = [(lambda t=t: ldu(ctx_s, slice(64 * i, 64 * i + 64), slice(128 * t, 128 * t + 128))) for t in range(7)]
        R = [(lambda t=t: ldu(wo_s, t, slice(None), slice(None))) for t in range(7)]
        c11, c12, c21, c22 = _strassen_mul(L, R)
        acc[r0:r0 + 128, 0:512] += c11
        acc[r0:r0 + 128, 512:1024] += c12
        acc[r0 + 128:r0 + 256, 0:512] += c21
        acc[r0 + 128:r0 + 256, 512:1024] += c22

    def unpack_kv(slot):
        uk, uv = wk_buf[slot], wv_buf[slot]
        def pair(u):
            return jnp.concatenate([_lo(u), _hi(u)], axis=1)
        R = _strassen_rhs(pair(uk[0:256]), pair(uv[0:256]), pair(uk[256:512]), pair(uv[256:512]))
        for t in range(7): wkv_s[t] = pltpu.bitcast(R[t].astype(bf16), u32)

    def unpack_q(slot):
        uq = wq_buf[slot]
        R = _strassen_rhs(_lo(uq[0:512]), _hi(uq[0:512]), _lo(uq[512:1024]), _hi(uq[512:1024]))
        for t in range(7): wq_s[t] = pltpu.bitcast(R[t].astype(bf16), u32)

    def unpack_weights(slot):
        unpack_kv(slot); unpack_q(slot)

    def prep_wo(slot):
        w = pltpu.bitcast(wo_buf[slot], bf16).astype(f32)
        R = _strassen_rhs(w[0:128, 0:512], w[0:128, 512:1024], w[128:256, 0:512], w[128:256, 512:1024])
        for t in range(7): wo_s[t] = pltpu.bitcast(R[t].astype(bf16), u32)

    def p2_unit(j, p, ps=(0, 1, 2), sub=(0, 1, 2, 3)):
        b0 = pl.multiple_of(j * 8, 8)
        bw = pl.multiple_of((j % 16) * 8, 8)
        ls = slice(128 * p, 128 * p + 128)
        def ld(idx):
            return ([ubuf[r, 0, pl.ds(b0, 8), ls] for r in idx], [ubuf[r, 1, pl.ds(b0, 8), ls] for r in idx])
        def sto(idx, vr, vi):
            for r, a_, b_ in zip(idx, vr, vi):
                ubuf[r, 0, pl.ds(b0, 8), ls] = a_
                ubuf[r, 1, pl.ds(b0, 8), ls] = b_
        for b in (sub if 0 in ps else ()):
            r, i = _bfly4(*ld([4 * a + b for a in range(4)]), -1)
            tw = [_twid16(r[c], i[c], b * c, -1) for c in range(4)]
            sto([4 * c + b for c in range(4)], [t[0] for t in tw], [t[1] for t in tw])
        for c in (sub if 1 in ps else ()):
            xr, xi = _bfly4(*ld([4 * c + b for b in range(4)]), -1)
            yr, yi = [], []
            for d in range(4):
                a = c + 4 * d
                wr = wt[0, pl.ds(128 * a + bw, 8), ls]
                wi = wt[1, pl.ds(128 * a + bw, 8), ls]
                yr.append(xr[d] * wr - xi[d] * wi)
                yi.append(xr[d] * wi + xi[d] * wr)
            r, i = _bfly4(yr, yi, +1)
            tw = [_twid16(r[c2], i[c2], c * c2, +1) for c2 in range(4)]
            sto([4 * c + c2 for c2 in range(4)], [t[0] for t in tw], [t[1] for t in tw])
        for c2 in (sub if 2 in ps else ()):
            r, i = _bfly4(*ld([4 * c + c2 for c in range(4)]), +1)
            sto([c2 + 4 * d2 for d2 in range(4)], r, i)

    ctx_s[0:64, :] = jnp.zeros((64, 7 * 128), u32)
    wo_s[...] = jnp.zeros(wo_s.shape, u32)
    for cp in raw_copies(0, 0): cp.wait()
    unpack_weights(0)

    def a_iter(j, carry):
        slot = j % 2
        jn = jnp.minimum(j + 1, NPAIR - 1)
        for cp in raw_copies(jn, 1 - slot): cp.wait()
        wo_copy(j, slot).wait()

        @pl.when(j + 1 < NPAIR)
        def _():
            for cp in raw_copies(jnp.minimum(j + 2, NPAIR - 1), slot): cp.start()
            wo_copy(j + 1, 1 - slot).start()
        Z[0] = pl.multiple_of(jax.lax.shift_right_logical(j, 8) * 8, 8) if OPT['dyn'] else 0
        @pl.when(j == 1)
        def _():
            w_transpose()
        g = jnp.where(j == 0, 16, j - 1)
        st = {}

        def chunks(i):
            km = i * BQ + 128
            cw = OPT["cw"]
            out, k0 = [], 0
            while k0 < km:
                n = min(cw, km - k0)
                out.append((k0, n)); k0 += n
            return out

        def QKc(hh, i, c):
            c0 = hh * D; r0 = i * BQ
            ch = chunks(i)
            if c == 0:
                st["q", hh, i] = _ld(q_s, r0, BQ, c0, D)
            q = st["q", hh, i]
            if c < len(ch):
                k0, n = ch[c]
                sc_ = jax.lax.dot_general(q, _ld(k_s, k0, n, c0, D), NT, preferred_element_type=f32)
                if k0 + n > r0:
                    top = sc_[0:128]
                    td = jnp.where(tri, top[:, n - 128:], -1e30)
                    top = jnp.concatenate([top[:, :n - 128], td], axis=1) if n > 128 else td
                    sc_ = jnp.concatenate([top, sc_[128:256]], axis=0)
                mx = sc_[:, 0:128]
                for t in range(1, n // 128): mx = jnp.maximum(mx, sc_[:, 128 * t:128 * t + 128])
                st["m", hh, i] = mx if c == 0 else jnp.maximum(st["m", hh, i], mx)
            else:
                sc_ = jax.lax.dot_general(q[128:256], _ld(k_s, r0 + 128, 128, c0, D), NT, preferred_element_type=f32)
                sc_ = jnp.where(tri, sc_, -1e30)
                m = st["m", hh, i]
                st["m", hh, i] = jnp.concatenate([m[0:128], jnp.maximum(m[128:256], sc_)], axis=0)
            st["s", hh, i, c] = sc_

        def SMc(hh, i, c):
            ch = chunks(i)
            if c == 0:
                st["mf", hh, i] = jnp.max(st.pop(("m", hh, i)), axis=1, keepdims=True)
            m = st["mf", hh, i]
            sc_ = st.pop(("s", hh, i, c))
            if c < len(ch):
                n = ch[c][1]
                p = jnp.exp2(sc_ - m)
                ls = p[:, 0:128]
                for t in range(1, n // 128): ls = ls + p[:, 128 * t:128 * t + 128]
                st["l", hh, i] = ls if c == 0 else st["l", hh, i] + ls
            else:
                p = jnp.exp2(sc_ - m[128:256])
                l = st["l", hh, i]
                st["l", hh, i] = jnp.concatenate([l[0:128], l[128:256] + p], axis=0)
            st["p", hh, i, c] = p.astype(bf16)

        def PVc(hh, i, c):
            c0 = hh * D; r0 = i * BQ
            ch = chunks(i)
            p = st.pop(("p", hh, i, c))
            if c < len(ch):
                k0, n = ch[c]
                o = jnp.dot(p, _ld(v_s, k0, n, c0, D), preferred_element_type=f32)
                st["o", hh, i] = o if c == 0 else st["o", hh, i] + o
            else:
                ob = jnp.dot(p, _ld(v_s, r0 + 128, 128, c0, D), preferred_element_type=f32)
                o = st.pop(("o", hh, i))
                l = jnp.sum(st.pop(("l", hh, i)), axis=1, keepdims=True)
                r = _recip(l)
                st["ctx", hh, i] = (o[0:128] * r[0:128], (o[128:256] + ob) * r[128:256])
                if hh == 1:
                    store_ctx(i, st.pop(("ctx", 0, i)), st.pop(("ctx", 1, i)))

        def O(i): oproj(i, slot)
        env = dict(KV=kvproj, Q=qproj, WO=lambda: prep_wo(slot), QK=QKc, PV=PVc, SM=SMc, O=O, P2=lambda p, ps=(0, 1, 2), sub=(0, 1, 2, 3): p2_unit(g, p, ps, sub),
                   OP=lambda i: oproj(i, slot), U=lambda: unpack_weights(1 - slot), UKV=lambda: unpack_kv(1 - slot), UQ=lambda: unpack_q(1 - slot))
        for t in SCHED: env[t[0]](*t[1:])
        return carry
    jax.lax.fori_loop(0, NPAIR, a_iter, 0)

    for p in range(5): p2_unit(15, p)
    for i in DEFER: oproj(i, 0)

    mi_copy.wait()
    out_u = out_hbm.bitcast(u32)

    def y_copy(a):
        return pltpu.make_async_copy(ybuf.at[a], out_u.at[:, a, pl.ds(DM, DM)], sem_o.at[0, a])

    def o_copy(a):
        return pltpu.make_async_copy(obuf.at[a], out_hbm.at[pl.ds(a * 16, 16), :, pl.ds(0, DM)], sem_o.at[1, a])

    def p3(a, carry):
        r0 = pl.multiple_of(a * 256, 256)
        obuf[a] = acc[pl.ds(r0, 256), :].astype(bf16).reshape(16, 16, DM)
        o_copy(a).start()
        a_copy(ai_hbm, ai_v, a, 1).wait()
        zs = []
        for h in range(2):
            r = 2 * a + h
            rhs = ubuf[r, :, 0:128, :].reshape(256, 640).astype(bf16)
            Z = jnp.dot(ai_v[r], rhs[:, 0:512], preferred_element_type=f32)
            Zn = jnp.dot(ai_v[r, 0:128, :], rhs[:, 512:640], preferred_element_type=f32)
            zs.append((Z, Zn))
        U = []
        for p in range(4):
            rows = []
            for h in range(2):
                Z, Zn = zs[h]
                zr = Z[0:128, 128 * p:128 * p + 128]
                zi = Z[128:256, 128 * p:128 * p + 128]
                if p == 0:
                    zi = jnp.where(lane == 0, Zn, zi)
                rows.append(jnp.concatenate([zr, zi], axis=1))
            lhs = jnp.concatenate(rows, axis=0).astype(bf16)
            u = jnp.dot(lhs, mi_v[p], preferred_element_type=f32)
            U.append((u[:, 0:128], u[:, 128:256]))
        xs = _inv_butterfly8(U)
        for b in range(8):
            ybuf[a, :, 128 * b:128 * b + 128] = _pack2(xs[b][0:128], xs[b][128:256])
        y_copy(a).start()
        return carry
    jax.lax.fori_loop(0, 8, p3, 0)
    for a in range(8):
        y_copy(a).wait(); o_copy(a).wait()


KVT = [("KV", i) for i in range(8)]


def nchunks(i, cw):
    return -(-(i * BQ + 128) // cw) + 1


def sprinkle(s, pieces, pred, start=0, stop=None):
    stop = len(s) if stop is None else stop
    pos = [k for k in range(start, stop) if pred(s[k])]
    out = list(s)
    ins = {}
    for n, pc in enumerate(pieces):
        k = pos[(n * len(pos)) // len(pieces)]
        ins.setdefault(k, []).append(pc)
    res = []
    for k, t in enumerate(out):
        res += ins.get(k, [])
        res.append(t)
    return res


def fine(defer, cw, small=2, p2="pass", p2where="all"):
    s = list(KVT[:2]) + [("OP", i) for i in defer] + list(KVT[2:])
    s += [("Q", 7)]
    for i in range(7, -1, -1):
        n = nchunks(i, cw)
        s += [("QK", 0, i, c) for c in range(n)]
        qk1 = [("QK", 1, i, c) for c in range(n)]
        s += qk1[:-1] + [("SM", 0, i, 0)] + qk1[-1:]
        if i == 7: s += [("WO",), ("UKV",)]
        if i <= small:
            s += [("Q", i - 1)] if i >= 1 else [("O", 1)]
        sm = [("SM", 0, i, c) for c in range(1, n)] + [("SM", 1, i, c) for c in range(n)]
        pv = [("PV", 0, i, c) for c in range(n)] + [("PV", 1, i, c) for c in range(n)]
        for k, t in enumerate(pv):
            if k < len(sm): s += [sm[k]]
            s += [t]
        if i > small: s += [("Q", i - 1)]
        if i < 7 and i >= 1: s += [("O", i + 1)]
        if i == 1: s += [("UQ",)]
    if 0 not in defer: s += [("O", 0)]
    if p2 == "unit": pcs = [("P2", p) for p in range(5)]
    elif p2 == "pass": pcs = [("P2", p, (q,)) for q in range(3) for p in range(5)]
    elif p2 == "bfly": pcs = [("P2", p, (q,), (b,)) for q in range(3) for p in range(5) for b in range(4)]
    elif p2 == "bfly2": pcs = [("P2", p, (q,), (b, b + 1)) for q in range(3) for p in range(5) for b in (0, 2)]
    if p2where == "all": pred = lambda t: t[0] in ("KV", "Q", "O", "QK", "PV")
    elif p2where == "light": pred = lambda t: t[0] in ("KV", "Q")
    elif p2where == "qk": pred = lambda t: t[0] in ("KV", "Q", "QK")
    elif p2where == "kv": pred = lambda t: t[0] in ("KV",)
    elif p2where == "o": pred = lambda t: t[0] in ("KV", "Q", "O")
    return sprinkle(s, pcs, pred)


SCHEDS = {}
SCHED, DEFER = fine((0,), 512), (0,)


OPT = dict(slab=16, pbuf=False, dyn=False, wunroll=2, cw=512)


_CONSTS = _np_consts()


def make(vmem_mb=110, sched=None, flags=None, **opt):
    global SCHED, DEFER
    OPT.update(opt)
    if sched is None: sched = dict(defer=(), small=0, p2="bfly", p2where="qk")
    if isinstance(sched, dict):
        SCHED, DEFER = fine(sched["defer"], OPT["cw"], small=sched.get("small", 2), p2=sched.get("p2", "pass"), p2where=sched.get("p2where", "all")), sched["defer"]
    else:
        SCHED, DEFER = sched
    M, Mi, A, Ai = _CONSTS
    anyspec = pl.BlockSpec(memory_space=pl.ANY)
    V = pltpu.VMEM
    call = pl.pallas_call(
        _kernel,
        in_specs=[anyspec] * 13, out_specs=anyspec,
        out_shape=jax.ShapeDtypeStruct((128, 16, 2 * DM), bf16),
        scratch_shapes=[
            V((S // 2, DM), u32), V((S // 2, DC), u32), V((5, S // 4, 512), u32), V((5, S // 4, 256), u32),
            V((2, DM, D), u32), V((2, DC, D), u32), V((2, DC, D), u32), V((2, 128, DM), u32),
            V((7, 256, 128), u32), V((7, 128, 256), u32), V((7, 64, 512), u32),
            V((S // 2, 256), u32), V((S // 2, 256), u32), V((S // 2, 256), u32), V((S // 4, 7 * 128), u32), V((S, DM), f32),
            V((8, 128, DM), u32), V((2, 16, 512, 128), bf16), V((2, 1, S), bf16), V((2, S, 640), f32),
            V((16, 2, 136, 640), f32),
            V((4, 256, 256), bf16), V((4, 256, 256), bf16), V((16, 256, 256), bf16), V((16, 256, 256), bf16),
            V((8, 128, DM), u32), V((8, 16, 16, DM), bf16), V((128, S), u32), V((128, S), u32), V((128, S), u32), V((128, S), u32),
            pltpu.SemaphoreType.DMA((8,)), pltpu.SemaphoreType.DMA((4, 2)), pltpu.SemaphoreType.DMA((3, 8)),
            pltpu.SemaphoreType.DMA((2, 17)), pltpu.SemaphoreType.DMA((2, 8)), pltpu.SemaphoreType.DMA((2, 8)),
        ],
        compiler_params=pltpu.CompilerParams(vmem_limit_bytes=vmem_mb * 1024 * 1024, flags=(flags or None)),
    )

    def f(A_x, A_c_kv, A_w_q, A_w_uk, A_w_uv, A_w_o, B_x, B_w_r, B_w_i):
        o = call(A_x.reshape(S, DM), A_c_kv.reshape(S, DC), A_w_q, A_w_uk, A_w_uv, A_w_o.reshape(NPAIR, 256, DM),
                 B_x.reshape(128, 16, DM), B_w_r.T, B_w_i.T, M, Mi, A, Ai)
        return o.reshape(1, S, 2 * DM)
    return f


_CALL = make()


@jax.jit
def pallas_concat_heads__compressed_kv_cla__spectral_gfnet__prompt_kernel(
        A_x, A_c_kv, A_w_q, A_w_uk, A_w_uv, A_w_o, B_x, B_w_r, B_w_i):
    return _CALL(A_x, A_c_kv, A_w_q, A_w_uk, A_w_uv, A_w_o, B_x, B_w_r, B_w_i)
```

```python
import functools
import numpy as np
import ml_dtypes
import jax
import jax.numpy as jnp
from jax.experimental import pallas as pl
from jax.experimental.pallas import tpu as pltpu

f32, bf16, u32 = jnp.float32, jnp.bfloat16, jnp.uint32
S, DM, H, D, DC = 2048, 1024, 32, 128, 512
NT = (((1,), (1,)), ((), ()))
QSCALE = float((D ** -0.5) * 1.4426950408889634)
R2 = float(np.sqrt(0.5))
NPAIR = H // 2


def _lane_freq():
    v = np.zeros((4, 128), np.int64)
    for p in range(4):
        ka, kb = (0, 4) if p == 0 else (p, 8 - p)
        v[p, :64] = ka + 8 * np.arange(64)
        v[p, 64:] = kb + 8 * np.arange(64)
    return v


def _fwd_butterfly8(x):
    a0, a1, a2, a3 = x[0] + x[4], x[1] + x[5], x[2] + x[6], x[3] + x[7]
    c0, c1, c2, c3 = x[0] - x[4], x[1] - x[5], x[2] - x[6], x[3] - x[7]
    s02, s13 = a0 + a2, a1 + a3
    d02, d13 = a0 - a2, a1 - a3
    t1, t2 = (c1 - c3) * R2, (c1 + c3) * R2
    return [(s02, s13), (c0 + t1, c2 + t2), (d02, d13), (c0 - t1, c2 - t2)]


def _inv_butterfly8(u):
    (s02, s13), (b1r, b1i), (d02, d13), (b3r, b3i) = u
    a0, a2 = s02 + d02, s02 - d02
    a1, a3 = s13 + d13, s13 - d13
    c0, t1 = b1r + b3r, b1r - b3r
    c2, t2 = b1i + b3i, b1i - b3i
    c1, c3 = (t1 + t2) * R2, (t2 - t1) * R2
    return [a0 + c0, a1 + c1, a2 + c2, a3 + c3, a0 - c0, a1 - c1, a2 - c2, a3 - c3]


def _d_axis_mats():
    v = _lane_freq()
    d = np.arange(DM)
    eye = np.eye(8)
    F = np.zeros((DM, 4, 2, 128))
    G = np.zeros((4, 2, 128, DM))
    for p in range(4):
        for l in range(128):
            th = 2 * np.pi * ((v[p, l] * d) % DM) / DM
            if v[p, l] == 0:
                ny = np.where(d % 2 == 0, 1.0, -1.0)
                F[:, p, 0, l], F[:, p, 1, l] = 1.0, ny
                G[p, 0, l], G[p, 1, l] = 1.0 / DM, ny / DM
            else:
                F[:, p, 0, l], F[:, p, 1, l] = np.cos(th), -np.sin(th)
                G[p, 0, l], G[p, 1, l] = 2 * np.cos(th) / DM, -2 * np.sin(th) / DM
    F = F.reshape(8, 128, 1024)
    L = np.array([[o for pr in _fwd_butterfly8([eye[i, j] for j in range(8)]) for o in pr] for i in range(8)])
    Mfull = np.einsum('ji,inc->jnc', np.linalg.inv(L), F)
    K = np.array([_inv_butterfly8([(eye[i, 2 * q], eye[i, 2 * q + 1]) for q in range(4)]) for i in range(8)])
    Ufull = np.einsum('sbn,bj->sjn', G.reshape(1024, 8, 128), np.linalg.inv(K))
    M = np.stack([Mfull[2 * p:2 * p + 2, :, 256 * p:256 * p + 256].reshape(256, 256) for p in range(4)])
    Mi = np.stack([Ufull[256 * p:256 * p + 256, 2 * p:2 * p + 2, :].reshape(256, 256) for p in range(4)])
    return M, Mi


def _s_axis_mats():
    A = np.zeros((32, 128, 128))
    Ai = np.zeros((32, 128, 128))
    m = np.arange(64)
    b = np.arange(64)
    for r in range(32):
        th = 2 * np.pi * (np.outer(b, 32 * m + r) % S) / S
        Mr, Mi = np.cos(th), -np.sin(th)
        A[r] = np.block([[Mr, -Mi], [Mi, Mr]])
        Nr, Ni = np.cos(th).T / S, np.sin(th).T / S
        Ai[r] = np.block([[Nr, -Ni], [Ni, Nr]])
    return A, Ai


def _np_consts():
    M, Mi = _d_axis_mats()
    A, Ai = _s_axis_mats()
    c = lambda a: np.asarray(a, np.float32).astype(ml_dtypes.bfloat16)
    return c(M), c(Mi), c(A), c(Ai)


def _bfly4(r, i, sign):
    t0r, t0i = r[0] + r[2], i[0] + i[2]
    t1r, t1i = r[0] - r[2], i[0] - i[2]
    t2r, t2i = r[1] + r[3], i[1] + i[3]
    t3r, t3i = r[1] - r[3], i[1] - i[3]
    if sign < 0:
        o1r, o1i, o3r, o3i = t1r + t3i, t1i - t3r, t1r - t3i, t1i + t3r
    else:
        o1r, o1i, o3r, o3i = t1r - t3i, t1i + t3r, t1r + t3i, t1i - t3r
    return [t0r + t2r, o1r, t0r - t2r, o3r], [t0i + t2i, o1i, t0i - t2i, o3i]


def _twid16(r, i, m, sign):
    if m == 0:
        return r, i
    c = np.cos(2 * np.pi * m / 16)
    s = sign * np.sin(2 * np.pi * m / 16)
    if m == 4:
        return (-i, r) if s > 0 else (i, -r)
    if m in (2, 6):
        cs = 1 if c > 0 else -1
        ss = 1 if s > 0 else -1
        a = (r - i) if cs * ss > 0 else (r + i)
        b = (i + r) if cs * ss > 0 else (i - r)
        return a * (cs * R2), b * (cs * R2)
    c, s = float(c), float(s)
    return r * c - i * s, i * c + r * s


def _twid(r, i, m, n, sign):
    m %= n
    if m == 0:
        return r, i
    if (4 * m) % n == 0:
        q = (4 * m) // n
        if sign < 0: q = (4 - q) % 4
        return [(r, i), (-i, r), (-r, -i), (i, -r)][q]
    c = np.cos(2 * np.pi * m / n)
    s = sign * np.sin(2 * np.pi * m / n)
    if (8 * m) % n == 0:
        cs = 1 if c > 0 else -1
        ss = 1 if s > 0 else -1
        a = (r - i) if cs * ss > 0 else (r + i)
        b = (i + r) if cs * ss > 0 else (i - r)
        return a * (cs * R2), b * (cs * R2)
    c, s = float(c), float(s)
    return r * c - i * s, i * c + r * s


def _bfly8(r, i, sign):
    er, ei = _bfly4(r[0::2], i[0::2], sign)
    orr, oi = _bfly4(r[1::2], i[1::2], sign)
    outr, outi = [None] * 8, [None] * 8
    for k in range(4):
        tr, ti = _twid(orr[k], oi[k], k, 8, sign)
        outr[k], outi[k] = er[k] + tr, ei[k] + ti
        outr[k + 4], outi[k + 4] = er[k] - tr, ei[k] - ti
    return outr, outi


def _dft16(zr, zi, sign):
    def bfly4(r, i):
        t0r, t0i = r[0] + r[2], i[0] + i[2]
        t1r, t1i = r[0] - r[2], i[0] - i[2]
        t2r, t2i = r[1] + r[3], i[1] + i[3]
        t3r, t3i = r[1] - r[3], i[1] - i[3]
        if sign < 0:
            o1r, o1i, o3r, o3i = t1r + t3i, t1i - t3r, t1r - t3i, t1i + t3r
        else:
            o1r, o1i, o3r, o3i = t1r - t3i, t1i + t3r, t1r + t3i, t1i - t3r
        return [t0r + t2r, o1r, t0r - t2r, o3r], [t0i + t2i, o1i, t0i - t2i, o3i]

    def twid(r, i, m):
        if m == 0:
            return r, i
        c = np.cos(2 * np.pi * m / 16)
        s = sign * np.sin(2 * np.pi * m / 16)
        if m == 4:
            return (-i, r) if s > 0 else (i, -r)
        if m in (2, 6):
            cs = 1 if c > 0 else -1
            ss = 1 if s > 0 else -1
            a = (r - i) if cs * ss > 0 else (r + i)
            b = (i + r) if cs * ss > 0 else (i - r)
            return a * (cs * R2), b * (cs * R2)
        c, s = float(c), float(s)
        return r * c - i * s, i * c + r * s

    yr = [[None] * 4 for _ in range(4)]
    yi = [[None] * 4 for _ in range(4)]
    for b in range(4):
        r, i = bfly4([zr[4 * a + b] for a in range(4)], [zi[4 * a + b] for a in range(4)])
        for c in range(4):
            yr[c][b], yi[c][b] = twid(r[c], i[c], b * c)
    outr, outi = [None] * 16, [None] * 16
    for c in range(4):
        r, i = bfly4(yr[c], yi[c])
        for d in range(4):
            outr[c + 4 * d], outi[c + 4 * d] = r[d], i[d]
    return outr, outi


def _lo(u):
    return pltpu.bitcast(u << 16, f32)


def _hi(u):
    return pltpu.bitcast(u & jnp.uint32(0xFFFF0000), f32)


def _recip(l):
    r = pl.reciprocal(l, approx=True)
    return r * (2.0 - l * r)


def _pack2(lo, hi):
    lo_b = pltpu.bitcast(lo.astype(bf16).astype(f32), u32) >> 16
    hi_b = pltpu.bitcast(hi.astype(bf16).astype(f32), u32)
    return lo_b | hi_b


import contextlib


def _mo(x, m):
    return x if isinstance(x, int) else pl.multiple_of(x, m)


def _cut(sc):
    k = OPT["short0"]
    if not k: return sc
    keep = ('W1','W2','W3','W4','PC','PX','UQ0','UKV','UQ','KV', 'Q', 'WO')
    return [t for t in sc if t[0] in keep or (t[0] in ("QK", "SM", "PV") and t[2] >= k) or (t[0] == "O" and t[1] >= k) ]


def _scope(name):
    return jax.named_scope(name) if OPT["scopes"] else contextlib.nullcontext()


OPT = dict(late=2, zpre=True, p2n=3, dmain=False, rot=(7,), cf=0, attn_only=False, p2gate=False, short0=False, ub_rows=136, dmawhen=True, a_static=False, pre_nr=8, bf_ns=32, scopes=False, slab=16, pbuf=False, dyn=False, wunroll=2, cw=512)

BQ = 256
NBLK = S // BQ


def _strassen_lhs(a11, a12, a21, a22):
    return a11 + a22, a21 + a22, a11 + a12, a21 - a11, a12 - a22


def _strassen_rhs(b11, b12, b21, b22):
    return b11 + b22, b11, b12 - b22, b21 - b11, b22, b11 + b12, b21 + b22


def _strassen_mul(L, R):
    m = [jnp.dot(L[t](), R[t](), preferred_element_type=f32) for t in range(7)]
    return m[0] + m[3] - m[4] + m[6], m[2] + m[4], m[1] + m[3], m[0] - m[1] + m[2] + m[5]


def _ld(ref, r0, nr, c0, nc):
    return pltpu.bitcast(ref[r0 // 2:(r0 + nr) // 2, c0:c0 + nc], bf16)


def _st(ref, r0, c0, val):
    nr, nc = val.shape
    ref[r0 // 2:(r0 + nr) // 2, c0:c0 + nc] = pltpu.bitcast(val, u32)


def _kernel(x_hbm, c_hbm, wq_hbm, wk_hbm, wv_hbm, wo_hbm, bx_hbm, wr_hbm, wi_hbm, m_hbm, mi_hbm, a_hbm, ai_hbm,
            out_hbm,
            x_v, c_v, xs, cs, wq_buf, wk_buf, wv_buf, wo_buf, wq_s, wkv_s, wo_s, q_s, k_s, v_s, ctx_s, acc,
            xbuf, lhs_s, wraw, wny, wt, ubuf, m_v, mi_v, a_v, ai_v, ybuf, obuf, pb0, pb1, pb2, pb3,
            sem_x, sem_w, sem_c, sem_wt, sem_o, sem_xc):
    class _Two:
        def __init__(self, cps): self.cps = cps
        def start(self):
            for cp in self.cps: cp.start()
        def wait(self):
            for cp in self.cps: cp.wait()

    def bx_copy(a):
        return _Two([pltpu.make_async_copy(bx_hbm.bitcast(u32).at[:, 2 * a + u, :], xbuf.at[a, pl.ds(64 * u, 64)], sem_x.at[a, u]) for u in range(2)])

    def a_copy(hbm, dst, a, k):
        return pltpu.make_async_copy(hbm.at[pl.ds(4 * a, 4)], dst.at[pl.ds(4 * a, 4)], sem_c.at[k, a])

    m_copy = pltpu.make_async_copy(m_hbm, m_v, sem_c.at[2, 0])
    mi_copy = pltpu.make_async_copy(mi_hbm, mi_v, sem_c.at[2, 1])

    def xa_copy(a):
        return pltpu.make_async_copy(x_hbm.bitcast(u32).at[pl.ds(a * 128, 128)], x_v.at[pl.ds(a * 128, 128)], sem_xc.at[0, a])

    def c_copy(a):
        return pltpu.make_async_copy(c_hbm.bitcast(u32).at[pl.ds(a * 128, 128)], c_v.at[pl.ds(a * 128, 128)], sem_xc.at[1, a])

    def wraw_copies(ri):
        src = (wr_hbm, wi_hbm)[ri]
        cps = [pltpu.make_async_copy(src.at[0:512, pl.ds(128 * a, 128)], wraw.at[ri, a], sem_wt.at[ri, a]) for a in range(16)]
        cps.append(pltpu.make_async_copy(src.at[pl.ds(512, 1), :], wny.at[ri], sem_wt.at[ri, 16]))
        return cps

    def raw_copies(j, slot):
        return (pltpu.make_async_copy(wk_hbm.bitcast(u32).at[:, j, :], wk_buf.at[slot], sem_w.at[1, slot]),
                pltpu.make_async_copy(wv_hbm.bitcast(u32).at[:, j, :], wv_buf.at[slot], sem_w.at[2, slot]),
                pltpu.make_async_copy(wq_hbm.bitcast(u32).at[:, j, :], wq_buf.at[slot], sem_w.at[0, slot]))

    def wo_copy(j, slot):
        return pltpu.make_async_copy(wo_hbm.bitcast(u32).at[j], wo_buf.at[slot], sem_w.at[3, slot])

    rk, rv, rq = raw_copies(0, 0)
    bx_copy(0).start(); m_copy.start()
    for a in range(8):
        if a < 7: bx_copy(a + 1).start()
        a_copy(a_hbm, a_v, a, 0).start()
        if a == 2: rk.start(); rv.start()
        if 3 <= a <= 6: c_copy(2 * (a - 3)).start(); c_copy(2 * (a - 3) + 1).start()
    def mid_starts():
        rq.start()
        for i in range(7, -1, -1): xa_copy(i).start()
        wo_copy(0, 0).start()
        for cp in raw_copies(1, 1): cp.start()

    def late_starts():
        for ri in range(2):
            for cp in wraw_copies(ri): cp.start()
        mi_copy.start()
        for a in range(8): a_copy(ai_hbm, ai_v, a, 1).start()
    if OPT['late'] in (0, 2, 3): mid_starts()
    if OPT['late'] == 0: late_starts()

    lane = jax.lax.broadcasted_iota(jnp.int32, (128, 128), 1)

    def zero_rows(a, carry):
        r0 = pl.multiple_of(a * 256, 256)
        acc[pl.ds(r0, 256), :] = jnp.zeros((256, DM), f32)
        for t in range(4):
            for ri in range(2):
                ubuf[4 * a + t, ri, 0, 64:72, :] = jnp.zeros((8, 128), f32)
                wt[ri, 0, pl.ds(r0 + 64 * t, 8), :] = jnp.zeros((8, 128), f32)
        return carry
    with _scope('zero'):
        if OPT["zpre"]: jax.lax.fori_loop(0, 8, zero_rows, 0)
    with _scope('wait_m'):
        m_copy.wait()

    def _gate(t):
        return pltpu.bitcast(jnp.minimum(jnp.abs(t[0:8, 0:128]), 0.0), u32)

    def _tile(g, nr, nc):
        g = jnp.concatenate([g] * (nc // 128), axis=1)
        return jnp.concatenate([g] * (nr // 8), axis=0)

    def prepass(i, which, g=None, part=None):
        src, dst, w = ((c_v, cs, 256), (x_v, xs, 512))[which]
        nr = OPT["pre_nr"]
        nparts = 64 // nr
        for q in (range(nparts) if part is None else part):
            r = _mo(i * 128 + q * nr, nr)
            h = _mo(i * 64 + q * nr, nr)
            ut, ub = src[pl.ds(r, nr), :], src[pl.ds(r + 64, nr), :]
            if g is not None:
                ut, ub = ut | _tile(g, nr, 2 * w), ub | _tile(g, nr, 2 * w)
            top = pltpu.bitcast(ut, bf16).astype(f32)
            bot = pltpu.bitcast(ub, bf16).astype(f32)
            L = _strassen_lhs(top[:, 0:w], top[:, w:2 * w], bot[:, 0:w], bot[:, w:2 * w])
            for t in range(5): dst[pl.ds(t * (S // 4) + h, nr), :] = pltpu.bitcast(L[t].astype(bf16), u32)

    def bfly_slab(a, h, s0, ns, g=None):
        half = _lo if h == 0 else _hi
        us = [xbuf[a, s0:s0 + ns, 128 * b:128 * b + 128] for b in range(8)]
        if g is not None: us = [u | _tile(g, ns, 128) for u in us]
        xb = [half(u) for u in us]
        Bp = _fwd_butterfly8(xb)
        for p in range(4):
            lhs_s[(4 * h + p) * 64 + s0 // 2:(4 * h + p) * 64 + (s0 + ns) // 2, :] = pltpu.bitcast(jnp.concatenate(Bp[p], axis=1).astype(bf16), u32)

    def bfs(a, h, q, g=None):
        ns = OPT["bf_ns"]
        for t in range(32 // ns): bfly_slab(a, h, 32 * q + t * ns, ns, g)

    def zero_acc(a, q, g=None):
        z = jnp.zeros((32, DM), f32) if g is None else pltpu.bitcast(_tile(g, 32, DM), f32)
        acc[pl.ds(_mo(a * 256 + q * 32, 32), 32), :] = z

    def unpack_kv(slot, parts=range(7)):
        uk, uv = wk_buf[slot], wv_buf[slot]
        def pair(u):
            return jnp.concatenate([_lo(u), _hi(u)], axis=1)
        R = _strassen_rhs(pair(uk[0:256]), pair(uv[0:256]), pair(uk[256:512]), pair(uv[256:512]))
        for t in parts: wkv_s[128 * t:128 * t + 128, :] = pltpu.bitcast(R[t].astype(bf16), u32)

    def unpack_q(slot, parts=range(7)):
        uq = wq_buf[slot]
        R = _strassen_rhs(_lo(uq[0:512]), _hi(uq[0:512]), _lo(uq[512:1024]), _hi(uq[512:1024]))
        for t in parts: wq_s[256 * t:256 * t + 256, :] = pltpu.bitcast(R[t].astype(bf16), u32)

    def unpack_weights(slot):
        unpack_kv(slot); unpack_q(slot)

    def p1(a, carry, last=False):
        with _scope('P1_wait'):
            a_copy(a_hbm, a_v, a, 0).wait()
            if last:
                rk.wait(); rv.wait(); c_copy(0).wait(); c_copy(1).wait()
            an = a + 1
            if not last: bx_copy(an).wait()
        T = {}
        def Ddot(h, p):
            T[h, p] = jnp.dot(pltpu.bitcast(lhs_s[(4 * h + p) * 64:(4 * h + p) * 64 + 64, :], bf16), m_v[p], preferred_element_type=f32)
        def Sdot(h, p):
            tr, ti = T[h, p][:, 0:128], T[h, p][:, 128:256]
            if p == 0:
                T["ny", h] = jnp.where(lane == 0, ti, 0.0)
                ti = jnp.where(lane == 0, 0.0, ti)
            for u in range(2):
                r = 4 * a + 2 * u + h
                rhs = jnp.concatenate([tr[64 * u:64 * u + 64], ti[64 * u:64 * u + 64]], axis=0).astype(bf16)
                U = jnp.dot(a_v[r], rhs, preferred_element_type=f32)
                ubuf[r, 0, p, 0:64, :] = U[0:64]
                ubuf[r, 1, p, 0:64, :] = U[64:128]
        def Sny(h):
            for u in range(2):
                r = 4 * a + 2 * u + h
                rhs = jnp.concatenate([T["ny", h][64 * u:64 * u + 64], jnp.zeros((64, 128), f32)], axis=0).astype(bf16)
                Un = jnp.dot(a_v[r], rhs, preferred_element_type=f32)
                ubuf[r, 0, 4, 0:64, :] = Un[0:64]
                ubuf[r, 1, 4, 0:64, :] = Un[64:128]
        G = lambda k: None if k is None else _gate(T[k])
        env = dict(D=Ddot, S=Sdot, N=Sny, B1=lambda q, k=None: bfly_slab(a, 1, 16 * q, 16, G(k)), B0=lambda q, k=None: bfly_slab(an, 0, 16 * q, 16, G(k)),
                   PC=lambda i, part: prepass(i, 0, None, part), UKV=lambda: unpack_kv(0), Z=lambda q, k=None: zero_acc(a, q, G(k)))
        for t in (P1LAST if last else P1SCHED): env[t[0]](*t[1:])
        return carry
    with _scope('P1'):
      if not OPT['attn_only']:
        with _scope('P1pre'):
            bx_copy(0).wait()
            for q in range(8): bfly_slab(0, 0, 16 * q, 16)
        if OPT['late'] == 1: mid_starts(); late_starts()
        jax.lax.fori_loop(0, 7, p1, 0)
        if OPT['late'] == 2: late_starts()
        p1(7, 0, last=True)

    wu = wraw.bitcast(u32)

    def wpiece(ri, a):
        a0 = 128 * a
        halves = {}
        for c in range(4):
            u = wu[ri, a, pl.ds(c, 64, stride=4), :]
            halves[2 * c], halves[2 * c + 1] = _lo(u), _hi(u)
        for p in range(4):
            ka, kb = (0, 4) if p == 0 else (p, 8 - p)
            t = jnp.concatenate([halves[ka], halves[kb]], axis=0)
            wt[ri, p, a0:a0 + 128, :] = t.T
        ny = wny[ri, :, a0:a0 + 128].astype(f32)
        wt[ri, 4, a0:a0 + 128, :] = jnp.broadcast_to(ny, (128, 128)).T

    row_i = jax.lax.broadcasted_iota(jnp.int32, (128, 128), 0)
    tri = lane <= row_i

    def ldu(ref, *idx):
        return pltpu.bitcast(ref[idx], bf16)

    def kvproj(i):
        t0, b0 = 128 * i, 128 * i + 64
        h0 = 64 * i
        L = [lambda: ldu(cs, slice(0 * (S // 4) + h0, 0 * (S // 4) + h0 + 64), slice(None)), lambda: ldu(cs, slice(1 * (S // 4) + h0, 1 * (S // 4) + h0 + 64), slice(None)),
             lambda: ldu(c_v, slice(t0, t0 + 64), slice(0, 256)), lambda: ldu(c_v, slice(b0, b0 + 64), slice(256, 512)),
             lambda: ldu(cs, slice(2 * (S // 4) + h0, 2 * (S // 4) + h0 + 64), slice(None)), lambda: ldu(cs, slice(3 * (S // 4) + h0, 3 * (S // 4) + h0 + 64), slice(None)),
             lambda: ldu(cs, slice(4 * (S // 4) + h0, 4 * (S // 4) + h0 + 64), slice(None))]
        R = [(lambda t=t: ldu(wkv_s, slice(128 * t, 128 * t + 128), slice(None))) for t in range(7)]
        c11, c12, c21, c22 = _strassen_mul(L, R)
        r0 = 256 * i
        _st(k_s, r0, 0, c11.astype(bf16)); _st(v_s, r0, 0, c12.astype(bf16))
        _st(k_s, r0 + 128, 0, c21.astype(bf16)); _st(v_s, r0 + 128, 0, c22.astype(bf16))

    def qproj(i):
        t0, b0 = 128 * i, 128 * i + 64
        h0 = 64 * i
        L = [lambda: ldu(xs, slice(0 * (S // 4) + h0, 0 * (S // 4) + h0 + 64), slice(None)), lambda: ldu(xs, slice(1 * (S // 4) + h0, 1 * (S // 4) + h0 + 64), slice(None)),
             lambda: ldu(x_v, slice(t0, t0 + 64), slice(0, 512)), lambda: ldu(x_v, slice(b0, b0 + 64), slice(512, 1024)),
             lambda: ldu(xs, slice(2 * (S // 4) + h0, 2 * (S // 4) + h0 + 64), slice(None)), lambda: ldu(xs, slice(3 * (S // 4) + h0, 3 * (S // 4) + h0 + 64), slice(None)),
             lambda: ldu(xs, slice(4 * (S // 4) + h0, 4 * (S // 4) + h0 + 64), slice(None))]
        R = [(lambda t=t: ldu(wq_s, slice(256 * t, 256 * t + 256), slice(None))) for t in range(7)]
        c11, c12, c21, c22 = _strassen_mul(L, R)
        r0 = 256 * i
        _st(q_s, r0, 0, (jnp.concatenate([c11, c12], axis=1) * QSCALE).astype(bf16))
        _st(q_s, r0 + 128, 0, (jnp.concatenate([c21, c22], axis=1) * QSCALE).astype(bf16))

    def qk(hh, i):
        c0 = hh * D
        r0 = i * BQ
        kmain = r0 + 128
        q = _ld(q_s, r0, BQ, c0, D)
        s = jax.lax.dot_general(q, _ld(k_s, 0, kmain, c0, D), NT, preferred_element_type=f32)
        sb = jax.lax.dot_general(q[128:256], _ld(k_s, kmain, 128, c0, D), NT, preferred_element_type=f32)
        top = s[0:128]
        top_d = jnp.where(tri, top[:, r0:kmain], -1e30)
        top = jnp.concatenate([top[:, 0:r0], top_d], axis=1) if r0 else top_d
        bot = jnp.concatenate([s[128:256], jnp.where(tri, sb, -1e30)], axis=1)
        return top, bot

    Z = [0]
    pbufs = [pb0, pb1, pb2, pb3]

    def softmax(hh, i, tb):
        r0 = i * BQ
        kend = r0 + 256
        ls = []
        ps = []
        for half, s in enumerate(tb):
            kk = s.shape[1]
            if OPT["slab"]:
                sl = OPT["slab"]
                lparts, pparts = [], []
                for t in range(0, 128, sl):
                    ss = s[t:t + sl]
                    m = jnp.max(ss, axis=1, keepdims=True)
                    p = jnp.exp2(ss - m)
                    lparts.append(jnp.sum(p, axis=1, keepdims=True))
                    pb = p
                    if OPT["pbuf"]:
                        pb = p.astype(bf16)
                        pbufs[2 * hh + i % 2][(128 * half + t) // 2:(128 * half + t + sl) // 2, 0:kk] = pltpu.bitcast(pb, u32)
                    pparts.append(pb)
                ls.append(jnp.concatenate(lparts, axis=0))
                ps.append(jnp.concatenate(pparts, axis=0))
            else:
                m = jnp.max(s, axis=1, keepdims=True)
                p = jnp.exp2(s - m)
                ls.append(jnp.sum(p, axis=1, keepdims=True))
                pb = p
                if OPT["pbuf"]:
                    pb = p.astype(bf16)
                    pbufs[2 * hh + i % 2][64 * half:64 * half + 64, 0:kk] = pltpu.bitcast(pb, u32)
                ps.append(pb)
        return ps, ls

    def pv(hh, i, pl_):
        ps, ls = pl_
        c0 = hh * D
        r0 = i * BQ
        kmain = r0 + 128
        if OPT["pbuf"]:
            pmain = pltpu.bitcast(pbufs[2 * hh + i % 2][pl.ds(Z[0], 128), 0:kmain], bf16)
            pb = pltpu.bitcast(pbufs[2 * hh + i % 2][pl.ds(Z[0] + 64, 64), kmain:kmain + 128], bf16)
        else:
            pmain = jnp.concatenate([ps[0], ps[1][:, 0:kmain]], axis=0).astype(bf16)
            pb = ps[1][:, kmain:kmain + 128].astype(bf16)
        o = jnp.dot(pmain, _ld(v_s, 0, kmain, c0, D), preferred_element_type=f32)
        ob = jnp.dot(pb, _ld(v_s, kmain, 128, c0, D), preferred_element_type=f32)
        return o[0:128] * _recip(ls[0]), (o[128:256] + ob) * _recip(ls[1])

    def store_ctx(i, c0_, c1_):
        (a11, a21), (a12, a22) = c0_, c1_
        l1, l2, l5, l6, l7 = _strassen_lhs(a11, a12, a21, a22)
        for t, v in enumerate((l1, l2, a11, a22, l5, l6, l7)):
            ctx_s[64 * i:64 * i + 64, 128 * t:128 * t + 128] = pltpu.bitcast(v.astype(bf16), u32)

    def oproj(i, first=False):
        r0 = i * BQ
        L = [(lambda t=t: ldu(ctx_s, slice(64 * i, 64 * i + 64), slice(128 * t, 128 * t + 128))) for t in range(7)]
        R = [(lambda t=t: ldu(wo_s, slice(64 * t, 64 * t + 64), slice(None))) for t in range(7)]
        c11, c12, c21, c22 = _strassen_mul(L, R)
        for rr, cc, v in ((r0, 0, c11), (r0, 512, c12), (r0 + 128, 0, c21), (r0 + 128, 512, c22)):
            if first: acc[rr:rr + 128, cc:cc + 512] = v
            else: acc[rr:rr + 128, cc:cc + 512] += v

    def prep_wo(slot, parts=range(7)):
        w = pltpu.bitcast(wo_buf[slot], bf16).astype(f32)
        R = _strassen_rhs(w[0:128, 0:512], w[0:128, 512:1024], w[128:256, 0:512], w[128:256, 512:1024])
        for t in parts: wo_s[64 * t:64 * t + 64, :] = pltpu.bitcast(R[t].astype(bf16), u32)

    def p2_unit(g, p, ps=(0, 1, 2), sub=None):
        b0 = _mo(g * 8, 8)
        bw = _mo((g % 8) * 8, 8)
        def ld(idx):
            return ([ubuf[r, 0, p, pl.ds(b0, 8), :] for r in idx], [ubuf[r, 1, p, pl.ds(b0, 8), :] for r in idx])
        def sto(idx, vr, vi):
            for r, a_, b_ in zip(idx, vr, vi):
                ubuf[r, 0, p, pl.ds(b0, 8), :] = a_
                ubuf[r, 1, p, pl.ds(b0, 8), :] = b_
        for n2 in ((range(8) if sub is None else sub) if 0 in ps else ()):
            r, i = _bfly4(*ld([8 * n1 + n2 for n1 in range(4)]), -1)
            tw = [_twid(r[k1], i[k1], n2 * k1, 32, -1) for k1 in range(4)]
            sto([8 * k1 + n2 for k1 in range(4)], [t[0] for t in tw], [t[1] for t in tw])
        for k1 in ((range(4) if sub is None else sub) if 1 in ps else ()):
            xr, xi = _bfly8(*ld([8 * k1 + n2 for n2 in range(8)]), -1)
            yr, yi = [], []
            for k2 in range(8):
                a = k1 + 4 * k2
                wr = wt[0, p, pl.ds(64 * a + bw, 8), :]
                wi = wt[1, p, pl.ds(64 * a + bw, 8), :]
                yr.append(xr[k2] * wr - xi[k2] * wi)
                yi.append(xr[k2] * wi + xi[k2] * wr)
            r, i = _bfly8(yr, yi, +1)
            tw = [_twid(r[n2], i[n2], k1 * n2, 32, +1) for n2 in range(8)]
            sto([8 * k1 + n2 for n2 in range(8)], [t[0] for t in tw], [t[1] for t in tw])
        for n2 in ((range(8) if sub is None else sub) if 2 in ps else ()):
            r, i = _bfly4(*ld([8 * k1 + n2 for k1 in range(4)]), +1)
            sto([8 * n1 + n2 for n1 in range(4)], r, i)

    def kv_first(nowo=False):
        allp = tuple(range(64 // OPT["pre_nr"]))
        for i in range(2, 8): c_copy(i).wait()
        if OPT['late'] == 3: late_starts()
        for i in range(8):
            if i < 6: prepass(i + 2, 0, None, allp)
            if i == 2:
                rq.wait(); unpack_q(0)
            if i >= 2:
                xa_copy(9 - i).wait(); prepass(9 - i, 1, None, allp)
            kvproj(i)
        for i in (1, 0):
            xa_copy(i).wait(); prepass(i, 1, None, allp)
        if not nowo: wo_copy(0, 0).wait()

    def kv_second():
        for ri in range(2):
            for cp in wraw_copies(ri): cp.wait()
        rest = [i for i in range(8) if i not in OPT["rot"]]
        pcs = [(t, a) for a in range(16) for t in range(2)]
        n = len(rest)
        for k, i in enumerate(rest):
            mine = pcs[(32 * k) // n:(32 * (k + 1)) // n]
            for t, a in mine[:len(mine) // 2]: wpiece(t, a)
            kvproj(i)
            for t, a in mine[len(mine) // 2:]: wpiece(t, a)

    def kv_plain():
        for i in range(8):
            if i not in OPT["rot"]: kvproj(i)

    def a_iter(j, carry):
        slot = j % 2
        jn = jnp.minimum(j + 1, NPAIR - 1)

        def dma_block():
            for cp in raw_copies(jnp.minimum(j + 2, NPAIR - 1), slot): cp.start()
            wo_copy(jn, 1 - slot).start()

        def wait_block():
            with _scope('A_wait'):
                for cp in raw_copies(jn, 1 - slot): cp.wait()
                wo_copy(j, slot).wait()

        def rare():
            @pl.when(j == 0)
            def _():
                with _scope('KV0'):
                    kv_first()
                for cp in raw_copies(1, 1): cp.wait()
                if not OPT["dmain"]: dma_block()

            @pl.when(j == 1)
            def _():
                wait_block()
                if not OPT["dmain"]: dma_block()
                with _scope('KV1'):
                    kv_second()

        def common():
            wait_block()
            if not OPT["dmain"]: dma_block()
            with _scope('KVn'):
                kv_plain()
        if OPT["cf"] == 2:
            pass
        elif OPT["cf"] == 0:
            jax.lax.cond(j < 2, rare, common)
        else:
            jax.lax.cond(j >= 2, common, rare)
        gp = []
        for k in range(OPT["p2n"]):
            u = OPT["p2n"] * (j - 1) + k
            ok = jnp.logical_and(u >= 0, u < 40)
            gp.append((jnp.where(ok, u % 8, 8), jnp.where(ok, u // 8, 0)))
        zmask = jax.lax.shift_right_logical(j, 8).astype(u32)
        st = {}

        def chunks(i):
            km = i * BQ + 128
            cw = OPT["cw"]
            out, k0 = [], 0
            while k0 < km:
                n = min(cw, km - k0)
                out.append((k0, n)); k0 += n
            return out

        def QKc(hh, i, c):
            c0 = hh * D; r0 = i * BQ
            ch = chunks(i)
            if c == 0:
                st["q", hh, i] = _ld(q_s, r0, BQ, c0, D)
            q = st["q", hh, i]
            if c < len(ch):
                k0, n = ch[c]
                sc_ = jax.lax.dot_general(q, _ld(k_s, k0, n, c0, D), NT, preferred_element_type=f32)
                if k0 + n > r0:
                    top = sc_[0:128]
                    td = jnp.where(tri, top[:, n - 128:], -1e30)
                    top = jnp.concatenate([top[:, :n - 128], td], axis=1) if n > 128 else td
                    sc_ = jnp.concatenate([top, sc_[128:256]], axis=0)
                mx = sc_[:, 0:128]
                for t in range(1, n // 128): mx = jnp.maximum(mx, sc_[:, 128 * t:128 * t + 128])
                st["m", hh, i] = mx if c == 0 else jnp.maximum(st["m", hh, i], mx)
            else:
                sc_ = jax.lax.dot_general(q[128:256], _ld(k_s, r0 + 128, 128, c0, D), NT, preferred_element_type=f32)
                sc_ = jnp.where(tri, sc_, -1e30)
                m = st["m", hh, i]
                st["m", hh, i] = jnp.concatenate([m[0:128], jnp.maximum(m[128:256], sc_)], axis=0)
            st["s", hh, i, c] = sc_

        def SMc(hh, i, c):
            ch = chunks(i)
            if c == 0:
                mm = st.pop(("m", hh, i))
                if OPT["p2gate"]:
                    for gv in st.pop("gates", []):
                        gz = pltpu.bitcast((gv & zmask) | jnp.uint32(0xF149F2CA), f32)
                        mm = jnp.concatenate([jnp.maximum(mm[0:8], gz), mm[8:]], axis=0)
                st["mf", hh, i] = jnp.max(mm, axis=1, keepdims=True)
            m = st["mf", hh, i]
            sc_ = st.pop(("s", hh, i, c))
            if c < len(ch):
                n = ch[c][1]
                p = jnp.exp2(sc_ - m)
                ls = p[:, 0:128]
                for t in range(1, n // 128): ls = ls + p[:, 128 * t:128 * t + 128]
                st["l", hh, i] = ls if c == 0 else st["l", hh, i] + ls
            else:
                p = jnp.exp2(sc_ - m[128:256])
                l = st["l", hh, i]
                st["l", hh, i] = jnp.concatenate([l[0:128], l[128:256] + p], axis=0)
            st["p", hh, i, c] = p.astype(bf16)

        def PVc(hh, i, c):
            c0 = hh * D; r0 = i * BQ
            ch = chunks(i)
            p = st.pop(("p", hh, i, c))
            if c < len(ch):
                k0, n = ch[c]
                o = jnp.dot(p, _ld(v_s, k0, n, c0, D), preferred_element_type=f32)
                st["o", hh, i] = o if c == 0 else st["o", hh, i] + o
            else:
                ob = jnp.dot(p, _ld(v_s, r0 + 128, 128, c0, D), preferred_element_type=f32)
                o = st.pop(("o", hh, i))
                l = jnp.sum(st.pop(("l", hh, i)), axis=1, keepdims=True)
                r = _recip(l)
                st["ctx", hh, i] = (o[0:128] * r[0:128], (o[128:256] + ob) * r[128:256])
                if hh == 1:
                    store_ctx(i, st.pop(("ctx", 0, i)), st.pop(("ctx", 1, i)))

        def O(i): oproj(i)
        def WRAWAIT():
            @pl.when(j == 0)
            def _():
                for ri in range(2):
                    for cp in wraw_copies(ri): cp.wait()
                for a in range(16):
                    for t in range(2): wpiece(t, a)
        env = dict(WAIT=wait_block, DMA=dma_block, WW=WRAWAIT, KV=kvproj, Q=qproj, WO=lambda parts=range(7): prep_wo(slot, parts), QK=QKc, PV=PVc, SM=SMc, O=O, P2=lambda k, ps=(0, 1, 2), sub=None: p2_unit(gp[k][0], gp[k][1], ps, sub),
                   UKV=lambda parts=range(7): unpack_kv(1 - slot, parts), UQ=lambda parts=range(7): unpack_q(1 - slot, parts))
        with _scope('ATT'):
            for t in SCHED: env[t[0]](*t[1:])
        return carry
    with _scope('A'):
        if OPT["cf"] == 2:
            kv_first(nowo=True)
        jax.lax.fori_loop(0, NPAIR, a_iter, 0)

    with _scope('epi'):
        for cp in raw_copies(0, 1): cp.wait()
        wo_copy(0, 0).wait()

    mi_copy.wait()
    out_u = out_hbm.bitcast(u32)

    def y_copy(a):
        return _Two([pltpu.make_async_copy(ybuf.at[a, pl.ds(64 * u, 64)], out_u.at[:, 2 * a + u, pl.ds(DM, DM)], sem_o.at[u, a]) for u in range(2)])

    def o_copy(a):
        return pltpu.make_async_copy(obuf.at[a], out_hbm.at[pl.ds(a * 8, 8), :, pl.ds(0, DM)], sem_o.at[2, a])

    def p3(a, carry):
        r0 = pl.multiple_of(a * 256, 256)
        obuf[a] = acc[pl.ds(r0, 256), :].astype(bf16).reshape(8, 32, DM)
        o_copy(a).start()
        a_copy(ai_hbm, ai_v, a, 1).wait()
        def ldz(r, p):
            return jnp.concatenate([ubuf[r, 0, p, 0:64, :], ubuf[r, 1, p, 0:64, :]], axis=0).astype(bf16)
        U = []
        for p in range(4):
            rows = []
            for h in range(2):
                for u in range(2):
                    r = 4 * a + 2 * u + h
                    Z = jnp.dot(ai_v[r], ldz(r, p), preferred_element_type=f32)
                    zr, zi = Z[0:64], Z[64:128]
                    if p == 0:
                        Zn = jnp.dot(ai_v[r, 0:64, :], ldz(r, 4), preferred_element_type=f32)
                        zi = jnp.where(lane[0:64] == 0, Zn, zi)
                    rows.append(jnp.concatenate([zr, zi], axis=1))
            lhs = jnp.concatenate(rows, axis=0).astype(bf16)
            u = jnp.dot(lhs, mi_v[p], preferred_element_type=f32)
            U.append((u[:, 0:128], u[:, 128:256]))
        xs = _inv_butterfly8(U)
        for b in range(8):
            ybuf[a, :, 128 * b:128 * b + 128] = _pack2(xs[b][0:128], xs[b][128:256])
        y_copy(a).start()
        return carry
    with _scope('P3'):
        if not OPT['attn_only']: jax.lax.fori_loop(0, 8, p3, 0)
    with _scope('out_wait'):
        for a in range(8 if not OPT['attn_only'] else 0):
            y_copy(a).wait(); o_copy(a).wait()


KVT = [("KV", i) for i in range(8)]


def nchunks(i, cw):
    return -(-(i * BQ + 128) // cw) + 1


def sprinkle(s, pieces, pred, start=0, stop=None):
    stop = len(s) if stop is None else stop
    pos = [k for k in range(start, stop) if pred(s[k])]
    out = list(s)
    ins = {}
    for n, pc in enumerate(pieces):
        k = pos[(n * len(pos)) // len(pieces)]
        ins.setdefault(k, []).append(pc)
    res = []
    for k, t in enumerate(out):
        res += ins.get(k, [])
        res.append(t)
    return res


def fine(defer, cw, small=2, p2="pass", p2where="all"):
    s = list(KVT[:2]) + [("OP", i) for i in defer] + list(KVT[2:])
    s += [("Q", 7)]
    for i in range(7, -1, -1):
        n = nchunks(i, cw)
        s += [("QK", 0, i, c) for c in range(n)]
        qk1 = [("QK", 1, i, c) for c in range(n)]
        s += qk1[:-1] + [("SM", 0, i, 0)] + qk1[-1:]
        if i == 7: s += [("WO",), ("UKV",)]
        if i <= small:
            s += [("Q", i - 1)] if i >= 1 else [("O", 1)]
        sm = [("SM", 0, i, c) for c in range(1, n)] + [("SM", 1, i, c) for c in range(n)]
        pv = [("PV", 0, i, c) for c in range(n)] + [("PV", 1, i, c) for c in range(n)]
        for k, t in enumerate(pv):
            if k < len(sm): s += [sm[k]]
            s += [t]
        if i > small: s += [("Q", i - 1)]
        if i < 7 and i >= 1: s += [("O", i + 1)]
        if i == 1: s += [("UQ",)]
    if 0 not in defer: s += [("O", 0)]
    if p2 == "unit": pcs = [("P2", p) for p in range(5)]
    elif p2 == "pass": pcs = [("P2", p, (q,)) for q in range(3) for p in range(5)]
    elif p2 == "bfly": pcs = [("P2", p, (q,), (b,)) for q in range(3) for p in range(OPT["p2n"]) for b in range(4 if q == 1 else 8)]
    elif p2 == "bfly2": pcs = [("P2", p, (q,), (b, b + 1)) for q in range(3) for p in range(5) for b in (0, 2)]
    if p2where == "all": pred = lambda t: t[0] in ("Q", "O", "QK", "PV")
    elif p2where == "light": pred = lambda t: t[0] in ("KV", "Q")
    elif p2where == "qk": pred = lambda t: t[0] in ("Q", "QK")
    elif p2where == "kv": pred = lambda t: t[0] in ("KV",)
    elif p2where == "o": pred = lambda t: t[0] in ("KV", "Q", "O")
    return sprinkle(s, pcs, pred)


P1MX = [("D", 0, 0), ("D", 0, 1), ("D", 0, 2), ("D", 0, 3), ("D", 1, 0), ("D", 1, 1), ("D", 1, 2), ("D", 1, 3),
        ("S", 0, 0), ("S", 0, 1), ("S", 0, 2), ("S", 0, 3), ("N", 0), ("S", 1, 0), ("S", 1, 1), ("S", 1, 2), ("S", 1, 3), ("N", 1)]


def _p1sched(extra):
    out = [("B1", 0), ("B1", 1), ("B1", 2)]
    b1 = [("B1", q) for q in range(3, 8)]
    for k, m in enumerate(P1MX):
        if k in (1, 2): out += b1[2 * (k - 1):2 * k]
        if k == 3: out += b1[4:]
        if k >= 8 and k - 8 < len(extra): out += extra[k - 8]
        out.append(m)
    return out


P1SCHED = _p1sched([[("B0", q)] for q in range(8)])
P1LAST = _p1sched([[("UKV",)], [("PC", 0, (0, 1))], [("PC", 0, (2, 3))], [("PC", 0, (4, 5))], [("PC", 0, (6, 7))],
                   [("PC", 1, (0, 1, 2))], [("PC", 1, (3, 4, 5))], [("PC", 1, (6, 7))]])
def first_sched(cw):
    base = [t for t in fine((), cw, small=0, p2="pass", p2where="qk") if t[0] not in ("P2", "UKV", "UQ")]
    s = []
    for t in base:
        if t == ("KV", 0): s += [("W1",)]
        if t[0] == "KV" and t[1] < 6: s += [("PC", t[1] + 2, tuple(range(8)))]
        if t == ("KV", 4): s += [("W2",), ("UQ0",)]
        if t == ("KV", 6): s += [("PX", 7, tuple(range(8)))]
        if t == ("KV", 7): s += [("PX", 6, tuple(range(8)))]
        if t == ("Q", 7): s += [("W3",)]
        if t == ("QK", 0, 7, 0): s += [("PX", 5, tuple(range(8)))]
        if t == ("QK", 1, 7, 0): s += [("PX", 4, tuple(range(8)))]
        if t == ("QK", 0, 6, 0): s += [("PX", 3, tuple(range(8)))]
        if t == ("QK", 1, 6, 0): s += [("PX", 2, tuple(range(8)))]
        if t == ("QK", 0, 5, 0): s += [("PX", 1, tuple(range(8)))]
        if t == ("QK", 1, 5, 0): s += [("PX", 0, tuple(range(8)))]
        if t == ("QK", 0, 4, 0): s += [("W4",), ("UKV",)]
        s.append(t)
    k0 = s.index(("W4",))
    s = sprinkle(s, [("WP", ri, a) for a in range(16) for ri in range(2)], lambda t: t[0] in ("Q", "O", "QK", "PV"), start=k0)
    s.insert(s.index(("Q", 0)) + 1, ("UQ",))
    return s


SCHEDS = {}
SCHED, DEFER = [t for t in fine((), 512, small=0, p2='bfly', p2where='qk') if t[0] != 'KV'], ()


_CONSTS = _np_consts()


def make(vmem_mb=110, sched=None, flags=None, p1sched=None, **opt):
    global SCHED, DEFER
    OPT.update(opt)
    global P1SCHED
    if p1sched is not None: P1SCHED = p1sched
    if sched is None: sched = dict(defer=(), small=0, p2="bfly", p2where="qk", ins=[(("KV", 7), ("O", 0), 0)])
    if isinstance(sched, dict):
        SCHED, DEFER = [t for t in fine(sched["defer"], OPT["cw"], small=sched.get("small", 2), p2=sched.get("p2", "pass"), p2where=sched.get("p2where", "all")) if t[0] != "KV"], sched["defer"]
        for t, anchor, off in sched.get("ins", ()):
            SCHED.insert(SCHED.index(anchor) + off, t)
    else:
        SCHED, DEFER = list(sched), ()
    M, Mi, A, Ai = _CONSTS
    anyspec = pl.BlockSpec(memory_space=pl.ANY)
    V = pltpu.VMEM
    call = pl.pallas_call(
        _kernel,
        in_specs=[anyspec] * 13, out_specs=anyspec,
        out_shape=jax.ShapeDtypeStruct((64, 32, 2 * DM), bf16),
        scratch_shapes=[
            V((S // 2, DM), u32), V((S // 2, DC), u32), V((5 * S // 4, 512), u32), V((5 * S // 4, 256), u32),
            V((2, DM, D), u32), V((2, DC, D), u32), V((2, DC, D), u32), V((2, 128, DM), u32),
            V((7 * 256, 128), u32), V((7 * 128, 256), u32), V((7 * 64, 512), u32),
            V((S // 2, 256), u32), V((S // 2, 256), u32), V((S // 2, 256), u32), V((S // 4, 7 * 128), u32), V((S, DM), f32),
            V((8, 128, DM), u32), V((8 * 64, 256), u32), V((2, 16, 512, 128), bf16), V((2, 1, S), bf16), V((2, 5, S, 128), f32),
            V((32, 2, 5, 72, 128), f32),
            V((4, 256, 256), bf16), V((4, 256, 256), bf16), V((32, 128, 128), bf16), V((32, 128, 128), bf16),
            V((8, 128, DM), u32), V((8, 8, 32, DM), bf16), V((128, S), u32), V((128, S), u32), V((128, S), u32), V((128, S), u32),
            pltpu.SemaphoreType.DMA((8, 2)), pltpu.SemaphoreType.DMA((4, 2)), pltpu.SemaphoreType.DMA((3, 8)),
            pltpu.SemaphoreType.DMA((2, 17)), pltpu.SemaphoreType.DMA((3, 8)), pltpu.SemaphoreType.DMA((2, 8)),
        ],
        compiler_params=pltpu.CompilerParams(vmem_limit_bytes=vmem_mb * 1024 * 1024, flags=(flags or None)),
    )

    def f(A_x, A_c_kv, A_w_q, A_w_uk, A_w_uv, A_w_o, B_x, B_w_r, B_w_i):
        o = call(A_x.reshape(S, DM), A_c_kv.reshape(S, DC), A_w_q, A_w_uk, A_w_uv, A_w_o.reshape(NPAIR, 256, DM),
                 B_x.reshape(64, 32, DM), B_w_r.T, B_w_i.T, M, Mi, A, Ai)
        return o.reshape(1, S, 2 * DM)
    return f


_CALL = make()


@jax.jit
def pallas_concat_heads__compressed_kv_cla__spectral_gfnet__prompt_kernel(
        A_x, A_c_kv, A_w_q, A_w_uk, A_w_uv, A_w_o, B_x, B_w_r, B_w_i):
    return _CALL(A_x, A_c_kv, A_w_q, A_w_uk, A_w_uv, A_w_o, B_x, B_w_r, B_w_i)
```

```python
import functools
import numpy as np
import ml_dtypes
import jax
import jax.numpy as jnp
from jax.experimental import pallas as pl
from jax.experimental.pallas import tpu as pltpu

f32, bf16, u32 = jnp.float32, jnp.bfloat16, jnp.uint32
S, DM, H, D, DC = 2048, 1024, 32, 128, 512
NT = (((1,), (1,)), ((), ()))
QSCALE = float((D ** -0.5) * 1.4426950408889634)
R2 = float(np.sqrt(0.5))
NPAIR = H // 2


def _lane_freq():
    v = np.zeros((4, 128), np.int64)
    for p in range(4):
        ka, kb = (0, 4) if p == 0 else (p, 8 - p)
        v[p, :64] = ka + 8 * np.arange(64)
        v[p, 64:] = kb + 8 * np.arange(64)
    return v


def _fwd_butterfly8(x):
    a0, a1, a2, a3 = x[0] + x[4], x[1] + x[5], x[2] + x[6], x[3] + x[7]
    c0, c1, c2, c3 = x[0] - x[4], x[1] - x[5], x[2] - x[6], x[3] - x[7]
    s02, s13 = a0 + a2, a1 + a3
    d02, d13 = a0 - a2, a1 - a3
    t1, t2 = (c1 - c3) * R2, (c1 + c3) * R2
    return [(s02, s13), (c0 + t1, c2 + t2), (d02, d13), (c0 - t1, c2 - t2)]


def _inv_butterfly8(u):
    (s02, s13), (b1r, b1i), (d02, d13), (b3r, b3i) = u
    a0, a2 = s02 + d02, s02 - d02
    a1, a3 = s13 + d13, s13 - d13
    c0, t1 = b1r + b3r, b1r - b3r
    c2, t2 = b1i + b3i, b1i - b3i
    c1, c3 = (t1 + t2) * R2, (t2 - t1) * R2
    return [a0 + c0, a1 + c1, a2 + c2, a3 + c3, a0 - c0, a1 - c1, a2 - c2, a3 - c3]


def _d_axis_mats():
    v = _lane_freq()
    d = np.arange(DM)
    eye = np.eye(8)
    F = np.zeros((DM, 4, 2, 128))
    G = np.zeros((4, 2, 128, DM))
    for p in range(4):
        for l in range(128):
            th = 2 * np.pi * ((v[p, l] * d) % DM) / DM
            if v[p, l] == 0:
                ny = np.where(d % 2 == 0, 1.0, -1.0)
                F[:, p, 0, l], F[:, p, 1, l] = 1.0, ny
                G[p, 0, l], G[p, 1, l] = 1.0 / DM, ny / DM
            else:
                F[:, p, 0, l], F[:, p, 1, l] = np.cos(th), -np.sin(th)
                G[p, 0, l], G[p, 1, l] = 2 * np.cos(th) / DM, -2 * np.sin(th) / DM
    F = F.reshape(8, 128, 1024)
    L = np.array([[o for pr in _fwd_butterfly8([eye[i, j] for j in range(8)]) for o in pr] for i in range(8)])
    Mfull = np.einsum('ji,inc->jnc', np.linalg.inv(L), F)
    K = np.array([_inv_butterfly8([(eye[i, 2 * q], eye[i, 2 * q + 1]) for q in range(4)]) for i in range(8)])
    Ufull = np.einsum('sbn,bj->sjn', G.reshape(1024, 8, 128), np.linalg.inv(K))
    M = np.stack([Mfull[2 * p:2 * p + 2, :, 256 * p:256 * p + 256].reshape(256, 256) for p in range(4)])
    Mi = np.stack([Ufull[256 * p:256 * p + 256, 2 * p:2 * p + 2, :].reshape(256, 256) for p in range(4)])
    return M, Mi


def _s_axis_mats():
    A = np.zeros((32, 128, 128))
    Ai = np.zeros((32, 128, 128))
    m = np.arange(64)
    b = np.arange(64)
    for r in range(32):
        th = 2 * np.pi * (np.outer(b, 32 * m + r) % S) / S
        Mr, Mi = np.cos(th), -np.sin(th)
        A[r] = np.block([[Mr, -Mi], [Mi, Mr]])
        Nr, Ni = np.cos(th).T / S, np.sin(th).T / S
        Ai[r] = np.block([[Nr, -Ni], [Ni, Nr]])
    return A, Ai


def _np_consts():
    M, Mi = _d_axis_mats()
    A, Ai = _s_axis_mats()
    c = lambda a: np.asarray(a, np.float32).astype(ml_dtypes.bfloat16)
    return c(M), c(Mi), c(A), c(Ai)


def _bfly4(r, i, sign):
    t0r, t0i = r[0] + r[2], i[0] + i[2]
    t1r, t1i = r[0] - r[2], i[0] - i[2]
    t2r, t2i = r[1] + r[3], i[1] + i[3]
    t3r, t3i = r[1] - r[3], i[1] - i[3]
    if sign < 0:
        o1r, o1i, o3r, o3i = t1r + t3i, t1i - t3r, t1r - t3i, t1i + t3r
    else:
        o1r, o1i, o3r, o3i = t1r - t3i, t1i + t3r, t1r + t3i, t1i - t3r
    return [t0r + t2r, o1r, t0r - t2r, o3r], [t0i + t2i, o1i, t0i - t2i, o3i]


def _twid16(r, i, m, sign):
    if m == 0:
        return r, i
    c = np.cos(2 * np.pi * m / 16)
    s = sign * np.sin(2 * np.pi * m / 16)
    if m == 4:
        return (-i, r) if s > 0 else (i, -r)
    if m in (2, 6):
        cs = 1 if c > 0 else -1
        ss = 1 if s > 0 else -1
        a = (r - i) if cs * ss > 0 else (r + i)
        b = (i + r) if cs * ss > 0 else (i - r)
        return a * (cs * R2), b * (cs * R2)
    c, s = float(c), float(s)
    return r * c - i * s, i * c + r * s


def _twid(r, i, m, n, sign):
    m %= n
    if m == 0:
        return r, i
    if (4 * m) % n == 0:
        q = (4 * m) // n
        if sign < 0: q = (4 - q) % 4
        return [(r, i), (-i, r), (-r, -i), (i, -r)][q]
    c = np.cos(2 * np.pi * m / n)
    s = sign * np.sin(2 * np.pi * m / n)
    if (8 * m) % n == 0:
        cs = 1 if c > 0 else -1
        ss = 1 if s > 0 else -1
        a = (r - i) if cs * ss > 0 else (r + i)
        b = (i + r) if cs * ss > 0 else (i - r)
        return a * (cs * R2), b * (cs * R2)
    c, s = float(c), float(s)
    return r * c - i * s, i * c + r * s


def _bfly8(r, i, sign):
    er, ei = _bfly4(r[0::2], i[0::2], sign)
    orr, oi = _bfly4(r[1::2], i[1::2], sign)
    outr, outi = [None] * 8, [None] * 8
    for k in range(4):
        tr, ti = _twid(orr[k], oi[k], k, 8, sign)
        outr[k], outi[k] = er[k] + tr, ei[k] + ti
        outr[k + 4], outi[k + 4] = er[k] - tr, ei[k] - ti
    return outr, outi


def _dft16(zr, zi, sign):
    def bfly4(r, i):
        t0r, t0i = r[0] + r[2], i[0] + i[2]
        t1r, t1i = r[0] - r[2], i[0] - i[2]
        t2r, t2i = r[1] + r[3], i[1] + i[3]
        t3r, t3i = r[1] - r[3], i[1] - i[3]
        if sign < 0:
            o1r, o1i, o3r, o3i = t1r + t3i, t1i - t3r, t1r - t3i, t1i + t3r
        else:
            o1r, o1i, o3r, o3i = t1r - t3i, t1i + t3r, t1r + t3i, t1i - t3r
        return [t0r + t2r, o1r, t0r - t2r, o3r], [t0i + t2i, o1i, t0i - t2i, o3i]

    def twid(r, i, m):
        if m == 0:
            return r, i
        c = np.cos(2 * np.pi * m / 16)
        s = sign * np.sin(2 * np.pi * m / 16)
        if m == 4:
            return (-i, r) if s > 0 else (i, -r)
        if m in (2, 6):
            cs = 1 if c > 0 else -1
            ss = 1 if s > 0 else -1
            a = (r - i) if cs * ss > 0 else (r + i)
            b = (i + r) if cs * ss > 0 else (i - r)
            return a * (cs * R2), b * (cs * R2)
        c, s = float(c), float(s)
        return r * c - i * s, i * c + r * s

    yr = [[None] * 4 for _ in range(4)]
    yi = [[None] * 4 for _ in range(4)]
    for b in range(4):
        r, i = bfly4([zr[4 * a + b] for a in range(4)], [zi[4 * a + b] for a in range(4)])
        for c in range(4):
            yr[c][b], yi[c][b] = twid(r[c], i[c], b * c)
    outr, outi = [None] * 16, [None] * 16
    for c in range(4):
        r, i = bfly4(yr[c], yi[c])
        for d in range(4):
            outr[c + 4 * d], outi[c + 4 * d] = r[d], i[d]
    return outr, outi


def _lo(u):
    return pltpu.bitcast(u << 16, f32)


def _hi(u):
    return pltpu.bitcast(u & jnp.uint32(0xFFFF0000), f32)


def _recip(l):
    r = pl.reciprocal(l, approx=True)
    return r * (2.0 - l * r)


def _pack2(lo, hi):
    lo_b = pltpu.bitcast(lo.astype(bf16).astype(f32), u32) >> 16
    hi_b = pltpu.bitcast(hi.astype(bf16).astype(f32), u32)
    return lo_b | hi_b


import contextlib


def _mo(x, m):
    return x if isinstance(x, int) else pl.multiple_of(x, m)


def _cut(sc):
    k = OPT["short0"]
    if not k: return sc
    keep = ('W1','W2','W3','W4','PC','PX','UQ0','UKV','UQ','KV', 'Q', 'WO')
    return [t for t in sc if t[0] in keep or (t[0] in ("QK", "SM", "PV") and t[2] >= k) or (t[0] == "O" and t[1] >= k) ]


def _scope(name):
    return jax.named_scope(name) if OPT["scopes"] else contextlib.nullcontext()


OPT = dict(opan=(64, 128), qrows=128, kf='K0 R W7 W6 W5 W4 X7 K1 X6 K2 X5 K3 X4 K4 W3 W2 W1 W0 X3 K5 X2 K6 X1 K7 X0', wo='acb', wwhen=False, uk1=False, p1o=(('S',),('B',0),('B',1),('P',),('D',)), p3s=(('C',), ('D', 0), ('D', 1), ('D', 2), ('D', 3), ('X', 0), ('X', 1), ('X', 2), ('X', 3), ('B',), ('OS',)), smlag=0, smslab=0, late=2, zpre=True, p2n=3, dmain=False, rot=(7,), cf=0, attn_only=False, p2gate=False, short0=False, ub_rows=136, dmawhen=True, a_static=False, pre_nr=8, bf_ns=16, scopes=False, slab=16, pbuf=False, dyn=False, wunroll=2, cw=512)

BQ = 256
NBLK = S // BQ


def _strassen_lhs(a11, a12, a21, a22):
    return a11 + a22, a21 + a22, a11 + a12, a21 - a11, a12 - a22


def _strassen_rhs(b11, b12, b21, b22):
    return b11 + b22, b11, b12 - b22, b21 - b11, b22, b11 + b12, b21 + b22


def _strassen_lhs7(a11, a12, a21, a22):
    l1, l2, l5, l6, l7 = _strassen_lhs(a11, a12, a21, a22)
    return l1, l2, a11, a22, l5, l6, l7


def _quad(a):
    r, c = a.shape[0] // 2, a.shape[1] // 2
    return a[:r, :c], a[:r, c:], a[r:, :c], a[r:, c:]


def _strassen_mul(L, R):
    return _strassen_out([jnp.dot(L[t](), R[t](), preferred_element_type=f32) for t in range(7)])


def _strassen_out(m):
    return m[0] + m[3] - m[4] + m[6], m[2] + m[4], m[1] + m[3], m[0] - m[1] + m[2] + m[5]


def _ld(ref, r0, nr, c0, nc):
    return pltpu.bitcast(ref[r0 // 2:(r0 + nr) // 2, c0:c0 + nc], bf16)


def _st(ref, r0, c0, val):
    nr, nc = val.shape
    ref[r0 // 2:(r0 + nr) // 2, c0:c0 + nc] = pltpu.bitcast(val, u32)


def _kernel(x_hbm, c_hbm, wq_hbm, wk_hbm, wv_hbm, wo_hbm, bx_hbm, wr_hbm, wi_hbm, m_hbm, mi_hbm, a_hbm, ai_hbm,
            out_hbm,
            x_v, c_v, xs, wq_buf, wk_buf, wv_buf, wo_buf, wq_s, wkv_s, wo_s, q_s, k_s, v_s, ctx_s, acc,
            xbuf, lhs_s, rs, wraw, wny, wt, ubuf, m_v, mi_v, a_v, ai_v, ybuf, obuf, cs, pb0, pb1, pb2, pb3,
            sem_x, sem_w, sem_c, sem_wt, sem_o, sem_xc):
    class _Two:
        def __init__(self, cps): self.cps = cps
        def start(self):
            for cp in self.cps: cp.start()
        def wait(self):
            for cp in self.cps: cp.wait()

    def bx_copy(a):
        return _Two([pltpu.make_async_copy(bx_hbm.bitcast(u32).at[:, 2 * a + u, :], xbuf.at[a, pl.ds(64 * u, 64)], sem_x.at[a, u]) for u in range(2)])

    def a_copy(hbm, dst, a, k):
        return pltpu.make_async_copy(hbm.at[pl.ds(4 * a, 4)], dst.at[pl.ds(4 * a, 4)], sem_c.at[k, a])

    m_copy = pltpu.make_async_copy(m_hbm, m_v, sem_c.at[2, 0])
    mi_copy = pltpu.make_async_copy(mi_hbm, mi_v, sem_c.at[2, 1])

    def xa_copy(a):
        return pltpu.make_async_copy(x_hbm.bitcast(u32).at[pl.ds(a * 128, 128)], x_v.at[pl.ds(a * 128, 128)], sem_xc.at[0, a])

    def c_copy(a):
        return pltpu.make_async_copy(c_hbm.bitcast(u32).at[pl.ds(a * 128, 128)], c_v.at[pl.ds(a * 128, 128)], sem_xc.at[1, a])

    def wraw_copies(ri):
        src = (wr_hbm, wi_hbm)[ri]
        cps = [pltpu.make_async_copy(src.at[0:512, pl.ds(128 * a, 128)], wraw.at[ri, a], sem_wt.at[ri, a]) for a in range(16)]
        cps.append(pltpu.make_async_copy(src.at[pl.ds(512, 1), :], wny.at[ri], sem_wt.at[ri, 16]))
        return cps

    def raw_copies(j, slot):
        return (pltpu.make_async_copy(wk_hbm.bitcast(u32).at[:, j, :], wk_buf.at[slot], sem_w.at[1, slot]),
                pltpu.make_async_copy(wv_hbm.bitcast(u32).at[:, j, :], wv_buf.at[slot], sem_w.at[2, slot]),
                pltpu.make_async_copy(wq_hbm.bitcast(u32).at[:, j, :], wq_buf.at[slot], sem_w.at[0, slot]))

    def wo_copy(j, slot):
        return pltpu.make_async_copy(wo_hbm.bitcast(u32).at[j], wo_buf.at[slot], sem_w.at[3, slot])

    rk, rv, rq = raw_copies(0, 0)
    for a in range(8):
        bx_copy(a).start()
        if a == 0: m_copy.start()
        a_copy(a_hbm, a_v, a, 0).start()
        c_copy(a).start()
        if a == 5: rk.start(); rv.start()
    def mid_starts():
        rq.start()
        for i in range(7, -1, -1): xa_copy(i).start()
        wo_copy(0, 0).start()
        for cp in raw_copies(1, 1): cp.start()

    def late_starts():
        for ri in range(2):
            for cp in wraw_copies(ri): cp.start()
        mi_copy.start()
        for a in range(8): a_copy(ai_hbm, ai_v, a, 1).start()
    if OPT['late'] in (0, 2, 3): mid_starts()
    if OPT['late'] == 0: late_starts()

    lane = jax.lax.broadcasted_iota(jnp.int32, (128, 128), 1)

    def zero_rows(a, carry):
        r0 = pl.multiple_of(a * 256, 256)
        acc[pl.ds(r0, 256), :] = jnp.zeros((256, DM), f32)
        for t in range(4):
            for ri in range(2):
                ubuf[4 * a + t, ri, 0, 64:72, :] = jnp.zeros((8, 128), f32)
                wt[ri, 0, pl.ds(r0 + 64 * t, 8), :] = jnp.zeros((8, 128), f32)
        return carry
    with _scope('zero'):
        if OPT["zpre"]: jax.lax.fori_loop(0, 8, zero_rows, 0)
    with _scope('wait_m'):
        m_copy.wait()

    def _gate(t):
        return pltpu.bitcast(jnp.minimum(jnp.abs(t[0:8, 0:128]), 0.0), u32)

    def _tile(g, nr, nc):
        g = jnp.concatenate([g] * (nc // 128), axis=1)
        return jnp.concatenate([g] * (nr // 8), axis=0)

    def prepass_c(i, part=None, g=None):
        nr = 8
        for q in (range(4) if part is None else part):
            rows = [c_v[pl.ds(_mo(i * 128 + 32 * k + q * nr, nr), nr), :] for k in range(4)]
            if g is not None: rows = [u | _tile(g, nr, 512) for u in rows]
            rows = [pltpu.bitcast(u, bf16).astype(f32) for u in rows]
            top = jnp.concatenate(rows[0:2], axis=0)
            bot = jnp.concatenate(rows[2:4], axis=0)
            L1 = _strassen_lhs7(top[:, 0:256], top[:, 256:512], bot[:, 0:256], bot[:, 256:512])
            for t in range(7):
                L2 = _strassen_lhs7(*_quad(L1[t]))
                cs[pl.ds(_mo(t * 256 + 32 * i + q * nr, nr), nr), :] = pltpu.bitcast(jnp.concatenate(L2, axis=1).astype(bf16), u32)

    def prepass(i, which, g=None, part=None):
        if which == 0:
            return prepass_c(i, None if part is None else tuple(sorted(set(q // 2 for q in part))))
        src, dst, w = ((c_v, cs, 256), (x_v, xs, 512))[which]
        nr = OPT["pre_nr"]
        nparts = 64 // nr
        for q in (range(nparts) if part is None else part):
            r = _mo(i * 128 + q * nr, nr)
            h = _mo(i * 64 + q * nr, nr)
            ut, ub = src[pl.ds(r, nr), :], src[pl.ds(r + 64, nr), :]
            if g is not None:
                ut, ub = ut | _tile(g, nr, 2 * w), ub | _tile(g, nr, 2 * w)
            top = pltpu.bitcast(ut, bf16).astype(f32)
            bot = pltpu.bitcast(ub, bf16).astype(f32)
            L = _strassen_lhs(top[:, 0:w], top[:, w:2 * w], bot[:, 0:w], bot[:, w:2 * w])
            for t in range(5): dst[pl.ds(t * (S // 4) + h, nr), :] = pltpu.bitcast(L[t].astype(bf16), u32)

    def bfly_slab(a, h, s0, ns, g=None):
        half = _lo if h == 0 else _hi
        us = [xbuf[a, s0:s0 + ns, 128 * b:128 * b + 128] for b in range(8)]
        if g is not None: us = [u | _tile(g, ns, 128) for u in us]
        xb = [half(u) for u in us]
        Bp = _fwd_butterfly8(xb)
        for p in range(4):
            lhs_s[(4 * h + p) * 64 + s0 // 2:(4 * h + p) * 64 + (s0 + ns) // 2, :] = pltpu.bitcast(jnp.concatenate(Bp[p], axis=1).astype(bf16), u32)

    def bfs(a, h, q, g=None):
        ns = OPT["bf_ns"]
        for t in range(32 // ns): bfly_slab(a, h, 32 * q + t * ns, ns, g)

    def zero_acc(a, q, g=None):
        z = jnp.zeros((32, DM), f32) if g is None else pltpu.bitcast(_tile(g, 32, DM), f32)
        acc[pl.ds(_mo(a * 256 + q * 32, 32), 32), :] = z

    def unpack_kv(slot, parts=range(7)):
        uk, uv = wk_buf[slot], wv_buf[slot]
        def pair(u):
            return jnp.concatenate([_lo(u), _hi(u)], axis=1)
        R = _strassen_rhs(pair(uk[0:256]), pair(uv[0:256]), pair(uk[256:512]), pair(uv[256:512]))
        for t in parts:
            R2 = _strassen_rhs(*_quad(R[t]))
            wkv_s[64 * t:64 * t + 64, :] = pltpu.bitcast(jnp.concatenate(R2, axis=1).astype(bf16), u32)

    def unpack_q(slot, parts=range(7)):
        uq = wq_buf[slot]
        R = _strassen_rhs(_lo(uq[0:512]), _hi(uq[0:512]), _lo(uq[512:1024]), _hi(uq[512:1024]))
        for t in parts: wq_s[256 * t:256 * t + 256, :] = pltpu.bitcast(R[t].astype(bf16), u32)

    def unpack_weights(slot):
        unpack_kv(slot); unpack_q(slot)

    def p1s(a):
        for h in range(2):
            for u in range(2):
                r = 4 * a + 2 * u + h
                for p in range(5):
                    k = (2 * h + u) * 5 + p
                    U = jnp.dot(a_v[r], pltpu.bitcast(rs[64 * k:64 * k + 64, :], bf16), preferred_element_type=f32)
                    ubuf[r, 0, p, 0:64, :] = U[0:64]
                    ubuf[r, 1, p, 0:64, :] = U[64:128]

    def p1d():
        for h in range(2):
            for p in range(4):
                T = jnp.dot(pltpu.bitcast(lhs_s[(4 * h + p) * 64:(4 * h + p) * 64 + 64, :], bf16), m_v[p], preferred_element_type=f32)
                tr, ti = T[:, 0:128], T[:, 128:256]
                if p == 0:
                    ny = jnp.where(lane == 0, ti, 0.0)
                    ti = jnp.where(lane == 0, 0.0, ti)
                for u in range(2):
                    k = (2 * h + u) * 5
                    rows = slice(64 * u, 64 * u + 64)
                    rs[64 * (k + p):64 * (k + p) + 64, :] = pltpu.bitcast(jnp.concatenate([tr[rows], ti[rows]], axis=0).astype(bf16), u32)
                    if p == 0:
                        rs[64 * (k + 4):64 * (k + 4) + 32, :] = pltpu.bitcast(ny[rows].astype(bf16), u32)

    def p1(a, carry):
        ap = jnp.maximum(a - 1, 0)
        with _scope('P1_wait'):
            ws = dict(a=a_copy(a_hbm, a_v, a, 0), c=c_copy(a), b=bx_copy(a))
            if OPT["wwhen"]:
                @pl.when(a >= 0)
                def _():
                    for k in OPT["wo"]: ws[k].wait()
            else:
                for k in OPT["wo"]: ws[k].wait()
        def B(h):
            for q in range(128 // OPT["bf_ns"]): bfly_slab(a, h, OPT["bf_ns"] * q, OPT["bf_ns"])
        env = dict(S=lambda: p1s(ap), B=B, P=lambda: prepass_c(a), D=p1d)
        for t in OPT["p1o"]: env[t[0]](*t[1:])
        return carry
    with _scope('P1'):
      if not OPT['attn_only']:
        rs[...] = jnp.zeros(rs.shape, u32)
        jax.lax.fori_loop(0, 8, p1, 0)
        late_starts()
        rk.wait(); rv.wait()
        if OPT["uk1"]: unpack_kv(0)
        p1s(7)
        if not OPT["uk1"]: unpack_kv(0)

    wu = wraw.bitcast(u32)

    def wpiece(ri, a):
        a0 = 128 * a
        halves = {}
        for c in range(4):
            u = wu[ri, a, pl.ds(c, 64, stride=4), :]
            halves[2 * c], halves[2 * c + 1] = _lo(u), _hi(u)
        for p in range(4):
            ka, kb = (0, 4) if p == 0 else (p, 8 - p)
            t = jnp.concatenate([halves[ka], halves[kb]], axis=0)
            wt[ri, p, a0:a0 + 128, :] = t.T
        ny = wny[ri, :, a0:a0 + 128].astype(f32)
        wt[ri, 4, a0:a0 + 128, :] = jnp.broadcast_to(ny, (128, 128)).T

    row_i = jax.lax.broadcasted_iota(jnp.int32, (128, 128), 0)
    tri = lane <= row_i

    def ldu(ref, *idx):
        return pltpu.bitcast(ref[idx], bf16)

    def kvproj(i):
        m = []
        for t in range(7):
            L = [(lambda u=u: ldu(cs, slice(t * 256 + 32 * i, t * 256 + 32 * i + 32), slice(128 * u, 128 * u + 128))) for u in range(7)]
            R = [(lambda u=u: ldu(wkv_s, slice(64 * t, 64 * t + 64), slice(128 * u, 128 * u + 128))) for u in range(7)]
            d11, d12, d21, d22 = _strassen_mul(L, R)
            m.append(jnp.concatenate([jnp.concatenate([d11, d12], axis=1), jnp.concatenate([d21, d22], axis=1)], axis=0))
        c11, c12, c21, c22 = _strassen_out(m)
        r0 = 256 * i
        _st(k_s, r0, 0, c11.astype(bf16)); _st(v_s, r0, 0, c12.astype(bf16))
        _st(k_s, r0 + 128, 0, c21.astype(bf16)); _st(v_s, r0 + 128, 0, c22.astype(bf16))

    def qproj(i):
        for q0 in range(0, 128, OPT["qrows"]): qproj_part(i, q0, OPT["qrows"])

    def qproj_part(i, q0, nr):
        t0, b0 = 128 * i + q0 // 2, 128 * i + 64 + q0 // 2
        h0 = 64 * i + q0 // 2
        L = [lambda: ldu(xs, slice(0 * (S // 4) + h0, 0 * (S // 4) + h0 + nr // 2), slice(None)), lambda: ldu(xs, slice(1 * (S // 4) + h0, 1 * (S // 4) + h0 + nr // 2), slice(None)),
             lambda: ldu(x_v, slice(t0, t0 + nr // 2), slice(0, 512)), lambda: ldu(x_v, slice(b0, b0 + nr // 2), slice(512, 1024)),
             lambda: ldu(xs, slice(2 * (S // 4) + h0, 2 * (S // 4) + h0 + nr // 2), slice(None)), lambda: ldu(xs, slice(3 * (S // 4) + h0, 3 * (S // 4) + h0 + nr // 2), slice(None)),
             lambda: ldu(xs, slice(4 * (S // 4) + h0, 4 * (S // 4) + h0 + nr // 2), slice(None))]
        R = [(lambda t=t: ldu(wq_s, slice(256 * t, 256 * t + 256), slice(None))) for t in range(7)]
        c11, c12, c21, c22 = _strassen_mul(L, R)
        r0 = 256 * i + q0
        _st(q_s, r0, 0, (jnp.concatenate([c11, c12], axis=1) * QSCALE).astype(bf16))
        _st(q_s, r0 + 128, 0, (jnp.concatenate([c21, c22], axis=1) * QSCALE).astype(bf16))

    def qk(hh, i):
        c0 = hh * D
        r0 = i * BQ
        kmain = r0 + 128
        q = _ld(q_s, r0, BQ, c0, D)
        s = jax.lax.dot_general(q, _ld(k_s, 0, kmain, c0, D), NT, preferred_element_type=f32)
        sb = jax.lax.dot_general(q[128:256], _ld(k_s, kmain, 128, c0, D), NT, preferred_element_type=f32)
        top = s[0:128]
        top_d = jnp.where(tri, top[:, r0:kmain], -1e30)
        top = jnp.concatenate([top[:, 0:r0], top_d], axis=1) if r0 else top_d
        bot = jnp.concatenate([s[128:256], jnp.where(tri, sb, -1e30)], axis=1)
        return top, bot

    Z = [0]
    pbufs = [pb0, pb1, pb2, pb3]

    def softmax(hh, i, tb):
        r0 = i * BQ
        kend = r0 + 256
        ls = []
        ps = []
        for half, s in enumerate(tb):
            kk = s.shape[1]
            if OPT["slab"]:
                sl = OPT["slab"]
                lparts, pparts = [], []
                for t in range(0, 128, sl):
                    ss = s[t:t + sl]
                    m = jnp.max(ss, axis=1, keepdims=True)
                    p = jnp.exp2(ss - m)
                    lparts.append(jnp.sum(p, axis=1, keepdims=True))
                    pb = p
                    if OPT["pbuf"]:
                        pb = p.astype(bf16)
                        pbufs[2 * hh + i % 2][(128 * half + t) // 2:(128 * half + t + sl) // 2, 0:kk] = pltpu.bitcast(pb, u32)
                    pparts.append(pb)
                ls.append(jnp.concatenate(lparts, axis=0))
                ps.append(jnp.concatenate(pparts, axis=0))
            else:
                m = jnp.max(s, axis=1, keepdims=True)
                p = jnp.exp2(s - m)
                ls.append(jnp.sum(p, axis=1, keepdims=True))
                pb = p
                if OPT["pbuf"]:
                    pb = p.astype(bf16)
                    pbufs[2 * hh + i % 2][64 * half:64 * half + 64, 0:kk] = pltpu.bitcast(pb, u32)
                ps.append(pb)
        return ps, ls

    def pv(hh, i, pl_):
        ps, ls = pl_
        c0 = hh * D
        r0 = i * BQ
        kmain = r0 + 128
        if OPT["pbuf"]:
            pmain = pltpu.bitcast(pbufs[2 * hh + i % 2][pl.ds(Z[0], 128), 0:kmain], bf16)
            pb = pltpu.bitcast(pbufs[2 * hh + i % 2][pl.ds(Z[0] + 64, 64), kmain:kmain + 128], bf16)
        else:
            pmain = jnp.concatenate([ps[0], ps[1][:, 0:kmain]], axis=0).astype(bf16)
            pb = ps[1][:, kmain:kmain + 128].astype(bf16)
        o = jnp.dot(pmain, _ld(v_s, 0, kmain, c0, D), preferred_element_type=f32)
        ob = jnp.dot(pb, _ld(v_s, kmain, 128, c0, D), preferred_element_type=f32)
        return o[0:128] * _recip(ls[0]), (o[128:256] + ob) * _recip(ls[1])

    def store_ctx(i, c0_, c1_):
        (a11, a21), (a12, a22) = c0_, c1_
        l1, l2, l5, l6, l7 = _strassen_lhs(a11, a12, a21, a22)
        for t, v in enumerate((l1, l2, a11, a22, l5, l6, l7)):
            ctx_s[64 * i:64 * i + 64, 128 * t:128 * t + 128] = pltpu.bitcast(v.astype(bf16), u32)

    def oproj(i, first=False):
        r0 = i * BQ
        nr, nc = OPT["opan"]
        if (nr, nc) != (128, 512):
            for c0 in range(0, 512, nc):
                for q0 in range(0, 128, nr):
                    L = [(lambda t=t: ldu(ctx_s, slice(64 * i + q0 // 2, 64 * i + (q0 + nr) // 2), slice(128 * t, 128 * t + 128))) for t in range(7)]
                    R = [(lambda t=t: ldu(wo_s, slice(64 * t, 64 * t + 64), slice(c0, c0 + nc))) for t in range(7)]
                    c11, c12, c21, c22 = _strassen_mul(L, R)
                    for rr, cc, v in ((r0, 0, c11), (r0, 512, c12), (r0 + 128, 0, c21), (r0 + 128, 512, c22)):
                        acc[rr + q0:rr + q0 + nr, cc + c0:cc + c0 + nc] += v
            return
        L = [(lambda t=t: ldu(ctx_s, slice(64 * i, 64 * i + 64), slice(128 * t, 128 * t + 128))) for t in range(7)]
        R = [(lambda t=t: ldu(wo_s, slice(64 * t, 64 * t + 64), slice(None))) for t in range(7)]
        c11, c12, c21, c22 = _strassen_mul(L, R)
        for rr, cc, v in ((r0, 0, c11), (r0, 512, c12), (r0 + 128, 0, c21), (r0 + 128, 512, c22)):
            if first: acc[rr:rr + 128, cc:cc + 512] = v
            else: acc[rr:rr + 128, cc:cc + 512] += v

    def prep_wo(slot, parts=range(7)):
        w = pltpu.bitcast(wo_buf[slot], bf16).astype(f32)
        R = _strassen_rhs(w[0:128, 0:512], w[0:128, 512:1024], w[128:256, 0:512], w[128:256, 512:1024])
        for t in parts: wo_s[64 * t:64 * t + 64, :] = pltpu.bitcast(R[t].astype(bf16), u32)

    def p2_unit(g, p, ps=(0, 1, 2), sub=None):
        b0 = _mo(g * 8, 8)
        bw = _mo((g % 8) * 8, 8)
        def ld(idx):
            return ([ubuf[r, 0, p, pl.ds(b0, 8), :] for r in idx], [ubuf[r, 1, p, pl.ds(b0, 8), :] for r in idx])
        def sto(idx, vr, vi):
            for r, a_, b_ in zip(idx, vr, vi):
                ubuf[r, 0, p, pl.ds(b0, 8), :] = a_
                ubuf[r, 1, p, pl.ds(b0, 8), :] = b_
        for n2 in ((range(8) if sub is None else sub) if 0 in ps else ()):
            r, i = _bfly4(*ld([8 * n1 + n2 for n1 in range(4)]), -1)
            tw = [_twid(r[k1], i[k1], n2 * k1, 32, -1) for k1 in range(4)]
            sto([8 * k1 + n2 for k1 in range(4)], [t[0] for t in tw], [t[1] for t in tw])
        for k1 in ((range(4) if sub is None else sub) if 1 in ps else ()):
            xr, xi = _bfly8(*ld([8 * k1 + n2 for n2 in range(8)]), -1)
            yr, yi = [], []
            for k2 in range(8):
                a = k1 + 4 * k2
                wr = wt[0, p, pl.ds(64 * a + bw, 8), :]
                wi = wt[1, p, pl.ds(64 * a + bw, 8), :]
                yr.append(xr[k2] * wr - xi[k2] * wi)
                yi.append(xr[k2] * wi + xi[k2] * wr)
            r, i = _bfly8(yr, yi, +1)
            tw = [_twid(r[n2], i[n2], k1 * n2, 32, +1) for n2 in range(8)]
            sto([8 * k1 + n2 for n2 in range(8)], [t[0] for t in tw], [t[1] for t in tw])
        for n2 in ((range(8) if sub is None else sub) if 2 in ps else ()):
            r, i = _bfly4(*ld([8 * k1 + n2 for k1 in range(4)]), +1)
            sto([8 * n1 + n2 for n1 in range(4)], r, i)

    def kv_first(nowo=False):
        allp = tuple(range(64 // OPT["pre_nr"]))
        if OPT['late'] == 3: late_starts()
        env = dict(K=kvproj, W=lambda i: xa_copy(i).wait(), X=lambda i: prepass(i, 1, None, allp), R=lambda: (rq.wait(), unpack_q(0)))
        for t in OPT["kf"].split(): env[t[0]](*[int(ch) for ch in t[1:]])
        if not nowo: wo_copy(0, 0).wait()

    def kv_second():
        for ri in range(2):
            for cp in wraw_copies(ri): cp.wait()
        rest = [i for i in range(8) if i not in OPT["rot"]]
        pcs = [(t, a) for a in range(16) for t in range(2)]
        n = len(rest)
        for k, i in enumerate(rest):
            mine = pcs[(32 * k) // n:(32 * (k + 1)) // n]
            for t, a in mine[:len(mine) // 2]: wpiece(t, a)
            kvproj(i)
            for t, a in mine[len(mine) // 2:]: wpiece(t, a)

    def kv_plain():
        for i in range(8):
            if i not in OPT["rot"]: kvproj(i)

    def a_iter(j, carry):
        slot = j % 2
        jn = jnp.minimum(j + 1, NPAIR - 1)

        def dma_block():
            for cp in raw_copies(jnp.minimum(j + 2, NPAIR - 1), slot): cp.start()
            wo_copy(jn, 1 - slot).start()

        def wait_block():
            with _scope('A_wait'):
                for cp in raw_copies(jn, 1 - slot): cp.wait()
                wo_copy(j, slot).wait()

        def rare():
            @pl.when(j == 0)
            def _():
                with _scope('KV0'):
                    kv_first()
                for cp in raw_copies(1, 1): cp.wait()
                if not OPT["dmain"]: dma_block()

            @pl.when(j == 1)
            def _():
                wait_block()
                if not OPT["dmain"]: dma_block()
                with _scope('KV1'):
                    kv_second()

        def common():
            wait_block()
            if not OPT["dmain"]: dma_block()
            with _scope('KVn'):
                kv_plain()
        if OPT["cf"] == 2:
            pass
        elif OPT["cf"] == 0:
            jax.lax.cond(j < 2, rare, common)
        else:
            jax.lax.cond(j >= 2, common, rare)
        gp = []
        for k in range(OPT["p2n"]):
            u = OPT["p2n"] * (j - 1) + k
            ok = jnp.logical_and(u >= 0, u < 40)
            gp.append((jnp.where(ok, u % 8, 8), jnp.where(ok, u // 8, 0)))
        zmask = jax.lax.shift_right_logical(j, 8).astype(u32)
        st = {}

        def chunks(i):
            km = i * BQ + 128
            cw = OPT["cw"]
            out, k0 = [], 0
            while k0 < km:
                n = min(cw, km - k0)
                out.append((k0, n)); k0 += n
            return out

        def QKc(hh, i, c):
            c0 = hh * D; r0 = i * BQ
            ch = chunks(i)
            if c == 0:
                st["q", hh, i] = _ld(q_s, r0, BQ, c0, D)
            q = st["q", hh, i]
            if c < len(ch):
                k0, n = ch[c]
                sc_ = jax.lax.dot_general(q, _ld(k_s, k0, n, c0, D), NT, preferred_element_type=f32)
                if k0 + n > r0:
                    top = sc_[0:128]
                    td = jnp.where(tri, top[:, n - 128:], -1e30)
                    top = jnp.concatenate([top[:, :n - 128], td], axis=1) if n > 128 else td
                    sc_ = jnp.concatenate([top, sc_[128:256]], axis=0)
                mx = sc_[:, 0:128]
                for t in range(1, n // 128): mx = jnp.maximum(mx, sc_[:, 128 * t:128 * t + 128])
                st["m", hh, i] = mx if c == 0 else jnp.maximum(st["m", hh, i], mx)
            else:
                sc_ = jax.lax.dot_general(q[128:256], _ld(k_s, r0 + 128, 128, c0, D), NT, preferred_element_type=f32)
                sc_ = jnp.where(tri, sc_, -1e30)
                m = st["m", hh, i]
                st["m", hh, i] = jnp.concatenate([m[0:128], jnp.maximum(m[128:256], sc_)], axis=0)
            st["s", hh, i, c] = sc_

        def SMc(hh, i, c):
            ch = chunks(i)
            if c == 0:
                mm = st.pop(("m", hh, i))
                if OPT["p2gate"]:
                    for gv in st.pop("gates", []):
                        gz = pltpu.bitcast((gv & zmask) | jnp.uint32(0xF149F2CA), f32)
                        mm = jnp.concatenate([jnp.maximum(mm[0:8], gz), mm[8:]], axis=0)
                st["mf", hh, i] = jnp.max(mm, axis=1, keepdims=True)
            m = st["mf", hh, i]
            sc_ = st.pop(("s", hh, i, c))
            sl = OPT["smslab"]
            if sl and c < len(ch):
                n = ch[c][1]
                lp, pp = [], []
                for t0 in range(0, 256, sl):
                    ms = m[t0:t0 + sl]
                    chain = st.setdefault("chain", [])
                    if OPT["smlag"] and len(chain) >= OPT["smlag"]:
                        gz = chain[-OPT["smlag"]][0:8, 0:128] & zmask
                        gz = jnp.concatenate([gz] * (sl // 8), axis=0)
                        ms = pltpu.bitcast(pltpu.bitcast(jnp.broadcast_to(ms, (sl, 128)), u32) | gz, f32)
                        ms = jnp.concatenate([ms] * (n // 128), axis=1)
                    p = jnp.exp2(sc_[t0:t0 + sl] - ms)
                    ls = p[:, 0:128]
                    for t in range(1, n // 128): ls = ls + p[:, 128 * t:128 * t + 128]
                    lp.append(ls)
                    pp.append(p)
                    chain.append(pltpu.bitcast(p[0:16, 0:128].astype(bf16), u32))
                ls = jnp.concatenate(lp, axis=0)
                st["l", hh, i] = ls if c == 0 else st["l", hh, i] + ls
                st["p", hh, i, c] = jnp.concatenate(pp, axis=0).astype(bf16)
                return
            if c < len(ch):
                n = ch[c][1]
                p = jnp.exp2(sc_ - m)
                ls = p[:, 0:128]
                for t in range(1, n // 128): ls = ls + p[:, 128 * t:128 * t + 128]
                st["l", hh, i] = ls if c == 0 else st["l", hh, i] + ls
            else:
                p = jnp.exp2(sc_ - m[128:256])
                l = st["l", hh, i]
                st["l", hh, i] = jnp.concatenate([l[0:128], l[128:256] + p], axis=0)
            if OPT["pbuf"]:
                k0 = ch[c][0] if c < len(ch) else i * BQ + 128
                pbufs[2 * hh + i % 2][0:p.shape[0] // 2, k0:k0 + p.shape[1]] = pltpu.bitcast(p.astype(bf16), u32)
            else:
                st["p", hh, i, c] = p.astype(bf16)

        def PVc(hh, i, c):
            c0 = hh * D; r0 = i * BQ
            ch = chunks(i)
            if OPT["pbuf"]:
                k0, n, nr = (ch[c][0], ch[c][1], 128) if c < len(ch) else (r0 + 128, 128, 64)
                p = pltpu.bitcast(pbufs[2 * hh + i % 2][0:nr, k0:k0 + n], bf16)
            else:
                p = st.pop(("p", hh, i, c))
            if c < len(ch):
                k0, n = ch[c]
                o = jnp.dot(p, _ld(v_s, k0, n, c0, D), preferred_element_type=f32)
                st["o", hh, i] = o if c == 0 else st["o", hh, i] + o
            else:
                ob = jnp.dot(p, _ld(v_s, r0 + 128, 128, c0, D), preferred_element_type=f32)
                o = st.pop(("o", hh, i))
                l = jnp.sum(st.pop(("l", hh, i)), axis=1, keepdims=True)
                r = _recip(l)
                st["ctx", hh, i] = (o[0:128] * r[0:128], (o[128:256] + ob) * r[128:256])
                if hh == 1:
                    store_ctx(i, st.pop(("ctx", 0, i)), st.pop(("ctx", 1, i)))

        def O(i): oproj(i)
        def WRAWAIT():
            @pl.when(j == 0)
            def _():
                for ri in range(2):
                    for cp in wraw_copies(ri): cp.wait()
                for a in range(16):
                    for t in range(2): wpiece(t, a)
        env = dict(WAIT=wait_block, DMA=dma_block, WW=WRAWAIT, KV=kvproj, Q=qproj, WO=lambda parts=range(7): prep_wo(slot, parts), QK=QKc, PV=PVc, SM=SMc, O=O, P2=lambda k, ps=(0, 1, 2), sub=None: p2_unit(gp[k][0], gp[k][1], ps, sub),
                   UKV=lambda parts=range(7): unpack_kv(1 - slot, parts), UQ=lambda parts=range(7): unpack_q(1 - slot, parts))
        with _scope('ATT'):
            for t in SCHED: env[t[0]](*t[1:])
        return carry
    with _scope('A'):
        if OPT["cf"] == 2:
            kv_first(nowo=True)
        jax.lax.fori_loop(0, NPAIR, a_iter, 0)

    with _scope('epi'):
        for cp in raw_copies(0, 1): cp.wait()
        wo_copy(0, 0).wait()

    mi_copy.wait()
    out_u = out_hbm.bitcast(u32)

    def y_copy(a):
        return _Two([pltpu.make_async_copy(ybuf.at[a, pl.ds(64 * u, 64)], out_u.at[:, 2 * a + u, pl.ds(DM, DM)], sem_o.at[u, a]) for u in range(2)])

    def o_copy(a):
        return pltpu.make_async_copy(obuf.at[a], out_hbm.at[pl.ds(a * 8, 8), :, pl.ds(0, DM)], sem_o.at[2, a])

    def p3(a, carry):
        r0 = pl.multiple_of(a * 256, 256)
        obuf[a] = acc[pl.ds(r0, 256), :].astype(bf16).reshape(8, 32, DM)
        o_copy(a).start()
        a_copy(ai_hbm, ai_v, a, 1).wait()
        def ldz(r, p):
            return jnp.concatenate([ubuf[r, 0, p, 0:64, :], ubuf[r, 1, p, 0:64, :]], axis=0).astype(bf16)
        U = []
        for p in range(4):
            rows = []
            for h in range(2):
                for u in range(2):
                    r = 4 * a + 2 * u + h
                    Z = jnp.dot(ai_v[r], ldz(r, p), preferred_element_type=f32)
                    zr, zi = Z[0:64], Z[64:128]
                    if p == 0:
                        Zn = jnp.dot(ai_v[r, 0:64, :], ldz(r, 4), preferred_element_type=f32)
                        zi = jnp.where(lane[0:64] == 0, Zn, zi)
                    rows.append(jnp.concatenate([zr, zi], axis=1))
            lhs = jnp.concatenate(rows, axis=0).astype(bf16)
            u = jnp.dot(lhs, mi_v[p], preferred_element_type=f32)
            U.append((u[:, 0:128], u[:, 128:256]))
        xs = _inv_butterfly8(U)
        for b in range(8):
            ybuf[a, :, 128 * b:128 * b + 128] = _pack2(xs[b][0:128], xs[b][128:256])
        y_copy(a).start()
        return carry
    with _scope('P3'):
        if not OPT['attn_only']: jax.lax.fori_loop(0, 8, p3, 0)
    with _scope('out_wait'):
        for a in range(8 if not OPT['attn_only'] else 0):
            y_copy(a).wait(); o_copy(a).wait()


KVT = [("KV", i) for i in range(8)]


def nchunks(i, cw):
    return -(-(i * BQ + 128) // cw) + 1


def sprinkle(s, pieces, pred, start=0, stop=None):
    stop = len(s) if stop is None else stop
    pos = [k for k in range(start, stop) if pred(s[k])]
    out = list(s)
    ins = {}
    for n, pc in enumerate(pieces):
        k = pos[(n * len(pos)) // len(pieces)]
        ins.setdefault(k, []).append(pc)
    res = []
    for k, t in enumerate(out):
        res += ins.get(k, [])
        res.append(t)
    return res


def fine(defer, cw, small=2, p2="pass", p2where="all"):
    s = list(KVT[:2]) + [("OP", i) for i in defer] + list(KVT[2:])
    s += [("Q", 7)]
    for i in range(7, -1, -1):
        n = nchunks(i, cw)
        s += [("QK", 0, i, c) for c in range(n)]
        qk1 = [("QK", 1, i, c) for c in range(n)]
        s += qk1[:-1] + [("SM", 0, i, 0)] + qk1[-1:]
        if i == 7: s += [("WO",), ("UKV",)]
        if i <= small:
            s += [("Q", i - 1)] if i >= 1 else [("O", 1)]
        sm = [("SM", 0, i, c) for c in range(1, n)] + [("SM", 1, i, c) for c in range(n)]
        pv = [("PV", 0, i, c) for c in range(n)] + [("PV", 1, i, c) for c in range(n)]
        for k, t in enumerate(pv):
            if k < len(sm): s += [sm[k]]
            s += [t]
        if i > small: s += [("Q", i - 1)]
        if i < 7 and i >= 1: s += [("O", i + 1)]
        if i == 1: s += [("UQ",)]
    if 0 not in defer: s += [("O", 0)]
    if p2 == "unit": pcs = [("P2", p) for p in range(5)]
    elif p2 == "pass": pcs = [("P2", p, (q,)) for q in range(3) for p in range(5)]
    elif p2 == "bfly": pcs = [("P2", p, (q,), (b,)) for q in range(3) for p in range(OPT["p2n"]) for b in range(4 if q == 1 else 8)]
    elif p2 == "bfly2": pcs = [("P2", p, (q,), (b, b + 1)) for q in range(3) for p in range(5) for b in (0, 2)]
    if p2where == "all": pred = lambda t: t[0] in ("Q", "O", "QK", "PV")
    elif p2where == "light": pred = lambda t: t[0] in ("KV", "Q")
    elif p2where == "qk": pred = lambda t: t[0] in ("Q", "QK")
    elif p2where == "kv": pred = lambda t: t[0] in ("KV",)
    elif p2where == "o": pred = lambda t: t[0] in ("KV", "Q", "O")
    return sprinkle(s, pcs, pred)


def first_sched(cw):
    base = [t for t in fine((), cw, small=0, p2="pass", p2where="qk") if t[0] not in ("P2", "UKV", "UQ")]
    s = []
    for t in base:
        if t == ("KV", 0): s += [("W1",)]
        if t[0] == "KV" and t[1] < 6: s += [("PC", t[1] + 2, tuple(range(8)))]
        if t == ("KV", 4): s += [("W2",), ("UQ0",)]
        if t == ("KV", 6): s += [("PX", 7, tuple(range(8)))]
        if t == ("KV", 7): s += [("PX", 6, tuple(range(8)))]
        if t == ("Q", 7): s += [("W3",)]
        if t == ("QK", 0, 7, 0): s += [("PX", 5, tuple(range(8)))]
        if t == ("QK", 1, 7, 0): s += [("PX", 4, tuple(range(8)))]
        if t == ("QK", 0, 6, 0): s += [("PX", 3, tuple(range(8)))]
        if t == ("QK", 1, 6, 0): s += [("PX", 2, tuple(range(8)))]
        if t == ("QK", 0, 5, 0): s += [("PX", 1, tuple(range(8)))]
        if t == ("QK", 1, 5, 0): s += [("PX", 0, tuple(range(8)))]
        if t == ("QK", 0, 4, 0): s += [("W4",), ("UKV",)]
        s.append(t)
    k0 = s.index(("W4",))
    s = sprinkle(s, [("WP", ri, a) for a in range(16) for ri in range(2)], lambda t: t[0] in ("Q", "O", "QK", "PV"), start=k0)
    s.insert(s.index(("Q", 0)) + 1, ("UQ",))
    return s


SCHEDS = {}
SCHED, DEFER = [t for t in fine((), 512, small=0, p2='bfly', p2where='qk') if t[0] != 'KV'], ()


_CONSTS = _np_consts()


def make(vmem_mb=110, sched=None, flags=None, p1sched=None, **opt):
    global SCHED, DEFER
    OPT.update(opt)
    if sched is None: sched = dict(defer=(), small=0, p2="bfly", p2where="qk", ins=[(("KV", 7), ("O", 0), 0)])
    if isinstance(sched, dict):
        SCHED, DEFER = [t for t in fine(sched["defer"], OPT["cw"], small=sched.get("small", 2), p2=sched.get("p2", "pass"), p2where=sched.get("p2where", "all")) if t[0] != "KV"], sched["defer"]
        for t, anchor, off in sched.get("ins", ()):
            SCHED.insert(SCHED.index(anchor) + off, t)
    else:
        SCHED, DEFER = list(sched), ()
    M, Mi, A, Ai = _CONSTS
    anyspec = pl.BlockSpec(memory_space=pl.ANY)
    V = pltpu.VMEM
    call = pl.pallas_call(
        _kernel,
        in_specs=[anyspec] * 13, out_specs=anyspec,
        out_shape=jax.ShapeDtypeStruct((64, 32, 2 * DM), bf16),
        scratch_shapes=[
            V((S // 2, DM), u32), V((S // 2, DC), u32), V((5 * S // 4, 512), u32),
            V((2, DM, D), u32), V((2, DC, D), u32), V((2, DC, D), u32), V((2, 128, DM), u32),
            V((7 * 256, 128), u32), V((7 * 64, 7 * 128), u32), V((7 * 64, 512), u32),
            V((S // 2, 256), u32), V((S // 2, 256), u32), V((S // 2, 256), u32), V((S // 4, 7 * 128), u32), V((S, DM), f32),
            V((8, 128, DM), u32), V((8 * 64, 256), u32), V((20 * 64, 128), u32), V((2, 16, 512, 128), bf16), V((2, 1, S), bf16), V((2, 5, S, 128), f32),
            V((32, 2, 5, 72, 128), f32),
            V((4, 256, 256), bf16), V((4, 256, 256), bf16), V((32, 128, 128), bf16), V((32, 128, 128), bf16),
            V((8, 128, DM), u32), V((8, 8, 32, DM), bf16), V((7 * 256, 7 * 128), u32), V((128, S), u32), V((128, S), u32), V((128, S), u32), V((128, S), u32),
            pltpu.SemaphoreType.DMA((8, 2)), pltpu.SemaphoreType.DMA((4, 2)), pltpu.SemaphoreType.DMA((3, 8)),
            pltpu.SemaphoreType.DMA((2, 17)), pltpu.SemaphoreType.DMA((3, 8)), pltpu.SemaphoreType.DMA((2, 8)),
        ],
        compiler_params=pltpu.CompilerParams(vmem_limit_bytes=vmem_mb * 1024 * 1024, flags=(flags or None)),
    )

    def f(A_x, A_c_kv, A_w_q, A_w_uk, A_w_uv, A_w_o, B_x, B_w_r, B_w_i):
        o = call(A_x.reshape(S, DM), A_c_kv.reshape(S, DC), A_w_q, A_w_uk, A_w_uv, A_w_o.reshape(NPAIR, 256, DM),
                 B_x.reshape(64, 32, DM), B_w_r.T, B_w_i.T, M, Mi, A, Ai)
        return o.reshape(1, S, 2 * DM)
    return f


_CALL = make()


@jax.jit
def pallas_concat_heads__compressed_kv_cla__spectral_gfnet__prompt_kernel(
        A_x, A_c_kv, A_w_q, A_w_uk, A_w_uv, A_w_o, B_x, B_w_r, B_w_i):
    return _CALL(A_x, A_c_kv, A_w_q, A_w_uk, A_w_uv, A_w_o, B_x, B_w_r, B_w_i)
```

```python
import functools
import numpy as np
import ml_dtypes
import jax
import jax.numpy as jnp
from jax.experimental import pallas as pl
from jax.experimental.pallas import tpu as pltpu

f32, bf16, u32 = jnp.float32, jnp.bfloat16, jnp.uint32
S, DM, H, D, DC = 2048, 1024, 32, 128, 512
NT = (((1,), (1,)), ((), ()))
QSCALE = float((D ** -0.5) * 1.4426950408889634)
R2 = float(np.sqrt(0.5))
NPAIR = H // 2


_CLS = ((0, 8), (4, 12), (1, 15), (9, 7), (2, 14), (10, 6), (3, 13), (11, 5))
_SG = (None, -1.0, -1.0, 1.0)


def _lane_freq():
    return np.array([np.concatenate([ka + 16 * np.arange(32), kb + 16 * np.arange(32)]) for ka, kb in _CLS])


def _cs(p):
    return float(np.cos(2 * np.pi * p / 16)), float(_SG[p] * np.sin(2 * np.pi * p / 16))


def _fwd16(x, roll, sel):
    pr = _fwd_butterfly8(x)
    a, b = pr[0]
    u0 = a + b
    out = [roll(u0) + u0 * sel(1.0, -1.0), a - b]
    for p in (1, 2, 3):
        a, b = pr[p]
        c, s_ = _cs(p)
        ar, br = roll(a), roll(b)
        base = sel(a, br)
        t = sel(ar, b) * c + sel(br, a) * sel(s_, -s_)
        out += [base + t, base - t]
    return out


def _inv16(u, roll, sel):
    u0 = roll(u[0]) + u[0] * sel(1.0, -1.0)
    pr = [(u0 + u[1], u0 - u[1])]
    for p in (1, 2, 3):
        c, s_ = _cs(p)
        base, t = u[2 * p] + u[2 * p + 1], u[2 * p] - u[2 * p + 1]
        g = t * c + roll(t) * sel(-s_, s_)
        pr.append((sel(base, roll(g)), sel(roll(base), g)))
    return _inv_butterfly8(pr)


def _fwd_butterfly8(x):
    a0, a1, a2, a3 = x[0] + x[4], x[1] + x[5], x[2] + x[6], x[3] + x[7]
    c0, c1, c2, c3 = x[0] - x[4], x[1] - x[5], x[2] - x[6], x[3] - x[7]
    s02, s13 = a0 + a2, a1 + a3
    d02, d13 = a0 - a2, a1 - a3
    t1, t2 = (c1 - c3) * R2, (c1 + c3) * R2
    return [(s02, s13), (c0 + t1, c2 + t2), (d02, d13), (c0 - t1, c2 - t2)]


def _inv_butterfly8(u):
    (s02, s13), (b1r, b1i), (d02, d13), (b3r, b3i) = u
    a0, a2 = s02 + d02, s02 - d02
    a1, a3 = s13 + d13, s13 - d13
    c0, t1 = b1r + b3r, b1r - b3r
    c2, t2 = b1i + b3i, b1i - b3i
    c1, c3 = (t1 + t2) * R2, (t2 - t1) * R2
    return [a0 + c0, a1 + c1, a2 + c2, a3 + c3, a0 - c0, a1 - c1, a2 - c2, a3 - c3]


def _d_axis_mats():
    v = _lane_freq()
    d = np.arange(DM)
    F = np.zeros((DM, 8, 2, 64))
    G = np.zeros((8, 2, 64, DM))
    for q in range(8):
        for l in range(64):
            th = 2 * np.pi * ((v[q, l] * d) % DM) / DM
            if v[q, l] == 0:
                ny = np.where(d % 2 == 0, 1.0, -1.0)
                F[:, q, 0, l], F[:, q, 1, l] = 1.0, ny
                G[q, 0, l], G[q, 1, l] = 1.0 / DM, ny / DM
            else:
                F[:, q, 0, l], F[:, q, 1, l] = np.cos(th), -np.sin(th)
                G[q, 0, l], G[q, 1, l] = 2 * np.cos(th) / DM, -2 * np.sin(th) / DM
    lo = np.arange(128) < 64
    roll = lambda t: np.roll(t, 64, axis=1)
    sel = lambda a, b: np.where(lo, a, b)
    eye = np.eye(DM)
    cols = [eye[:, 128 * j:128 * j + 128] for j in range(8)]
    L = np.concatenate(_fwd16(cols, roll, sel), axis=1)
    K = np.concatenate(_inv16(cols, roll, sel), axis=1)
    Mfull = np.linalg.solve(L, F.reshape(DM, DM))
    Ufull = G.reshape(DM, DM) @ np.linalg.inv(K)
    blk = lambda A: np.stack([A[128 * q:128 * q + 128, 128 * q:128 * q + 128] for q in range(8)])
    return blk(Mfull), blk(Ufull)


def _s_axis_mats():
    A = np.zeros((32, 128, 128))
    Ai = np.zeros((32, 128, 128))
    m = np.arange(64)
    b = np.arange(64)
    for r in range(32):
        th = 2 * np.pi * (np.outer(b, 32 * m + r) % S) / S
        Mr, Mi = np.cos(th), -np.sin(th)
        A[r] = np.block([[Mr, -Mi], [Mi, Mr]])
        Nr, Ni = np.cos(th).T / S, np.sin(th).T / S
        Ai[r] = np.block([[Nr, -Ni], [Ni, Nr]])
    return A, Ai


def _np_consts():
    M, Mi = _d_axis_mats()
    A, Ai = _s_axis_mats()
    c = lambda a: np.asarray(a, np.float32).astype(ml_dtypes.bfloat16)
    return c(M), c(Mi), c(A), c(Ai)


def _bfly4(r, i, sign):
    t0r, t0i = r[0] + r[2], i[0] + i[2]
    t1r, t1i = r[0] - r[2], i[0] - i[2]
    t2r, t2i = r[1] + r[3], i[1] + i[3]
    t3r, t3i = r[1] - r[3], i[1] - i[3]
    if sign < 0:
        o1r, o1i, o3r, o3i = t1r + t3i, t1i - t3r, t1r - t3i, t1i + t3r
    else:
        o1r, o1i, o3r, o3i = t1r - t3i, t1i + t3r, t1r + t3i, t1i - t3r
    return [t0r + t2r, o1r, t0r - t2r, o3r], [t0i + t2i, o1i, t0i - t2i, o3i]


def _twid(r, i, m, n, sign):
    m %= n
    if m == 0:
        return r, i
    if (4 * m) % n == 0:
        q = (4 * m) // n
        if sign < 0: q = (4 - q) % 4
        return [(r, i), (-i, r), (-r, -i), (i, -r)][q]
    c = np.cos(2 * np.pi * m / n)
    s = sign * np.sin(2 * np.pi * m / n)
    if (8 * m) % n == 0:
        cs = 1 if c > 0 else -1
        ss = 1 if s > 0 else -1
        a = (r - i) if cs * ss > 0 else (r + i)
        b = (i + r) if cs * ss > 0 else (i - r)
        return a * (cs * R2), b * (cs * R2)
    c, s = float(c), float(s)
    return r * c - i * s, i * c + r * s


def _bfly8(r, i, sign):
    er, ei = _bfly4(r[0::2], i[0::2], sign)
    orr, oi = _bfly4(r[1::2], i[1::2], sign)
    outr, outi = [None] * 8, [None] * 8
    for k in range(4):
        tr, ti = _twid(orr[k], oi[k], k, 8, sign)
        outr[k], outi[k] = er[k] + tr, ei[k] + ti
        outr[k + 4], outi[k + 4] = er[k] - tr, ei[k] - ti
    return outr, outi


def _lo(u):
    return pltpu.bitcast(u << 16, f32)


def _hi(u):
    return pltpu.bitcast(u & jnp.uint32(0xFFFF0000), f32)


def _recip(l):
    r = pl.reciprocal(l, approx=True)
    return r * (2.0 - l * r)


def _pack2(lo, hi):
    lo_b = pltpu.bitcast(lo.astype(bf16).astype(f32), u32) >> 16
    hi_b = pltpu.bitcast(hi.astype(bf16).astype(f32), u32)
    return lo_b | hi_b


def _mo(x, m):
    return x if isinstance(x, int) else pl.multiple_of(x, m)


BQ = 256
NBLK = S // BQ


def _strassen_lhs(a11, a12, a21, a22):
    return a11 + a22, a21 + a22, a11 + a12, a21 - a11, a12 - a22


def _strassen_rhs(b11, b12, b21, b22):
    return b11 + b22, b11, b12 - b22, b21 - b11, b22, b11 + b12, b21 + b22


def _strassen_lhs7(a11, a12, a21, a22):
    l1, l2, l5, l6, l7 = _strassen_lhs(a11, a12, a21, a22)
    return l1, l2, a11, a22, l5, l6, l7


def _quad(a):
    r, c = a.shape[0] // 2, a.shape[1] // 2
    return a[:r, :c], a[:r, c:], a[r:, :c], a[r:, c:]


def _strassen_mul(L, R):
    return _strassen_out([jnp.dot(L[t](), R[t](), preferred_element_type=f32) for t in range(7)])


def _strassen_out(m):
    return m[0] + m[3] - m[4] + m[6], m[2] + m[4], m[1] + m[3], m[0] - m[1] + m[2] + m[5]


def _ld(ref, r0, nr, c0, nc):
    return pltpu.bitcast(ref[r0 // 2:(r0 + nr) // 2, c0:c0 + nc], bf16)


def _st(ref, r0, c0, val):
    nr, nc = val.shape
    ref[r0 // 2:(r0 + nr) // 2, c0:c0 + nc] = pltpu.bitcast(val, u32)


def _kernel(x_hbm, c_hbm, wq_hbm, wk_hbm, wv_hbm, wo_hbm, bx_hbm, wr_hbm, wi_hbm, m_hbm, mi_hbm, a_hbm, ai_hbm,
            out_hbm,
            x_v, c_v, xs, wq_buf, wk_buf, wv_buf, wo_buf, wq_s, wkv_s, wo_s, q_s, k_s, v_s, ctx_s, acc,
            xbuf, lhs_s, rs, wraw, wny, wt, ubuf, m_v, mi_v, a_v, ai_v, ybuf, obuf, cs,
            sem_x, sem_w, sem_c, sem_wt, sem_o, sem_xc):
    class _Two:
        def __init__(self, cps): self.cps = cps
        def start(self):
            for cp in self.cps: cp.start()
        def wait(self):
            for cp in self.cps: cp.wait()

    def bx_copy(a):
        return _Two([pltpu.make_async_copy(bx_hbm.bitcast(u32).at[:, 2 * a + u, :], xbuf.at[a, pl.ds(64 * u, 64)], sem_x.at[a, u]) for u in range(2)])

    def a_copy(hbm, dst, a, k):
        return pltpu.make_async_copy(hbm.at[pl.ds(4 * a, 4)], dst.at[pl.ds(4 * a, 4)], sem_c.at[k, a])

    m_copy = pltpu.make_async_copy(m_hbm, m_v, sem_c.at[2, 0])
    mi_copy = pltpu.make_async_copy(mi_hbm, mi_v, sem_c.at[2, 1])

    def xa_copy(a):
        return pltpu.make_async_copy(x_hbm.bitcast(u32).at[pl.ds(a * 128, 128)], x_v.at[pl.ds(a * 128, 128)], sem_xc.at[0, a])

    def c_copy(a):
        return pltpu.make_async_copy(c_hbm.bitcast(u32).at[pl.ds(a * 128, 128)], c_v.at[pl.ds(a * 128, 128)], sem_xc.at[1, a])

    def wraw_copies(ri):
        src = (wr_hbm, wi_hbm)[ri]
        cps = [pltpu.make_async_copy(src.at[0:512, pl.ds(128 * a, 128)], wraw.at[ri, a], sem_wt.at[ri, a]) for a in range(16)]
        cps.append(pltpu.make_async_copy(src.at[pl.ds(512, 1), :], wny.at[ri], sem_wt.at[ri, 16]))
        return cps

    def raw_copies(j, slot):
        return (pltpu.make_async_copy(wk_hbm.bitcast(u32).at[:, j, :], wk_buf.at[slot], sem_w.at[1, slot]),
                pltpu.make_async_copy(wv_hbm.bitcast(u32).at[:, j, :], wv_buf.at[slot], sem_w.at[2, slot]),
                pltpu.make_async_copy(wq_hbm.bitcast(u32).at[:, j, :], wq_buf.at[slot], sem_w.at[0, slot]))

    def wo_copy(j, slot):
        return pltpu.make_async_copy(wo_hbm.bitcast(u32).at[j], wo_buf.at[slot], sem_w.at[3, slot])

    rk, rv, rq = raw_copies(0, 0)
    for a in range(8):
        bx_copy(a).start()
        if a == 0: m_copy.start()
        a_copy(a_hbm, a_v, a, 0).start()
        c_copy(a).start()
        if a == 5: rk.start(); rv.start()
    def mid_starts():
        rq.start()
        for i in range(7, -1, -1): xa_copy(i).start()
        wo_copy(0, 0).start()
        for cp in raw_copies(1, 1): cp.start()

    def late_starts():
        for ri in range(2):
            for cp in wraw_copies(ri): cp.start()
        mi_copy.start()
        for a in range(8): a_copy(ai_hbm, ai_v, a, 1).start()
    mid_starts()

    lane = jax.lax.broadcasted_iota(jnp.int32, (128, 128), 1)

    def roll(t): return pltpu.roll(t, 64, 1)

    def sel(a_, b_):
        ref = a_ if hasattr(a_, "shape") else None
        if ref is None: return jnp.where(lane[0:8] < 64, a_, b_)[0:1]
        return jnp.where(jax.lax.broadcasted_iota(jnp.int32, ref.shape, 1) < 64, a_, b_)

    def zero_rows(a, carry):
        r0 = pl.multiple_of(a * 256, 256)
        acc[pl.ds(r0, 256), :] = jnp.zeros((256, DM), f32)
        for t in range(4):
            for ri in range(2):
                ubuf[4 * a + t, ri, 0, 64:72, :] = jnp.zeros((8, 128), f32)
                wt[ri, 0, pl.ds(r0 + 64 * t, 8), :] = jnp.zeros((8, 128), f32)
        return carry
    jax.lax.fori_loop(0, 8, zero_rows, 0)
    m_copy.wait()

    def prepass_c(i):
        nr = 8
        for q in range(4):
            rows = [c_v[pl.ds(_mo(i * 128 + 32 * k + q * nr, nr), nr), :] for k in range(4)]
            rows = [pltpu.bitcast(u, bf16).astype(f32) for u in rows]
            top = jnp.concatenate(rows[0:2], axis=0)
            bot = jnp.concatenate(rows[2:4], axis=0)
            L1 = _strassen_lhs7(top[:, 0:256], top[:, 256:512], bot[:, 0:256], bot[:, 256:512])
            for t in range(7):
                L2 = _strassen_lhs7(*_quad(L1[t]))
                cs[pl.ds(_mo(t * 256 + 32 * i + q * nr, nr), nr), :] = pltpu.bitcast(jnp.concatenate(L2, axis=1).astype(bf16), u32)

    def prepass_x(i):
        nr, w = 8, 512
        for q in range(8):
            top = pltpu.bitcast(x_v[pl.ds(i * 128 + q * nr, nr), :], bf16).astype(f32)
            bot = pltpu.bitcast(x_v[pl.ds(i * 128 + 64 + q * nr, nr), :], bf16).astype(f32)
            L = _strassen_lhs(top[:, 0:w], top[:, w:2 * w], bot[:, 0:w], bot[:, w:2 * w])
            for t in range(5): xs[pl.ds(t * (S // 4) + i * 64 + q * nr, nr), :] = pltpu.bitcast(L[t].astype(bf16), u32)

    def bfly_slab(a, h, s0, ns):
        half = _lo if h == 0 else _hi
        us = [xbuf[a, s0:s0 + ns, 128 * b:128 * b + 128] for b in range(8)]
        xb = [half(u) for u in us]
        Bq = _fwd16(xb, roll, sel)
        lhs_s[64 * h + s0 // 2:64 * h + (s0 + ns) // 2, :] = pltpu.bitcast(jnp.concatenate(Bq, axis=1).astype(bf16), u32)

    def unpack_kv(slot, parts=range(7)):
        uk, uv = wk_buf[slot], wv_buf[slot]
        def pair(u):
            return jnp.concatenate([_lo(u), _hi(u)], axis=1)
        R = _strassen_rhs(pair(uk[0:256]), pair(uv[0:256]), pair(uk[256:512]), pair(uv[256:512]))
        for t in parts:
            R2 = _strassen_rhs(*_quad(R[t]))
            wkv_s[64 * t:64 * t + 64, :] = pltpu.bitcast(jnp.concatenate(R2, axis=1).astype(bf16), u32)

    def unpack_q(slot, parts=range(7)):
        uq = wq_buf[slot]
        R = _strassen_rhs(_lo(uq[0:512]), _hi(uq[0:512]), _lo(uq[512:1024]), _hi(uq[512:1024]))
        for t in parts: wq_s[256 * t:256 * t + 256, :] = pltpu.bitcast(R[t].astype(bf16), u32)

    def p1s(a):
        for h in range(2):
            for u in range(2):
                r = 4 * a + 2 * u + h
                for p in range(5):
                    k = (2 * h + u) * 5 + p
                    U = jnp.dot(a_v[r], pltpu.bitcast(rs[64 * k:64 * k + 64, :], bf16), preferred_element_type=f32)
                    ubuf[r, 0, p, 0:64, :] = U[0:64]
                    ubuf[r, 1, p, 0:64, :] = U[64:128]

    def p1d():
        for h in range(2):
            for p in range(4):
                Ta, Tb = [jnp.dot(pltpu.bitcast(lhs_s[64 * h:64 * h + 64, 128 * q:128 * q + 128], bf16), m_v[q], preferred_element_type=f32)
                          for q in (2 * p, 2 * p + 1)]
                tr, ti = sel(Ta, roll(Tb)), sel(roll(Ta), Tb)
                if p == 0:
                    ny = jnp.where(lane == 0, ti, 0.0)
                    ti = jnp.where(lane == 0, 0.0, ti)
                for u in range(2):
                    k = (2 * h + u) * 5
                    rows = slice(64 * u, 64 * u + 64)
                    rs[64 * (k + p):64 * (k + p) + 64, :] = pltpu.bitcast(jnp.concatenate([tr[rows], ti[rows]], axis=0).astype(bf16), u32)
                    if p == 0:
                        rs[64 * (k + 4):64 * (k + 4) + 32, :] = pltpu.bitcast(ny[rows].astype(bf16), u32)

    def p1(a, carry):
        ap = jnp.maximum(a - 1, 0)
        a_copy(a_hbm, a_v, a, 0).wait(); c_copy(a).wait(); bx_copy(a).wait()
        p1s(ap)
        for h in range(2):
            for q in range(8): bfly_slab(a, h, 16 * q, 16)
        prepass_c(a)
        p1d()
        return carry
    rs[...] = jnp.zeros(rs.shape, u32)
    jax.lax.fori_loop(0, 8, p1, 0)
    late_starts()
    rk.wait(); rv.wait()
    p1s(7)
    unpack_kv(0)

    wu = wraw.bitcast(u32)

    def wpiece(ri, a):
        a0 = 128 * a
        halves = {}
        for c in range(8):
            u = wu[ri, a, pl.ds(c, 32, stride=8), :]
            halves[2 * c], halves[2 * c + 1] = _lo(u), _hi(u)
        for p in range(4):
            t = jnp.concatenate([halves[k] for k in _CLS[2 * p] + _CLS[2 * p + 1]], axis=0)
            wt[ri, p, a0:a0 + 128, :] = t.T
        ny = wny[ri, :, a0:a0 + 128].astype(f32)
        wt[ri, 4, a0:a0 + 128, :] = jnp.broadcast_to(ny, (128, 128)).T

    row_i = jax.lax.broadcasted_iota(jnp.int32, (128, 128), 0)
    tri = lane <= row_i

    def ldu(ref, *idx):
        return pltpu.bitcast(ref[idx], bf16)

    def kvproj(i):
        m = []
        for t in range(7):
            L = [(lambda u=u: ldu(cs, slice(t * 256 + 32 * i, t * 256 + 32 * i + 32), slice(128 * u, 128 * u + 128))) for u in range(7)]
            R = [(lambda u=u: ldu(wkv_s, slice(64 * t, 64 * t + 64), slice(128 * u, 128 * u + 128))) for u in range(7)]
            d11, d12, d21, d22 = _strassen_mul(L, R)
            m.append(jnp.concatenate([jnp.concatenate([d11, d12], axis=1), jnp.concatenate([d21, d22], axis=1)], axis=0))
        c11, c12, c21, c22 = _strassen_out(m)
        r0 = 256 * i
        _st(k_s, r0, 0, c11.astype(bf16)); _st(v_s, r0, 0, c12.astype(bf16))
        _st(k_s, r0 + 128, 0, c21.astype(bf16)); _st(v_s, r0 + 128, 0, c22.astype(bf16))

    def qproj(i):
        qproj_part(i, 0, 128)

    def qproj_part(i, q0, nr):
        t0, b0 = 128 * i + q0 // 2, 128 * i + 64 + q0 // 2
        h0 = 64 * i + q0 // 2
        L = [lambda: ldu(xs, slice(0 * (S // 4) + h0, 0 * (S // 4) + h0 + nr // 2), slice(None)), lambda: ldu(xs, slice(1 * (S // 4) + h0, 1 * (S // 4) + h0 + nr // 2), slice(None)),
             lambda: ldu(x_v, slice(t0, t0 + nr // 2), slice(0, 512)), lambda: ldu(x_v, slice(b0, b0 + nr // 2), slice(512, 1024)),
             lambda: ldu(xs, slice(2 * (S // 4) + h0, 2 * (S // 4) + h0 + nr // 2), slice(None)), lambda: ldu(xs, slice(3 * (S // 4) + h0, 3 * (S // 4) + h0 + nr // 2), slice(None)),
             lambda: ldu(xs, slice(4 * (S // 4) + h0, 4 * (S // 4) + h0 + nr // 2), slice(None))]
        R = [(lambda t=t: ldu(wq_s, slice(256 * t, 256 * t + 256), slice(None))) for t in range(7)]
        c11, c12, c21, c22 = _strassen_mul(L, R)
        r0 = 256 * i + q0
        _st(q_s, r0, 0, (jnp.concatenate([c11, c12], axis=1) * QSCALE).astype(bf16))
        _st(q_s, r0 + 128, 0, (jnp.concatenate([c21, c22], axis=1) * QSCALE).astype(bf16))

    def store_ctx(i, c0_, c1_):
        (a11, a21), (a12, a22) = c0_, c1_
        l1, l2, l5, l6, l7 = _strassen_lhs(a11, a12, a21, a22)
        for t, v in enumerate((l1, l2, a11, a22, l5, l6, l7)):
            ctx_s[64 * i:64 * i + 64, 128 * t:128 * t + 128] = pltpu.bitcast(v.astype(bf16), u32)

    def oproj(i, pan):
        r0 = i * BQ
        nr, nc = 64, 128
        if True:
            for c0 in [pan * nc]:
                for q0 in range(0, 128, nr):
                    L = [(lambda t=t: ldu(ctx_s, slice(64 * i + q0 // 2, 64 * i + (q0 + nr) // 2), slice(128 * t, 128 * t + 128))) for t in range(7)]
                    R = [(lambda t=t: ldu(wo_s, slice(64 * t, 64 * t + 64), slice(c0, c0 + nc))) for t in range(7)]
                    c11, c12, c21, c22 = _strassen_mul(L, R)
                    for rr, cc, v in ((r0, 0, c11), (r0, 512, c12), (r0 + 128, 0, c21), (r0 + 128, 512, c22)):
                        acc[rr + q0:rr + q0 + nr, cc + c0:cc + c0 + nc] += v

    def prep_wo(slot, parts=range(7)):
        w = pltpu.bitcast(wo_buf[slot], bf16).astype(f32)
        R = _strassen_rhs(w[0:128, 0:512], w[0:128, 512:1024], w[128:256, 0:512], w[128:256, 512:1024])
        for t in parts: wo_s[64 * t:64 * t + 64, :] = pltpu.bitcast(R[t].astype(bf16), u32)

    def p2_unit(g, p, ps=(0, 1, 2), sub=None):
        b0 = _mo(g * 8, 8)
        bw = _mo((g % 8) * 8, 8)
        def ld(idx):
            return ([ubuf[r, 0, p, pl.ds(b0, 8), :] for r in idx], [ubuf[r, 1, p, pl.ds(b0, 8), :] for r in idx])
        def sto(idx, vr, vi):
            for r, a_, b_ in zip(idx, vr, vi):
                ubuf[r, 0, p, pl.ds(b0, 8), :] = a_
                ubuf[r, 1, p, pl.ds(b0, 8), :] = b_
        for n2 in ((range(8) if sub is None else sub) if 0 in ps else ()):
            r, i = _bfly4(*ld([8 * n1 + n2 for n1 in range(4)]), -1)
            tw = [_twid(r[k1], i[k1], n2 * k1, 32, -1) for k1 in range(4)]
            sto([8 * k1 + n2 for k1 in range(4)], [t[0] for t in tw], [t[1] for t in tw])
        for k1 in ((range(4) if sub is None else sub) if 1 in ps else ()):
            xr, xi = _bfly8(*ld([8 * k1 + n2 for n2 in range(8)]), -1)
            yr, yi = [], []
            for k2 in range(8):
                a = k1 + 4 * k2
                wr = wt[0, p, pl.ds(64 * a + bw, 8), :]
                wi = wt[1, p, pl.ds(64 * a + bw, 8), :]
                yr.append(xr[k2] * wr - xi[k2] * wi)
                yi.append(xr[k2] * wi + xi[k2] * wr)
            r, i = _bfly8(yr, yi, +1)
            tw = [_twid(r[n2], i[n2], k1 * n2, 32, +1) for n2 in range(8)]
            sto([8 * k1 + n2 for n2 in range(8)], [t[0] for t in tw], [t[1] for t in tw])
        for n2 in ((range(8) if sub is None else sub) if 2 in ps else ()):
            r, i = _bfly4(*ld([8 * k1 + n2 for k1 in range(4)]), +1)
            sto([8 * n1 + n2 for n1 in range(4)], r, i)

    def kv_first():
        env = dict(K=kvproj, W=lambda i: xa_copy(i).wait(), X=prepass_x, R=lambda: (rq.wait(), unpack_q(0)))
        for t in "K0 R W7 W6 W5 W4 X7 K1 X6 K2 X5 K3 X4 K4 W3 W2 W1 W0 X3 K5 X2 K6 X1 K7 X0".split(): env[t[0]](*[int(ch) for ch in t[1:]])
        wo_copy(0, 0).wait()

    def kv_second():
        for ri in range(2):
            for cp in wraw_copies(ri): cp.wait()
        rest = list(range(7))
        pcs = [(t, a) for a in range(16) for t in range(2)]
        n = len(rest)
        for k, i in enumerate(rest):
            mine = pcs[(32 * k) // n:(32 * (k + 1)) // n]
            for t, a in mine[:len(mine) // 2]: wpiece(t, a)
            kvproj(i)
            for t, a in mine[len(mine) // 2:]: wpiece(t, a)

    def kv_plain():
        for i in range(7): kvproj(i)

    def a_iter(j, carry):
        slot = j % 2
        jn = jnp.minimum(j + 1, NPAIR - 1)

        def dma_block():
            for cp in raw_copies(jnp.minimum(j + 2, NPAIR - 1), slot): cp.start()
            wo_copy(jn, 1 - slot).start()

        def wait_block():
            for cp in raw_copies(jn, 1 - slot): cp.wait()
            wo_copy(j, slot).wait()

        def rare():
            @pl.when(j == 0)
            def _():
                kv_first()
                for cp in raw_copies(1, 1): cp.wait()
                dma_block()

            @pl.when(j == 1)
            def _():
                wait_block()
                dma_block()
                kv_second()

        def common():
            wait_block()
            dma_block()
            kv_plain()
        jax.lax.cond(j < 2, rare, common)
        gp = []
        for k in range(3):
            u = 3 * (j - 1) + k
            ok = jnp.logical_and(u >= 0, u < 40)
            gp.append((jnp.where(ok, u % 8, 8), jnp.where(ok, u // 8, 0)))
        st = {}

        def chunks(i):
            km = i * BQ + 128
            cw = 512
            out, k0 = [], 0
            while k0 < km:
                n = min(cw, km - k0)
                out.append((k0, n)); k0 += n
            return out

        def QKc(hh, i, c):
            c0 = hh * D; r0 = i * BQ
            ch = chunks(i)
            if c == 0:
                st["q", hh, i] = _ld(q_s, r0, BQ, c0, D)
            q = st["q", hh, i]
            if c < len(ch):
                k0, n = ch[c]
                sc_ = jax.lax.dot_general(q, _ld(k_s, k0, n, c0, D), NT, preferred_element_type=f32)
                if k0 + n > r0:
                    top = sc_[0:128]
                    td = jnp.where(tri, top[:, n - 128:], -1e30)
                    top = jnp.concatenate([top[:, :n - 128], td], axis=1) if n > 128 else td
                    sc_ = jnp.concatenate([top, sc_[128:256]], axis=0)
                mx = sc_[:, 0:128]
                for t in range(1, n // 128): mx = jnp.maximum(mx, sc_[:, 128 * t:128 * t + 128])
                st["m", hh, i] = mx if c == 0 else jnp.maximum(st["m", hh, i], mx)
            else:
                sc_ = jax.lax.dot_general(q[128:256], _ld(k_s, r0 + 128, 128, c0, D), NT, preferred_element_type=f32)
                sc_ = jnp.where(tri, sc_, -1e30)
                m = st["m", hh, i]
                st["m", hh, i] = jnp.concatenate([m[0:128], jnp.maximum(m[128:256], sc_)], axis=0)
            st["s", hh, i, c] = sc_

        def SMc(hh, i, c):
            ch = chunks(i)
            if c == 0:
                mm = st.pop(("m", hh, i))
                st["mf", hh, i] = jnp.max(mm, axis=1, keepdims=True)
            m = st["mf", hh, i]
            sc_ = st.pop(("s", hh, i, c))
            if c < len(ch):
                n = ch[c][1]
                p = jnp.exp2(sc_ - m)
                ls = p[:, 0:128]
                for t in range(1, n // 128): ls = ls + p[:, 128 * t:128 * t + 128]
                st["l", hh, i] = ls if c == 0 else st["l", hh, i] + ls
            else:
                p = jnp.exp2(sc_ - m[128:256])
                l = st["l", hh, i]
                st["l", hh, i] = jnp.concatenate([l[0:128], l[128:256] + p], axis=0)
            st["p", hh, i, c] = p.astype(bf16)

        def PVc(hh, i, c):
            c0 = hh * D; r0 = i * BQ
            ch = chunks(i)
            p = st.pop(("p", hh, i, c))
            if c < len(ch):
                k0, n = ch[c]
                o = jnp.dot(p, _ld(v_s, k0, n, c0, D), preferred_element_type=f32)
                st["o", hh, i] = o if c == 0 else st["o", hh, i] + o
            else:
                ob = jnp.dot(p, _ld(v_s, r0 + 128, 128, c0, D), preferred_element_type=f32)
                o = st.pop(("o", hh, i))
                l = jnp.sum(st.pop(("l", hh, i)), axis=1, keepdims=True)
                r = _recip(l)
                st["ctx", hh, i] = (o[0:128] * r[0:128], (o[128:256] + ob) * r[128:256])
                if hh == 1:
                    store_ctx(i, st.pop(("ctx", 0, i)), st.pop(("ctx", 1, i)))


        env = dict(KV=kvproj, Q=qproj, WO=lambda parts=range(7): prep_wo(slot, parts), QK=QKc, PV=PVc, SM=SMc, O=oproj, P2=lambda k, ps=(0, 1, 2), sub=None: p2_unit(gp[k][0], gp[k][1], ps, sub),
                   UKV=lambda parts=range(7): unpack_kv(1 - slot, parts), UQ=lambda parts=range(7): unpack_q(1 - slot, parts))
        for t in SCHED: env[t[0]](*t[1:])
        return carry
    jax.lax.fori_loop(0, NPAIR, a_iter, 0)
    for cp in raw_copies(0, 1): cp.wait()
    wo_copy(0, 0).wait()

    mi_copy.wait()
    out_u = out_hbm.bitcast(u32)

    def y_copy(a):
        return _Two([pltpu.make_async_copy(ybuf.at[a, pl.ds(64 * u, 64)], out_u.at[:, 2 * a + u, pl.ds(DM, DM)], sem_o.at[u, a]) for u in range(2)])

    def o_copy(a):
        return pltpu.make_async_copy(obuf.at[a], out_hbm.at[pl.ds(a * 8, 8), :, pl.ds(0, DM)], sem_o.at[2, a])

    def p3(a, carry):
        r0 = pl.multiple_of(a * 256, 256)
        obuf[a] = acc[pl.ds(r0, 256), :].astype(bf16).reshape(8, 32, DM)
        o_copy(a).start()
        a_copy(ai_hbm, ai_v, a, 1).wait()
        def ldz(r, p):
            return jnp.concatenate([ubuf[r, 0, p, 0:64, :], ubuf[r, 1, p, 0:64, :]], axis=0).astype(bf16)
        U = []
        for p in range(4):
            rows = []
            for h in range(2):
                for u in range(2):
                    r = 4 * a + 2 * u + h
                    Z = jnp.dot(ai_v[r], ldz(r, p), preferred_element_type=f32)
                    zr, zi = Z[0:64], Z[64:128]
                    if p == 0:
                        Zn = jnp.dot(ai_v[r, 0:64, :], ldz(r, 4), preferred_element_type=f32)
                        zi = jnp.where(lane[0:64] == 0, Zn, zi)
                    rows.append((sel(zr, roll(zi)), sel(roll(zr), zi)))
            for e in range(2):
                lhs = jnp.concatenate([t[e] for t in rows], axis=0).astype(bf16)
                U.append(jnp.dot(lhs, mi_v[2 * p + e], preferred_element_type=f32))
        xs = _inv16(U, roll, sel)
        for b in range(8):
            ybuf[a, :, 128 * b:128 * b + 128] = _pack2(xs[b][0:128], xs[b][128:256])
        y_copy(a).start()
        return carry
    jax.lax.fori_loop(0, 8, p3, 0)
    for a in range(8):
        y_copy(a).wait(); o_copy(a).wait()


SCHED = [('P2', 0, (0,), (4,)), ('P2', 1, (0,), (0,)), ('P2', 0, (0,), (0,)), ('Q', 7), ('P2', 0, (0,), (1,)), ('QK', 0, 7, 0), ('P2', 0, (0,), (2,)), ('QK', 0, 7, 1), ('P2', 0, (0,), (3,)), ('QK', 0, 7, 2), ('QK', 0, 7, 3), ('P2', 0, (0,), (5,)), ('QK', 0, 7, 4), ('P2', 0, (0,), (6,)), ('QK', 1, 7, 0), ('WO',), ('QK', 1, 7, 1), ('QK', 1, 7, 2), ('UKV',), ('QK', 1, 7, 3), ('P2', 1, (0,), (2,)), ('P2', 1, (0,), (1,)), ('QK', 1, 7, 4), ('SM', 0, 7, 0), ('SM', 0, 7, 1), ('PV', 0, 7, 0), ('SM', 0, 7, 2), ('P2', 1, (0,), (4,)), ('PV', 0, 7, 1), ('SM', 0, 7, 3), ('Q', 6), ('PV', 0, 7, 2), ('SM', 0, 7, 4), ('PV', 0, 7, 3), ('PV', 0, 7, 4), ('SM', 1, 7, 0), ('SM', 1, 7, 1), ('PV', 1, 7, 0), ('PV', 1, 7, 1), ('P2', 1, (0,), (7,)), ('P2', 0, (0,), (7,)), ('SM', 1, 7, 2), ('PV', 1, 7, 2), ('SM', 1, 7, 3), ('P2', 2, (0,), (3,)), ('SM', 1, 7, 4), ('PV', 1, 7, 3), ('P2', 1, (0,), (3,)), ('QK', 0, 6, 0), ('PV', 1, 7, 4), ('P2', 1, (0,), (5,)), ('QK', 0, 6, 1), ('P2', 1, (0,), (6,)), ('QK', 0, 6, 2), ('QK', 0, 6, 3), ('QK', 0, 6, 4), ('P2', 2, (0,), (0,)), ('QK', 1, 6, 0), ('P2', 2, (0,), (1,)), ('QK', 1, 6, 1), ('P2', 2, (0,), (2,)), ('QK', 1, 6, 2), ('QK', 1, 6, 3), ('SM', 0, 6, 0), ('P2', 2, (0,), (4,)), ('QK', 1, 6, 4), ('SM', 0, 6, 1), ('PV', 0, 6, 0), ('SM', 0, 6, 2), ('PV', 0, 6, 1), ('SM', 0, 6, 3), ('PV', 0, 6, 2), ('SM', 0, 6, 4), ('PV', 0, 6, 3), ('SM', 1, 6, 0), ('P2', 0, (1,), (0,)), ('PV', 0, 6, 4), ('SM', 1, 6, 1), ('PV', 1, 6, 0), ('SM', 1, 6, 2), ('SM', 1, 6, 3), ('PV', 1, 6, 1), ('PV', 1, 6, 2), ('SM', 1, 6, 4), ('PV', 1, 6, 3), ('PV', 1, 6, 4), ('P2', 2, (0,), (5,)), ('Q', 5), ('P2', 0, (1,), (3,)), ('O', 7, 0), ('O', 7, 2), ('O', 7, 1), ('P2', 2, (0,), (6,)), ('QK', 0, 5, 0), ('P2', 2, (0,), (7,)), ('QK', 0, 5, 1), ('QK', 0, 5, 2), ('P2', 0, (1,), (1,)), ('QK', 0, 5, 3), ('P2', 0, (1,), (2,)), ('QK', 1, 5, 0), ('QK', 1, 5, 1), ('O', 7, 3), ('SM', 0, 5, 0), ('QK', 1, 5, 2), ('P2', 1, (1,), (1,)), ('SM', 0, 5, 1), ('QK', 1, 5, 3), ('P2', 1, (1,), (0,)), ('SM', 0, 5, 2), ('PV', 0, 5, 0), ('PV', 0, 5, 1), ('SM', 0, 5, 3), ('PV', 0, 5, 2), ('PV', 0, 5, 3), ('SM', 1, 5, 0), ('SM', 1, 5, 1), ('PV', 1, 5, 0), ('SM', 1, 5, 2), ('O', 6, 0), ('PV', 1, 5, 1), ('Q', 4), ('PV', 1, 5, 2), ('SM', 1, 5, 3), ('PV', 1, 5, 3), ('O', 6, 1), ('O', 6, 2), ('O', 6, 3), ('P2', 1, (1,), (2,)), ('QK', 0, 4, 0), ('P2', 1, (1,), (3,)), ('QK', 0, 4, 1), ('P2', 2, (1,), (0,)), ('QK', 0, 4, 2), ('P2', 2, (1,), (1,)), ('QK', 0, 4, 3), ('QK', 1, 4, 0), ('P2', 2, (1,), (2,)), ('QK', 1, 4, 1), ('P2', 0, (2,), (0,)), ('QK', 1, 4, 2), ('SM', 0, 4, 0), ('P2', 0, (2,), (1,)), ('QK', 1, 4, 3), ('P2', 2, (1,), (3,)), ('SM', 0, 4, 1), ('PV', 0, 4, 0), ('SM', 0, 4, 2), ('PV', 0, 4, 1), ('SM', 0, 4, 3), ('PV', 0, 4, 2), ('SM', 1, 4, 0), ('PV', 0, 4, 3), ('SM', 1, 4, 1), ('PV', 1, 4, 0), ('SM', 1, 4, 2), ('PV', 1, 4, 1), ('Q', 3), ('SM', 1, 4, 3), ('PV', 1, 4, 2), ('PV', 1, 4, 3), ('P2', 0, (2,), (2,)), ('O', 5, 0), ('O', 5, 1), ('O', 5, 3), ('P2', 0, (2,), (3,)), ('QK', 0, 3, 0), ('QK', 0, 3, 1), ('O', 5, 2), ('P2', 0, (2,), (5,)), ('QK', 0, 3, 2), ('P2', 0, (2,), (6,)), ('QK', 1, 3, 0), ('P2', 0, (2,), (7,)), ('QK', 1, 3, 1), ('P2', 0, (2,), (4,)), ('SM', 0, 3, 0), ('QK', 1, 3, 2), ('SM', 1, 3, 0), ('SM', 0, 3, 1), ('PV', 0, 3, 0), ('SM', 0, 3, 2), ('PV', 0, 3, 1), ('O', 4, 3), ('O', 4, 1), ('PV', 0, 3, 2), ('PV', 1, 3, 0), ('SM', 1, 3, 1), ('P2', 1, (2,), (0,)), ('O', 4, 2), ('SM', 1, 3, 2), ('P2', 1, (2,), (4,)), ('PV', 1, 3, 1), ('PV', 1, 3, 2), ('Q', 2), ('O', 4, 0), ('P2', 1, (2,), (1,)), ('QK', 0, 2, 0), ('QK', 0, 2, 1), ('P2', 1, (2,), (3,)), ('QK', 0, 2, 2), ('QK', 1, 2, 0), ('P2', 1, (2,), (2,)), ('P2', 1, (2,), (5,)), ('QK', 1, 2, 1), ('SM', 0, 2, 0), ('QK', 1, 2, 2), ('SM', 0, 2, 1), ('PV', 0, 2, 0), ('SM', 0, 2, 2), ('PV', 0, 2, 1), ('SM', 1, 2, 0), ('P2', 1, (2,), (6,)), ('SM', 1, 2, 1), ('PV', 0, 2, 2), ('PV', 1, 2, 0), ('SM', 1, 2, 2), ('PV', 1, 2, 1), ('PV', 1, 2, 2), ('O', 3, 2), ('P2', 1, (2,), (7,)), ('O', 3, 3), ('Q', 1), ('O', 3, 1), ('P2', 2, (2,), (0,)), ('QK', 0, 1, 0), ('P2', 2, (2,), (1,)), ('P2', 2, (2,), (2,)), ('QK', 0, 1, 1), ('QK', 1, 1, 0), ('O', 3, 0), ('P2', 2, (2,), (6,)), ('SM', 0, 1, 0), ('P2', 2, (2,), (3,)), ('QK', 1, 1, 1), ('SM', 0, 1, 1), ('PV', 0, 1, 0), ('SM', 1, 1, 0), ('PV', 0, 1, 1), ('SM', 1, 1, 1), ('PV', 1, 1, 0), ('Q', 0), ('UQ',), ('PV', 1, 1, 1), ('P2', 2, (2,), (4,)), ('O', 2, 0), ('O', 2, 2), ('O', 2, 1), ('O', 2, 3), ('P2', 2, (2,), (5,)), ('QK', 0, 0, 0), ('O', 1, 2), ('QK', 0, 0, 1), ('P2', 2, (2,), (7,)), ('QK', 1, 0, 0), ('SM', 0, 0, 0), ('QK', 1, 0, 1), ('SM', 1, 0, 0), ('O', 1, 0), ('O', 1, 3), ('O', 1, 1), ('PV', 0, 0, 0), ('SM', 0, 0, 1), ('PV', 0, 0, 1), ('SM', 1, 0, 1), ('PV', 1, 0, 0), ('PV', 1, 0, 1), ('KV', 7), ('O', 0, 1), ('O', 0, 2), ('O', 0, 3), ('O', 0, 0)]


_CONSTS = _np_consts()


def make():
    M, Mi, A, Ai = _CONSTS
    anyspec = pl.BlockSpec(memory_space=pl.ANY)
    V = pltpu.VMEM
    call = pl.pallas_call(
        _kernel,
        in_specs=[anyspec] * 13, out_specs=anyspec,
        out_shape=jax.ShapeDtypeStruct((64, 32, 2 * DM), bf16),
        scratch_shapes=[
            V((S // 2, DM), u32), V((S // 2, DC), u32), V((5 * S // 4, 512), u32),
            V((2, DM, D), u32), V((2, DC, D), u32), V((2, DC, D), u32), V((2, 128, DM), u32),
            V((7 * 256, 128), u32), V((7 * 64, 7 * 128), u32), V((7 * 64, 512), u32),
            V((S // 2, 256), u32), V((S // 2, 256), u32), V((S // 2, 256), u32), V((S // 4, 7 * 128), u32), V((S, DM), f32),
            V((8, 128, DM), u32), V((2 * 64, DM), u32), V((20 * 64, 128), u32), V((2, 16, 512, 128), bf16), V((2, 1, S), bf16), V((2, 5, S, 128), f32),
            V((32, 2, 5, 72, 128), f32),
            V((8, 128, 128), bf16), V((8, 128, 128), bf16), V((32, 128, 128), bf16), V((32, 128, 128), bf16),
            V((8, 128, DM), u32), V((8, 8, 32, DM), bf16), V((7 * 256, 7 * 128), u32),
            pltpu.SemaphoreType.DMA((8, 2)), pltpu.SemaphoreType.DMA((4, 2)), pltpu.SemaphoreType.DMA((3, 8)),
            pltpu.SemaphoreType.DMA((2, 17)), pltpu.SemaphoreType.DMA((3, 8)), pltpu.SemaphoreType.DMA((2, 8)),
        ],
        compiler_params=pltpu.CompilerParams(vmem_limit_bytes=110 * 1024 * 1024),
    )

    def f(A_x, A_c_kv, A_w_q, A_w_uk, A_w_uv, A_w_o, B_x, B_w_r, B_w_i):
        o = call(A_x.reshape(S, DM), A_c_kv.reshape(S, DC), A_w_q, A_w_uk, A_w_uv, A_w_o.reshape(NPAIR, 256, DM),
                 B_x.reshape(64, 32, DM), B_w_r.T, B_w_i.T, M, Mi, A, Ai)
        return o.reshape(1, S, 2 * DM)
    return f


_CALL = make()


@jax.jit
def pallas_concat_heads__compressed_kv_cla__spectral_gfnet__prompt_kernel(
        A_x, A_c_kv, A_w_q, A_w_uk, A_w_uv, A_w_o, B_x, B_w_r, B_w_i):
    return _CALL(A_x, A_c_kv, A_w_q, A_w_uk, A_w_uv, A_w_o, B_x, B_w_r, B_w_i)
```
